```python
import jax
import jax.numpy as jnp

def _softmax(x, axis=-1):
    return jax.nn.softmax(x, axis=axis)

def _gelu(x):
    return jax.nn.gelu(x, approximate=True)

def _silu(x):
    return jax.nn.silu(x)

def _sigmoid(x):
    return jax.nn.sigmoid(x)

def _layernorm(x, axis=-1, eps=1e-05):
    m = jnp.mean(x, axis=axis, keepdims=True)
    v = jnp.var(x, axis=axis, keepdims=True)
    return (x - m) / jnp.sqrt(v + eps)

def _scatter_add(tgt, idx, src, axis=0):
    return tgt.at[idx].add(src)

def _segment_sum(src, seg, n):
    return jax.ops.segment_sum(src, seg, n)

class _Rng:

    def __init__(self, key):
        self._k = key

    def _next(self):
        self._k, sub = jax.random.split(self._k)
        return sub

    def normal(self, shape):
        return jax.random.normal(self._next(), shape, dtype=jnp.bfloat16)

    def randint(self, lo, hi, shape):
        return jax.random.randint(self._next(), shape, lo, hi, dtype=jnp.int32)

    def uniform(self, shape, lo=0.0, hi=1.0):
        return jax.random.uniform(self._next(), shape, jnp.bfloat16, lo, hi)

    def permutation(self, n):
        return jax.random.permutation(self._next(), n)
kernel_name = 'interleave_layers__memory_aug_infini_attn__moe_arch_mod__prompt'

def setup_inputs():
    _rng = _Rng(jax.random.key(int.from_bytes(__import__("os").urandom(4), "little")))
    _w = lambda a: (lambda t: t.astype(jnp.bfloat16) if jnp.issubdtype(t.dtype, jnp.floating) else t)(jnp.asarray(a))

    def _A_setup():
        B, S, D, H = (1, 2048, 1024, 32)
        N = 4
        L = max(1, S // N)
        sc = D ** (-0.5)
        return {'x': _w((lambda *s: _rng.normal(s) * 0.05)(B, N * L, D)), 'wq': _w((lambda *s: _rng.normal(s) * 0.05)(D, D) * sc), 'wk': _w((lambda *s: _rng.normal(s) * 0.05)(D, D) * sc), 'wv': _w((lambda *s: _rng.normal(s) * 0.05)(D, D) * sc), 'wo': _w((lambda *s: _rng.normal(s) * 0.05)(D, D) * sc), 'beta': _w((lambda *s: _rng.normal(s) * 0.05)(H))}
    _A_in = _A_setup()

    def _B_setup():
        B, S, D, F, C = (1, 2048, 1024, 3584, 2)
        return {'x': _w((lambda *s: _rng.normal(s) * 0.05)(B, S, D)), 'w_r': _w((lambda *s: _rng.normal(s) * 0.05)(D)), 'w_gate': _w((lambda *s: _rng.normal(s) * 0.05)(D, F)), 'w_up': _w((lambda *s: _rng.normal(s) * 0.05)(D, F)), 'w_down': _w((lambda *s: _rng.normal(s) * 0.05)(F, D))}
    _B_in = _B_setup()
    return {'A_x': _A_in['x'], 'A_wq': _A_in['wq'], 'A_wk': _A_in['wk'], 'A_wv': _A_in['wv'], 'A_wo': _A_in['wo'], 'A_beta': _A_in['beta'], 'B_x': _B_in['x'], 'B_w_r': _B_in['w_r'], 'B_w_gate': _B_in['w_gate'], 'B_w_up': _B_in['w_up'], 'B_w_down': _B_in['w_down']}

def reference(A_x, A_wq, A_wk, A_wv, A_wo, A_beta, B_x, B_w_r, B_w_gate, B_w_up, B_w_down):

    def _A_ref(x, wq, wk, wv, wo, beta):
        B, S, D = x.shape
        H = 32
        Dh = D // H
        N = 4
        L = S // N
        q = (lambda x, *d: x.transpose(*d))((x @ wq).reshape(B, S, H, Dh), 0, 2, 1, 3).reshape(B, H, N, L, Dh)
        k = (lambda x, *d: x.transpose(*d))((x @ wk).reshape(B, S, H, Dh), 0, 2, 1, 3).reshape(B, H, N, L, Dh)
        v = (lambda x, *d: x.transpose(*d))((x @ wv).reshape(B, S, H, Dh), 0, 2, 1, 3).reshape(B, H, N, L, Dh)
        phi = lambda t: jnp.where(t > 0, t + 1.0, jnp.exp(t))
        scale = Dh ** (-0.5)
        ar = jnp.arange(L)
        mask = (lambda x, dt: x.astype(dt))(ar[:, None] < ar[None, :], x.dtype) * -1000000000.0
        g = _sigmoid(beta).reshape(1, H, 1, 1)
        M = jnp.einsum('bhd,bhe->bhde', q[:, :, 0, 0, :] * 0.0, q[:, :, 0, 0, :] * 0.0)
        z = q[:, :, 0, 0, :] * 0.0
        outs = []
        for s in range(N):
            qs, ks, vs = (q[:, :, s].copy(), k[:, :, s].copy(), v[:, :, s].copy())
            logits = jnp.einsum('bhqd,bhkd->bhqk', qs, ks) * scale + mask
            p = _softmax(logits, axis=-1)
            a_dot = jnp.einsum('bhqk,bhkd->bhqd', p, vs)
            pq = phi(qs)
            num = jnp.einsum('bhld,bhde->bhle', pq, M)
            den = jnp.einsum('bhld,bhd->bhl', pq, z)[..., None] + 1e-06
            a_mem = num / den
            o = g * a_mem + (1.0 - g) * a_dot
            outs.append(o)
            pk = phi(ks)
            M = M + jnp.einsum('bhld,bhle->bhde', pk, vs)
            z = z + jnp.einsum('bhld->bhd', pk)
        o = (lambda x, *d: x.transpose(*d))(jnp.stack(outs, 2).reshape(B, H, S, Dh), 0, 2, 1, 3).reshape(B, S, D)
        return o @ wo

    def _B_ref(x, w_r, w_gate, w_up, w_down):
        B, S, D = x.shape
        C = 2
        r = x @ w_r
        idx = jnp.argsort(-r, axis=-1)[:, :C]
        idx_e = jnp.repeat(idx.reshape(B, C, 1), D, axis=2)
        x_sel = jnp.take_along_axis(x, idx_e, axis=1)
        g = _silu(x_sel @ w_gate)
        u = x_sel @ w_up
        y = g * u @ w_down
        r_sel = _sigmoid(jnp.take_along_axis(r, idx, axis=1))
        y = y * r_sel.reshape(B, C, 1)
        b_off = (jnp.arange(B) * S).reshape(B, 1)
        flat_idx = (idx + b_off).reshape(B * C)
        zero = (x * 0.0).reshape(B * S, D)
        upd = _scatter_add(zero, flat_idx, y.reshape(B * C, D), axis=0)
        return x + upd.reshape(B, S, D)
    x = A_x
    x = x + _A_ref(_layernorm(x, axis=-1), A_wq, A_wk, A_wv, A_wo, A_beta)
    x = x + _B_ref(_layernorm(x, axis=-1), B_w_r, B_w_gate, B_w_up, B_w_down)
    x = x + _A_ref(_layernorm(x, axis=-1), A_wq, A_wk, A_wv, A_wo, A_beta)
    x = x + _B_ref(_layernorm(x, axis=-1), B_w_r, B_w_gate, B_w_up, B_w_down)
    return x
```

```python
import math

import jax
import jax.numpy as jnp
from jax import lax
import jax.experimental.pallas as pl
import jax.experimental.pallas.tpu as pltpu

S = 2048
D = 1024
H = 32
DH = D // H
NSEG = 4
L = S // NSEG
G = 8
F = 3584
XCH = 256
OB = 256
FCH = 512

bf16 = jnp.bfloat16
f32 = jnp.float32
i32 = jnp.int32

QSCALE = (DH ** -0.5) * math.log2(math.e)
SAFE_BOUND = 24.0
NEG = -1e30
EPS_BF16 = 1.0013580322265625e-05

_NT = (((1,), (1,)), ((), ()))


def _r(x):
    return x.astype(bf16).astype(f32)


def _layernorm(xf):
    mean = jnp.sum(xf, axis=1, keepdims=True) * (1.0 / D)
    c = xf - mean
    var = jnp.sum(c * c, axis=1, keepdims=True) * (1.0 / D)
    d = _r(xf - _r(mean))
    s = _r(jnp.sqrt(_r(_r(var) + EPS_BF16)))
    return _r(d * (1.0 / s))


def _phi(t):
    return jnp.where(t > 0, t + 1.0, jnp.exp(t))


def _mask_head_lanes(qt, h):
    qi = pltpu.bitcast(qt, i32)
    lane = lax.broadcasted_iota(i32, qi.shape, 1)
    return pltpu.bitcast(jnp.where((lane >> 5) == h, qi, 0), bf16)


def _fold8(x):
    return x.reshape(x.shape[0] // 8, 8, x.shape[1])


def _kernel(beta_ref, wr_ref,
            x_hbm, wq_hbm, wk_hbm, wv_hbm, wo_hbm, wg_hbm, wu_hbm, wd_hbm,
            out_hbm,
            xa, xn, wq, wk, wv, wo, qs, pq, ks, pk, vt, o_s, y_s, x1_s,
            zs, gt, r_s, wg, wu, wd, sems):
    nx = S // XCH
    x_cp = [pltpu.make_async_copy(x_hbm.at[0, pl.ds(i * XCH, XCH), :],
                                  xa.at[pl.ds(i * XCH, XCH), :], sems.at[i])
            for i in range(nx)]
    w_cp = [pltpu.make_async_copy(src, dst, sems.at[nx + i]) for i, (src, dst) in
            enumerate([(wv_hbm, wv), (wq_hbm, wq), (wk_hbm, wk), (wo_hbm, wo),
                       (wg_hbm, wg), (wu_hbm, wu), (wd_hbm, wd)])]
    for c in x_cp:
        c.start()
    for c in w_cp:
        c.start()

    b = jnp.broadcast_to(beta_ref[...].astype(f32).reshape(1, H), (H, H))
    rr = lax.broadcasted_iota(i32, (H, H), 0)
    cc = lax.broadcasted_iota(i32, (H, H), 1)
    bcol = jnp.sum(jnp.where(rr == cc, b, 0.0), axis=1, keepdims=True)
    gt[...] = _r(jax.nn.sigmoid(jnp.broadcast_to(bcol, (H, 128))))

    for i in range(nx):
        x_cp[i].wait()
        xf = xa[i * XCH:(i + 1) * XCH, :].astype(f32)
        xn[i * XCH:(i + 1) * XCH, :] = _layernorm(xf).astype(bf16)

    for c in w_cp[:4]:
        c.wait()

    lane = lax.broadcasted_iota(i32, (128, 128), 1)
    row = lax.broadcasted_iota(i32, (128, 128), 0)

    def proj_block(s, carry):
        qmax, kmax = carry
        r0 = pl.multiple_of(s * L, L)
        xb = xn[pl.ds(r0, L), :]
        CB = 256
        for c0 in range(0, D, CB):
            v = jnp.dot(xb, wv[:, c0:c0 + CB], preferred_element_type=f32)
            vt[s, c0:c0 + CB, :] = v.astype(bf16).T
        for c0 in range(0, D, CB):
            q = jnp.dot(xb, wq[:, c0:c0 + CB], preferred_element_type=f32)
            k = jnp.dot(xb, wk[:, c0:c0 + CB], preferred_element_type=f32)
            for j in range(CB // 128):
                g = c0 // 128 + j
                qg = q[:, j * 128:(j + 1) * 128]
                kg = k[:, j * 128:(j + 1) * 128]
                qsc = qg * QSCALE
                qs[g, pl.ds(r0, L), :] = qsc.astype(bf16)
                pq[g, pl.ds(r0, L), :] = _phi(qg).astype(bf16)
                ks[g, pl.ds(r0, L), :] = kg.astype(bf16)
                pkg = _phi(kg)
                pk[g, pl.ds(r0, L), :] = pkg.astype(bf16)
                zs[s, g] = jnp.sum(_fold8(pkg), axis=0)
                qmax = jnp.maximum(qmax, jnp.max(_fold8(jnp.abs(qsc)), axis=0))
                kmax = jnp.maximum(kmax, jnp.max(_fold8(jnp.abs(kg)), axis=0))
        return qmax, kmax

    def attn_group(g, use_max):
        g128 = pl.multiple_of(g * 128, 128)
        causal = row <= lane
        gate = [gt[pl.ds(g * 4 + h, 1), :] for h in range(4)]
        blockdiag = (row >> 5) == (lane >> 5)
        lane16 = lax.broadcasted_iota(i32, (16, 128), 1)
        row16 = lax.broadcasted_iota(i32, (16, 128), 0)
        zmask = (lane16 >> 5) == row16

        def qk(s, t):
            qt = qs[g, s * L + t * 128:s * L + (t + 1) * 128, :]
            qm = [_mask_head_lanes(qt, h) for h in range(4)]
            Sc = [[None] * (t + 1) for _ in range(4)]
            for j in range(t + 1):
                kk = ks[g, s * L + j * 128:s * L + (j + 1) * 128, :]
                for h in range(4):
                    Sc[h][j] = lax.dot_general(kk, qm[h], _NT, preferred_element_type=f32)
            return Sc

        def sm(Sc, t):
            P = [None] * 4
            Linv = [None] * 4
            for h in range(4):
                sc = list(Sc[h])
                sc[t] = jnp.where(causal, sc[t], NEG)
                if use_max:
                    m = sc[0]
                    for j in range(1, t + 1):
                        m = jnp.maximum(m, sc[j])
                    m = jnp.max(m, axis=0, keepdims=True)
                    p = [jnp.exp2(x - m) for x in sc]
                else:
                    p = [jnp.exp2(x) for x in sc]
                l = p[0]
                for j in range(1, t + 1):
                    l = l + p[j]
                Linv[h] = 1.0 / jnp.sum(l, axis=0, keepdims=True)
                P[h] = [x.astype(bf16) for x in p]
            return P, Linv

        def pv(PL, s, t, lhs_m):
            P, Linv = PL
            acc = [None] * 4
            for j in range(t + 1):
                for h in range(4):
                    vth = vt[s, pl.ds(g128 + 32 * h, 32), j * 128:(j + 1) * 128]
                    o = jnp.dot(vth, P[h][j], preferred_element_type=f32)
                    acc[h] = o if acc[h] is None else acc[h] + o
            if lhs_m is not None:
                pqt = pq[g, s * L + t * 128:s * L + (t + 1) * 128, :]
                nd = lax.dot_general(lhs_m, pqt, _NT, preferred_element_type=f32)
            outs = []
            for h in range(4):
                o = acc[h] * ((1.0 - gate[h]) * Linv[h])
                if lhs_m is not None:
                    den = nd[128 + h:129 + h, :] + 1e-6
                    o = o + nd[32 * h:32 * h + 32, :] * (gate[h] / den)
                outs.append(o)
            ot = jnp.concatenate(outs, axis=0).astype(bf16)
            o_s[g, s * L + t * 128:s * L + (t + 1) * 128, :] = ot.T

        def mem_update(s, R):
            vtg = vt[s, pl.ds(g128, 128), :]
            upd = jnp.dot(vtg, pk[g, s * L:(s + 1) * L, :], preferred_element_type=f32)
            return upd if R is None else R + upd

        def mem_lhs(s, R):
            mt = jnp.where(blockdiag, R, 0.0)
            z = zs[0, g]
            for s2 in range(1, s):
                z = z + zs[s2, g]
            z = jnp.sum(z, axis=0, keepdims=True)
            zr = jnp.where(zmask, z, 0.0)
            return jnp.concatenate([mt, zr], axis=0).astype(bf16)

        steps = [(s, t) for s in range(NSEG) for t in range(4)]
        n = len(steps)
        Sc, PL = {}, {}
        R = None
        lhs = {0: None}
        for i in range(n + 2):
            if i < n:
                Sc[i] = qk(*steps[i])
                s, t = steps[i]
                if t == 3 and s < NSEG - 1:
                    R = mem_update(s, R)
                    lhs[s + 1] = mem_lhs(s + 1, R)
            if 0 <= i - 1 < n:
                PL[i - 1] = sm(Sc.pop(i - 1), steps[i - 1][1])
            if 0 <= i - 2 < n:
                s, t = steps[i - 2]
                pv(PL.pop(i - 2), s, t, lhs[s])

    wr = wr_ref[...].astype(f32).reshape(1, D)

    def oproj_block(i, carry):
        r0 = pl.multiple_of(i * OB, OB)
        ob = jnp.concatenate([o_s[g, pl.ds(r0, OB), :] for g in range(G)], axis=1)
        out = jnp.dot(ob, wo[...], preferred_element_type=f32)
        x1 = _r(xa[pl.ds(r0, OB), :].astype(f32) + _r(out))
        x1_s[pl.ds(r0, OB), :] = x1.astype(bf16)
        y = _layernorm(x1)
        y_s[pl.ds(r0, OB), :] = y.astype(bf16)
        rcol = _r(jnp.sum(y * wr, axis=1, keepdims=True))
        for c in range(OB // 128):
            rb = jnp.broadcast_to(rcol[c * 128:(c + 1) * 128], (128, 128))
            rrow = jnp.sum(jnp.where(row == lane, rb, 0.0), axis=0, keepdims=True)
            r_s[pl.ds(i * (OB // 128) + c, 1), :] = rrow
        x2 = _r(x1 + y)
        xa[pl.ds(r0, OB), :] = x2.astype(bf16)
        xn[pl.ds(r0, OB), :] = _layernorm(x2).astype(bf16)
        return carry

    def moe_phase():
        r_all = r_s[...]
        ridx = (lax.broadcasted_iota(i32, r_all.shape, 0) * 128
                + lax.broadcasted_iota(i32, r_all.shape, 1))
        ridx_f = ridx.astype(f32)
        m1 = jnp.max(r_all)
        i1f = jnp.min(jnp.where(r_all == m1, ridx_f, 1e9))
        r2 = jnp.where(ridx_f == i1f, -jnp.inf, r_all)
        m2 = jnp.max(r2)
        i2f = jnp.min(jnp.where((r2 == m2) & (ridx_f != i1f), ridx_f, 1e9))
        idx = [jnp.clip(i1f.astype(i32), 0, S - 1), jnp.clip(i2f.astype(i32), 0, S - 1)]
        base = [pl.multiple_of((ix >> 4) << 4, 16) for ix in idx]
        off = [ix & 15 for ix in idx]
        row16 = lax.broadcasted_iota(i32, (16, D), 0)

        def gather(ref):
            res = None
            for kk in range(2):
                blk = ref[pl.ds(base[kk], 16), :].astype(f32)
                one = jnp.sum(jnp.where(row16 == off[kk], blk, 0.0), axis=0, keepdims=True)
                part = jnp.where(row16 == kk, one, 0.0)
                res = part if res is None else res + part
            return res

        ysel = gather(y_s)
        x1sel = gather(x1_s)
        xsel = ysel.astype(bf16)
        yf = None
        for c0 in range(0, F, FCH):
            gte = _r(jnp.dot(xsel, wg[:, c0:c0 + FCH], preferred_element_type=f32))
            up = _r(jnp.dot(xsel, wu[:, c0:c0 + FCH], preferred_element_type=f32))
            act = _r(gte * jax.nn.sigmoid(gte))
            hcol = (act * up).astype(bf16)
            part = jnp.dot(hcol, wd[c0:c0 + FCH, :], preferred_element_type=f32)
            yf = part if yf is None else yf + part
        rsel = _r(jax.nn.sigmoid(jnp.where(row16 == 0, m1, m2)))
        upd = _r(_r(yf) * rsel)
        x2 = _r(x1sel + _r(ysel + upd))
        xn2 = _layernorm(x2)
        for ref, val in ((xa, x2), (xn, xn2)):
            for kk in range(2):
                one = jnp.sum(jnp.where(row16 == kk, val, 0.0), axis=0, keepdims=True)
                blk = ref[pl.ds(base[kk], 16), :].astype(f32)
                ref[pl.ds(base[kk], 16), :] = jnp.where(row16 == off[kk], one, blk).astype(bf16)

    def layer(li, carry):
        z8 = jnp.zeros((8, 128), f32)
        qmax, kmax = lax.fori_loop(0, NSEG, proj_block, (z8, z8))
        bound = DH * jnp.max(qmax) * jnp.max(kmax)
        safe = bound <= SAFE_BOUND

        @pl.when(safe)
        def _():
            lax.fori_loop(0, G, lambda g, c: (attn_group(g, False), c)[1], 0)

        @pl.when(jnp.logical_not(safe))
        def _():
            lax.fori_loop(0, G, lambda g, c: (attn_group(g, True), c)[1], 0)

        lax.fori_loop(0, S // OB, oproj_block, 0)

        @pl.when(li == 0)
        def _():
            for c in w_cp[4:]:
                c.wait()

        moe_phase()
        return carry

    lax.fori_loop(0, 2, layer, 0)

    oc = pltpu.make_async_copy(xa, out_hbm.at[0], sems.at[0])
    oc.start()
    oc.wait()


@jax.jit
def pallas_interleave_layers__memory_aug_infini_attn__moe_arch_mod__prompt_kernel(
    A_x: jax.Array,
    A_wq: jax.Array,
    A_wk: jax.Array,
    A_wv: jax.Array,
    A_wo: jax.Array,
    A_beta: jax.Array,
    B_x: jax.Array,
    B_w_r: jax.Array,
    B_w_gate: jax.Array,
    B_w_up: jax.Array,
    B_w_down: jax.Array,
):
    del B_x
    any_spec = pl.BlockSpec(memory_space=pl.ANY)
    vm = pltpu.VMEM
    return pl.pallas_call(
        _kernel,
        out_shape=jax.ShapeDtypeStruct((1, S, D), bf16),
        in_specs=[pl.BlockSpec(memory_space=vm), pl.BlockSpec(memory_space=vm)] + [any_spec] * 8,
        out_specs=any_spec,
        scratch_shapes=[
            vm((S, D), bf16), vm((S, D), bf16),
            vm((D, D), bf16), vm((D, D), bf16), vm((D, D), bf16), vm((D, D), bf16),
            vm((G, S, 128), bf16), vm((G, S, 128), bf16),
            vm((G, S, 128), bf16), vm((G, S, 128), bf16),
            vm((NSEG, D, L), bf16),
            vm((G, S, 128), bf16),
            vm((S, D), bf16), vm((S, D), bf16),
            vm((NSEG, G, 8, 128), f32),
            vm((H, 128), f32),
            vm((S // 128, 128), f32),
            vm((D, F), bf16), vm((D, F), bf16), vm((F, D), bf16),
            pltpu.SemaphoreType.DMA((S // XCH + 7,)),
        ],
        compiler_params=pltpu.CompilerParams(vmem_limit_bytes=110 * 1024 * 1024),
    )(A_beta, B_w_r, A_x, A_wq, A_wk, A_wv, A_wo, B_w_gate, B_w_up, B_w_down)
```

```python
import math

import jax
import jax.numpy as jnp
from jax import lax
import jax.experimental.pallas as pl
import jax.experimental.pallas.tpu as pltpu

S = 2048
D = 1024
H = 32
DH = D // H
NSEG = 4
L = S // NSEG
G = 8
F = 3584
OB = 64
OSTEP = 6
ONP = 4
AG = 2
LAG = 2
FCH = 512

bf16 = jnp.bfloat16
f32 = jnp.float32
i32 = jnp.int32

QSCALE = (DH ** -0.5) * math.log2(math.e)
SAFE_BOUND = 24.0
NEG = -1e30
EPS_BF16 = 1.0013580322265625e-05

_NT = (((1,), (1,)), ((), ()))


def _r(x):
    return x.astype(bf16).astype(f32)


def _pack(x):
    return pltpu.bitcast(x.astype(bf16), i32)


def _unpack(w):
    return pltpu.bitcast(w, bf16)


def _layernorm(xf):
    mean = jnp.sum(xf, axis=1, keepdims=True) * (1.0 / D)
    c = xf - mean
    var = jnp.sum(c * c, axis=1, keepdims=True) * (1.0 / D)
    d = _r(xf - _r(mean))
    s = _r(jnp.sqrt(_r(_r(var) + EPS_BF16)))
    return _r(d * (1.0 / s))


def _phi(t):
    return jnp.where(t > 0, t + 1.0, jnp.exp(t))


def _head_lanes(qi, h):
    lane = lax.broadcasted_iota(i32, qi.shape, 1)
    return _unpack(jnp.where((lane >> 5) == h, qi, 0))


def _fold8(x):
    return x.reshape(x.shape[0] // 8, 8, x.shape[1])


def _half(i, n):
    return pl.ds(i // 2 if isinstance(i, int) else pl.multiple_of(i // 2, n // 2), n // 2)


def _kernel(beta_ref, wr_ref,
            x_hbm, wq_hbm, wk_hbm, wv_hbm, wo_hbm, wg_hbm, wu_hbm, wd_hbm,
            out_hbm,
            xio, wst, xa, xn, wq, wk, wv, wo, qs, pq, ks, pk, vt, o_s, y_s, x1_s,
            zs, gt, r_s, oc, wg, wu, wd, sems):
    nx = NSEG
    x_cp = [pltpu.make_async_copy(x_hbm.at[0, pl.ds(i * L, L), :],
                                  xio.at[pl.ds(i * L, L), :], sems.at[i])
            for i in range(nx)]
    w_cp = [pltpu.make_async_copy(src, dst, sems.at[nx + i]) for i, (src, dst) in
            enumerate([(wv_hbm, wst.at[0]), (wq_hbm, wst.at[1]), (wk_hbm, wst.at[2]),
                       (wo_hbm, wst.at[3]), (wg_hbm, wg), (wu_hbm, wu), (wd_hbm, wd)])]
    x_cp[0].start()
    w_cp[0].start()
    for c in x_cp[1:]:
        c.start()
    for c in w_cp[1:]:
        c.start()

    b = jnp.broadcast_to(beta_ref[...].astype(f32).reshape(1, H), (H, H))
    rr = lax.broadcasted_iota(i32, (H, H), 0)
    cc = lax.broadcasted_iota(i32, (H, H), 1)
    bcol = jnp.sum(jnp.where(rr == cc, b, 0.0), axis=1, keepdims=True)
    gt[...] = _r(jax.nn.sigmoid(jnp.broadcast_to(bcol, (H, 128))))

    lane = lax.broadcasted_iota(i32, (128, 128), 1)
    row = lax.broadcasted_iota(i32, (128, 128), 0)

    def widen_x(r0):
        xa[pl.ds(r0, L), :] = xio[pl.ds(r0, L), :].astype(f32)

    def ln_block(r0):
        xn[_half(r0, L), :] = _pack(_layernorm(xa[pl.ds(r0, L), :]))

    def repack(i, dst):
        dst[...] = _pack(wst[i])

    def vproj_block(s, li):
        nxt = pl.multiple_of(jnp.minimum(s + 1, NSEG - 1) * L, L)
        if li == 0:
            for i in range(1, nx):
                @pl.when(s == i - 1)
                def _():
                    x_cp[i].wait()
                    widen_x(i * L)

        r0 = pl.multiple_of(s * L, L)
        xb = _unpack(xn[_half(r0, L), :])
        CB = 256
        for c0 in range(0, D, CB):
            v = jnp.dot(xb, _unpack(wv[:, c0:c0 + CB]), preferred_element_type=f32)
            vt[s, c0 // 2:(c0 + CB) // 2, :] = pltpu.bitcast(v.astype(bf16).T, i32)
        ln_block(nxt)

    def qkproj_block(s, carry):
        qmax, kmax = carry
        r0 = pl.multiple_of(s * L, L)
        xb = _unpack(xn[_half(r0, L), :])
        CB = 256
        for c0 in range(0, D, CB):
            q = jnp.dot(xb, _unpack(wq[:, c0:c0 + CB]), preferred_element_type=f32)
            k = jnp.dot(xb, _unpack(wk[:, c0:c0 + CB]), preferred_element_type=f32)
            for j in range(CB // 128):
                g = c0 // 128 + j
                qg = q[:, j * 128:(j + 1) * 128]
                kg = k[:, j * 128:(j + 1) * 128]
                qsc = qg * QSCALE
                qs[g, _half(r0, L), :] = _pack(qsc)
                pq[g, _half(r0, L), :] = _pack(_phi(qg))
                ks[g, _half(r0, L), :] = _pack(kg)
                pkg = _phi(kg)
                pk[g, _half(r0, L), :] = _pack(pkg)
                zs[s, g] = jnp.sum(_fold8(pkg), axis=0)
                qmax = jnp.maximum(qmax, jnp.max(_fold8(jnp.abs(qsc)), axis=0))
                kmax = jnp.maximum(kmax, jnp.max(_fold8(jnp.abs(kg)), axis=0))
        return qmax, kmax

    def attn_groups(g0, ng, use_max):
        causal = row <= lane
        gs = [g0 + i for i in range(ng)]
        g64 = [pl.multiple_of(g * 64, 64) for g in gs]
        gate = [[gt[pl.ds(g * 4 + h, 1), :] for h in range(4)] for g in gs]
        blockdiag = (row >> 5) == (lane >> 5)
        lane16 = lax.broadcasted_iota(i32, (16, 128), 1)
        row16 = lax.broadcasted_iota(i32, (16, 128), 0)
        zmask = (lane16 >> 5) == row16

        def tile(ref, g, s, t):
            return ref[g, (s * L + t * 128) // 2:(s * L + (t + 1) * 128) // 2, :]

        def qk(gi, s, t):
            g = gs[gi]
            qt = tile(qs, g, s, t)
            qm = [_head_lanes(qt, h) for h in range(4)]
            Sc = [[None] * (t + 1) for _ in range(4)]
            for j in range(t + 1):
                kk = _unpack(tile(ks, g, s, j))
                for h in range(4):
                    Sc[h][j] = lax.dot_general(kk, qm[h], _NT, preferred_element_type=f32)
            return Sc

        def sm(Sc, t):
            P = [None] * 4
            Linv = [None] * 4
            for h in range(4):
                sc = list(Sc[h])
                sc[t] = jnp.where(causal, sc[t], NEG)
                if use_max:
                    m = sc[0]
                    for j in range(1, t + 1):
                        m = jnp.maximum(m, sc[j])
                    m = jnp.max(m, axis=0, keepdims=True)
                    p = [jnp.exp2(x - m) for x in sc]
                else:
                    p = [jnp.exp2(x) for x in sc]
                l = p[0]
                for j in range(1, t + 1):
                    l = l + p[j]
                Linv[h] = 1.0 / jnp.sum(l, axis=0, keepdims=True)
                P[h] = [x.astype(bf16) for x in p]
            return P, Linv

        def pv(PL, gi, s, t, lhs_m):
            g = gs[gi]
            P, Linv = PL
            acc = [None] * 4
            for j in range(t + 1):
                for h in range(4):
                    vth = _unpack(vt[s, pl.ds(g64[gi] + 16 * h, 16), j * 128:(j + 1) * 128])
                    o = jnp.dot(vth, P[h][j], preferred_element_type=f32)
                    acc[h] = o if acc[h] is None else acc[h] + o
            if lhs_m is not None:
                pqt = _unpack(tile(pq, g, s, t))
                nd = lax.dot_general(lhs_m, pqt, _NT, preferred_element_type=f32)
            outs = []
            for h in range(4):
                o = acc[h] * ((1.0 - gate[gi][h]) * Linv[h])
                if lhs_m is not None:
                    den = nd[128 + h:129 + h, :] + 1e-6
                    o = o + nd[32 * h:32 * h + 32, :] * (gate[gi][h] / den)
                outs.append(o)
            ot = jnp.concatenate(outs, axis=0).astype(bf16)
            o_s[g, (s * L + t * 128) // 2:(s * L + (t + 1) * 128) // 2, :] = (
                pltpu.bitcast(ot.T, i32))

        def mem_update(gi, s, R):
            g = gs[gi]
            vtg = _unpack(vt[s, pl.ds(g64[gi], 64), :])
            pks = _unpack(pk[g, s * L // 2:(s + 1) * L // 2, :])
            upd = jnp.dot(vtg, pks, preferred_element_type=f32)
            return upd if R is None else R + upd

        def mem_lhs(gi, s, R):
            g = gs[gi]
            mt = jnp.where(blockdiag, R, 0.0)
            z = zs[0, g]
            for s2 in range(1, s):
                z = z + zs[s2, g]
            z = jnp.sum(z, axis=0, keepdims=True)
            zr = jnp.where(zmask, z, 0.0)
            return jnp.concatenate([mt, zr], axis=0).astype(bf16)

        steps = [(gi, s, t) for gi in range(ng) for s in range(NSEG) for t in range(4)]
        n = len(steps)
        Sc, PL = {}, {}
        R = None
        lhs = {}
        for i in range(n + LAG):
            if i < n:
                Sc[i] = qk(*steps[i])
                gi, s, t = steps[i]
                if t == 0 and s == 0:
                    R = None
                    lhs[gi, 0] = None
                if t == 3 and s < NSEG - 1:
                    R = mem_update(gi, s, R)
                    lhs[gi, s + 1] = mem_lhs(gi, s + 1, R)
                PL[i] = sm(Sc.pop(i), t)
            if 0 <= i - LAG < n:
                gi, s, t = steps[i - LAG]
                pv(PL.pop(i - LAG), gi, s, t, lhs[gi, s])

    wr = wr_ref[...].astype(f32).reshape(1, D)
    CP, RP = D // ONP, OB // ONP
    lane_ob = lax.broadcasted_iota(i32, (OB, 128), 1)
    row_ob = lax.broadcasted_iota(i32, (OB, 128), 0)

    def o_lhs(r0):
        return jnp.concatenate([_unpack(o_s[g, _half(r0, OB), :]) for g in range(G)], axis=1)

    def o_epilogue(refs, r0, out, last):
        xa_, x1_, y_, xo_ = refs
        x1 = _r(xa_[r0:r0 + RP, :] + _r(out))
        x1_[r0 // 2:(r0 + RP) // 2, :] = _pack(x1)
        y = _layernorm(x1)
        y_[r0 // 2:(r0 + RP) // 2, :] = _pack(y)
        if last:
            xo_[r0:r0 + RP, :] = (x1 + y).astype(bf16)
        else:
            xa_[r0:r0 + RP, :] = _r(x1 + y)
        return _r(jnp.sum(y * wr, axis=1, keepdims=True))

    def o_refs(r0, n):
        return [xa.at[pl.ds(r0, n)], x1_s.at[_half(r0, n)], y_s.at[_half(r0, n)],
                xio.at[pl.ds(r0, n)]]

    def o_step(refs, k, blk, src, dst, last):
        if dst is not None:
            ob = o_lhs((blk + 1) * OB)
        rcols = []
        for p in range(ONP):
            if dst is not None:
                dst[:, p * CP:(p + 1) * CP] = jnp.dot(
                    ob, _unpack(wo[:, p * CP:(p + 1) * CP]), preferred_element_type=f32)
            rcols.append(o_epilogue(refs, k * OB + p * RP, src[p * RP:(p + 1) * RP, :], last))
        rb = jnp.broadcast_to(jnp.concatenate(rcols, axis=0), (OB, 128))
        r_s[pl.ds(blk, 1), :] = jnp.max(jnp.where(row_ob == lane_ob, rb, -jnp.inf),
                                        axis=0, keepdims=True)

    def o_phase(last):
        nb = S // OB
        oc[0] = jnp.dot(o_lhs(0), _unpack(wo[...]), preferred_element_type=f32)
        nloop = (nb - 2) // OSTEP
        assert nloop * OSTEP == nb - 2 and OSTEP % 2 == 0

        def body(i, carry):
            refs = o_refs(pl.multiple_of(i * OSTEP * OB, OSTEP * OB), OSTEP * OB)
            for k in range(OSTEP):
                o_step(refs, k, i * OSTEP + k, oc.at[k % 2], oc.at[(k + 1) % 2], last)
            return carry

        lax.fori_loop(0, nloop, body, 0)
        refs = o_refs((nb - 2) * OB, 2 * OB)
        o_step(refs, 0, nb - 2, oc.at[0], oc.at[1], last)
        o_step(refs, 1, nb - 1, oc.at[1], None, last)

    out_cp = pltpu.make_async_copy(xio, out_hbm.at[0], sems.at[2])

    def moe_phase(last):
        r_all = r_s[...]
        ridx = (lax.broadcasted_iota(i32, r_all.shape, 0) * OB
                + lax.broadcasted_iota(i32, r_all.shape, 1)).astype(f32)
        m1 = jnp.max(r_all)
        i1f = jnp.min(jnp.where(r_all == m1, ridx, 1e9))
        r2 = jnp.where(ridx == i1f, -jnp.inf, r_all)
        m2 = jnp.max(r2)
        i2f = jnp.min(jnp.where((r2 == m2) & (ridx != i1f), ridx, 1e9))
        idx = [jnp.clip(i1f.astype(i32), 0, S - 1), jnp.clip(i2f.astype(i32), 0, S - 1)]
        base = [pl.multiple_of((ix >> 4) << 4, 16) for ix in idx]
        off = [ix & 15 for ix in idx]
        row16 = lax.broadcasted_iota(i32, (16, D), 0)

        def gather(ref):
            res = None
            for kk in range(2):
                blk = _unpack(ref[_half(base[kk], 16), :]).astype(f32)
                one = jnp.sum(jnp.where(row16 == off[kk], blk, 0.0), axis=0, keepdims=True)
                part = jnp.where(row16 == kk, one, 0.0)
                res = part if res is None else res + part
            return res

        ysel = gather(y_s)
        x1sel = gather(x1_s)
        xsel = ysel.astype(bf16)
        if not last:
            ln_block(0)
        yf = None
        for c0 in range(0, F, FCH):
            gte = _r(jnp.dot(xsel, wg[:, c0:c0 + FCH], preferred_element_type=f32))
            up = _r(jnp.dot(xsel, wu[:, c0:c0 + FCH], preferred_element_type=f32))
            act = _r(gte * jax.nn.sigmoid(gte))
            hcol = (act * up).astype(bf16)
            part = jnp.dot(hcol, wd[c0:c0 + FCH, :], preferred_element_type=f32)
            yf = part if yf is None else yf + part
        rsel = _r(jax.nn.sigmoid(jnp.where(row16 == 0, m1, m2)))
        upd = _r(_r(yf) * rsel)
        x2 = _r(x1sel + _r(ysel + upd))
        rows2 = [jnp.sum(jnp.where(row16 == kk, x2, 0.0), axis=0, keepdims=True)
                 for kk in range(2)]
        if not last:
            xn2 = _layernorm(x2)
            for kk in range(2):
                xa[pl.ds(idx[kk], 1), :] = rows2[kk]
                one = jnp.sum(jnp.where(row16 == kk, xn2, 0.0), axis=0, keepdims=True)
                blk = _unpack(xn[_half(base[kk], 16), :]).astype(f32)
                xn[_half(base[kk], 16), :] = _pack(jnp.where(row16 == off[kk], one, blk))
        else:
            out_cp.wait()
            for kk in range(2):
                blk = xio[pl.ds(base[kk], 16), :].astype(f32)
                xio[pl.ds(base[kk], 16), :] = jnp.where(
                    row16 == off[kk], rows2[kk], blk).astype(bf16)
            cp0 = pltpu.make_async_copy(xio.at[pl.ds(base[0], 16), :],
                                        out_hbm.at[0, pl.ds(base[0], 16), :], sems.at[0])
            cp1 = pltpu.make_async_copy(xio.at[pl.ds(base[1], 16), :],
                                        out_hbm.at[0, pl.ds(base[1], 16), :], sems.at[1])
            cp0.start()

            @pl.when(base[0] != base[1])
            def _():
                cp1.start()
                cp1.wait()

            cp0.wait()

    x_cp[0].wait()
    widen_x(0)
    ln_block(0)
    w_cp[0].wait()
    repack(0, wv)

    for li in range(2):
        last = li == 1
        lax.fori_loop(0, NSEG, lambda s, c: (vproj_block(s, li), c)[1], 0)
        if li == 0:
            for i, dst in ((1, wq), (2, wk)):
                w_cp[i].wait()
                repack(i, dst)
        z8 = jnp.zeros((8, 128), f32)
        qmax, kmax = lax.fori_loop(0, NSEG, qkproj_block, (z8, z8))
        bound = DH * jnp.max(qmax) * jnp.max(kmax)
        safe = bound <= SAFE_BOUND

        @pl.when(safe)
        def _():
            lax.fori_loop(0, G // AG, lambda i, c: (attn_groups(i * AG, AG, False), c)[1], 0)

        @pl.when(jnp.logical_not(safe))
        def _():
            lax.fori_loop(0, G, lambda g, c: (attn_groups(g, 1, True), c)[1], 0)

        if li == 0:
            w_cp[3].wait()
            repack(3, wo)
        o_phase(last)
        if li == 0:
            for c in w_cp[4:]:
                c.wait()
        else:
            out_cp.start()
        moe_phase(last)


@jax.jit
def pallas_interleave_layers__memory_aug_infini_attn__moe_arch_mod__prompt_kernel(
    A_x: jax.Array,
    A_wq: jax.Array,
    A_wk: jax.Array,
    A_wv: jax.Array,
    A_wo: jax.Array,
    A_beta: jax.Array,
    B_x: jax.Array,
    B_w_r: jax.Array,
    B_w_gate: jax.Array,
    B_w_up: jax.Array,
    B_w_down: jax.Array,
):
    del B_x
    any_spec = pl.BlockSpec(memory_space=pl.ANY)
    vm = pltpu.VMEM
    return pl.pallas_call(
        _kernel,
        out_shape=jax.ShapeDtypeStruct((1, S, D), bf16),
        in_specs=[pl.BlockSpec(memory_space=vm), pl.BlockSpec(memory_space=vm)] + [any_spec] * 8,
        out_specs=any_spec,
        scratch_shapes=[
            vm((S, D), bf16),
            vm((4, D, D), bf16),
            vm((S, D), f32),
            vm((S // 2, D), i32),
            vm((D // 2, D), i32), vm((D // 2, D), i32),
            vm((D // 2, D), i32), vm((D // 2, D), i32),
            vm((G, S // 2, 128), i32), vm((G, S // 2, 128), i32),
            vm((G, S // 2, 128), i32), vm((G, S // 2, 128), i32),
            vm((NSEG, D // 2, L), i32),
            vm((G, S // 2, 128), i32),
            vm((S // 2, D), i32), vm((S // 2, D), i32),
            vm((NSEG, G, 8, 128), f32),
            vm((H, 128), f32),
            vm((S // OB, 128), f32),
            vm((2, OB, D), f32),
            vm((D, F), bf16), vm((D, F), bf16), vm((F, D), bf16),
            pltpu.SemaphoreType.DMA((NSEG + 7,)),
        ],
        compiler_params=pltpu.CompilerParams(vmem_limit_bytes=120 * 1024 * 1024),
    )(A_beta, B_w_r, A_x, A_wq, A_wk, A_wv, A_wo, B_w_gate, B_w_up, B_w_down)
```

```python
import math

import jax
import jax.numpy as jnp
from jax import lax
import jax.experimental.pallas as pl
import jax.experimental.pallas.tpu as pltpu

S = 2048
D = 1024
H = 32
DH = D // H
NSEG = 4
L = S // NSEG
G = 8
F = 3584
OB = 32
OSTEP = 20
ONP = 2
VT_IN_V = 1
AG = 2
LAG = 2
FCH = 512

bf16 = jnp.bfloat16
f32 = jnp.float32
i32 = jnp.int32

QSCALE = (DH ** -0.5) * math.log2(math.e)
SAFE_BOUND = 24.0
NEG = -1e30
EPS_BF16 = 1.0013580322265625e-05

_NT = (((1,), (1,)), ((), ()))
_ONLY = None


def _r(x):
    return x.astype(bf16).astype(f32)


def _pack(x):
    return pltpu.bitcast(x.astype(bf16), i32)


def _unpack(w):
    return pltpu.bitcast(w, bf16)


def _layernorm(xf):
    mean = jnp.sum(xf, axis=1, keepdims=True) * (1.0 / D)
    c = xf - mean
    var = jnp.sum(c * c, axis=1, keepdims=True) * (1.0 / D)
    d = _r(xf - _r(mean))
    s = _r(jnp.sqrt(_r(_r(var) + EPS_BF16)))
    return _r(d * (1.0 / s))


def _phi(t):
    return jnp.where(t > 0, t + 1.0, jnp.exp(t))


def _head_lanes(qi, h):
    lane = lax.broadcasted_iota(i32, qi.shape, 1)
    return _unpack(jnp.where((lane >> 5) == h, qi, 0))


def _fold8(x):
    return x.reshape(x.shape[0] // 8, 8, x.shape[1])


def _half(i, n):
    return pl.ds(i // 2 if isinstance(i, int) else pl.multiple_of(i // 2, n // 2), n // 2)


def _kernel(beta_ref, wr_ref,
            x_hbm, wq_hbm, wk_hbm, wv_hbm, wo_hbm, wg_hbm, wu_hbm, wd_hbm,
            out_hbm,
            xio, wst, xa, xn, vn, wq, wk, wv, wo, qs, pq, ks, pk, vt, o_s, y_s, x1_s,
            zs, gt, r_s, oc, wg, wu, wd, sems):
    nx = NSEG
    x_cp = [pltpu.make_async_copy(x_hbm.at[0, pl.ds(i * L, L), :],
                                  xio.at[pl.ds(i * L, L), :], sems.at[i])
            for i in range(nx)]
    w_cp = [pltpu.make_async_copy(src, dst, sems.at[nx + i]) for i, (src, dst) in
            enumerate([(wv_hbm, wst.at[0]), (wq_hbm, wst.at[1]), (wk_hbm, wst.at[2]),
                       (wo_hbm, wst.at[3]), (wg_hbm, wg), (wu_hbm, wu), (wd_hbm, wd)])]
    x_cp[0].start()
    w_cp[0].start()
    for c in x_cp[1:]:
        c.start()
    for c in w_cp[1:]:
        c.start()

    b = jnp.broadcast_to(beta_ref[...].astype(f32).reshape(1, H), (H, H))
    rr = lax.broadcasted_iota(i32, (H, H), 0)
    cc = lax.broadcasted_iota(i32, (H, H), 1)
    bcol = jnp.sum(jnp.where(rr == cc, b, 0.0), axis=1, keepdims=True)
    gt[...] = _r(jax.nn.sigmoid(jnp.broadcast_to(bcol, (H, 128))))

    lane = lax.broadcasted_iota(i32, (128, 128), 1)
    row = lax.broadcasted_iota(i32, (128, 128), 0)

    def widen_x(r0):
        xa[pl.ds(r0, L), :] = xio[pl.ds(r0, L), :].astype(f32)

    def ln_block(r0):
        xn[_half(r0, L), :] = _pack(_layernorm(xa[pl.ds(r0, L), :]))

    def repack(i, dst):
        dst[...] = _pack(wst[i])

    CB = 256

    def next_block(s):
        return pl.multiple_of(jnp.minimum(s + 1, NSEG - 1) * L, L)

    def vproj_block(s):
        for i in range(1, nx):
            @pl.when(s == i - 1)
            def _():
                x_cp[i].wait()
                widen_x(i * L)

        r0 = pl.multiple_of(s * L, L)
        xb = _unpack(xn[_half(r0, L), :])
        for c0 in range(0, D, CB):
            v = jnp.dot(xb, _unpack(wv[:, c0:c0 + CB]), preferred_element_type=f32)
            if VT_IN_V:
                vt[s, c0 // 2:(c0 + CB) // 2, :] = pltpu.bitcast(v.astype(bf16).T, i32)
            else:
                vn[_half(r0, L), c0:c0 + CB] = _pack(v)
        ln_block(next_block(s))

    def qkproj_block(s, carry, with_v):
        qmax, kmax = carry
        r0 = pl.multiple_of(s * L, L)
        xb = _unpack(xn[_half(r0, L), :])
        for c0 in range(0, D, CB):
            if with_v:
                v = jnp.dot(xb, _unpack(wv[:, c0:c0 + CB]),
                            preferred_element_type=f32).astype(bf16)
            elif VT_IN_V:
                break
            else:
                v = _unpack(vn[_half(r0, L), c0:c0 + CB])
            vt[s, c0 // 2:(c0 + CB) // 2, :] = pltpu.bitcast(v.T, i32)
        for c0 in range(0, D, CB):
            q = jnp.dot(xb, _unpack(wq[:, c0:c0 + CB]), preferred_element_type=f32)
            k = jnp.dot(xb, _unpack(wk[:, c0:c0 + CB]), preferred_element_type=f32)
            for j in range(CB // 128):
                g = c0 // 128 + j
                qg = q[:, j * 128:(j + 1) * 128]
                kg = k[:, j * 128:(j + 1) * 128]
                qsc = qg * QSCALE
                qs[g, _half(r0, L), :] = _pack(qsc)
                pq[g, _half(r0, L), :] = _pack(_phi(qg))
                ks[g, _half(r0, L), :] = _pack(kg)
                pkg = _phi(kg)
                pk[g, _half(r0, L), :] = _pack(pkg)
                zs[s, g] = jnp.sum(_fold8(pkg), axis=0)
                qmax = jnp.maximum(qmax, jnp.max(_fold8(jnp.abs(qsc)), axis=0))
                kmax = jnp.maximum(kmax, jnp.max(_fold8(jnp.abs(kg)), axis=0))
        if with_v:
            ln_block(next_block(s))
        return qmax, kmax

    def attn_groups(g0, ng, use_max):
        causal = row <= lane
        gs = [g0 + i for i in range(ng)]
        g64 = [pl.multiple_of(g * 64, 64) for g in gs]
        gate = [[gt[pl.ds(g * 4 + h, 1), :] for h in range(4)] for g in gs]
        blockdiag = (row >> 5) == (lane >> 5)
        lane16 = lax.broadcasted_iota(i32, (16, 128), 1)
        row16 = lax.broadcasted_iota(i32, (16, 128), 0)
        zmask = (lane16 >> 5) == row16

        def tile(ref, g, s, t):
            return ref[g, (s * L + t * 128) // 2:(s * L + (t + 1) * 128) // 2, :]

        def qk(gi, s, t):
            g = gs[gi]
            qt = tile(qs, g, s, t)
            qm = [_head_lanes(qt, h) for h in range(4)]
            Sc = [[None] * (t + 1) for _ in range(4)]
            for j in range(t + 1):
                kk = _unpack(tile(ks, g, s, j))
                for h in range(4):
                    Sc[h][j] = lax.dot_general(kk, qm[h], _NT, preferred_element_type=f32)
            return Sc

        def sm(Sc, t):
            P = [None] * 4
            Linv = [None] * 4
            for h in range(4):
                sc = list(Sc[h])
                sc[t] = jnp.where(causal, sc[t], NEG)
                if use_max:
                    m = sc[0]
                    for j in range(1, t + 1):
                        m = jnp.maximum(m, sc[j])
                    m = jnp.max(m, axis=0, keepdims=True)
                    p = [jnp.exp2(x - m) for x in sc]
                else:
                    p = [jnp.exp2(x) for x in sc]
                l = p[0]
                for j in range(1, t + 1):
                    l = l + p[j]
                Linv[h] = 1.0 / jnp.sum(l, axis=0, keepdims=True)
                P[h] = [x.astype(bf16) for x in p]
            return P, Linv

        def pv(PL, gi, s, t, lhs_m):
            g = gs[gi]
            P, Linv = PL
            acc = [None] * 4
            for j in range(t + 1):
                for h in range(4):
                    vth = _unpack(vt[s, pl.ds(g64[gi] + 16 * h, 16), j * 128:(j + 1) * 128])
                    o = jnp.dot(vth, P[h][j], preferred_element_type=f32)
                    acc[h] = o if acc[h] is None else acc[h] + o
            if lhs_m is not None:
                pqt = _unpack(tile(pq, g, s, t))
                nd = lax.dot_general(lhs_m, pqt, _NT, preferred_element_type=f32)
            outs = []
            for h in range(4):
                o = acc[h] * ((1.0 - gate[gi][h]) * Linv[h])
                if lhs_m is not None:
                    den = nd[128 + h:129 + h, :] + 1e-6
                    o = o + nd[32 * h:32 * h + 32, :] * (gate[gi][h] / den)
                outs.append(o)
            ot = jnp.concatenate(outs, axis=0).astype(bf16)
            o_s[g, (s * L + t * 128) // 2:(s * L + (t + 1) * 128) // 2, :] = (
                pltpu.bitcast(ot.T, i32))

        def mem_update(gi, s, R):
            g = gs[gi]
            vtg = _unpack(vt[s, pl.ds(g64[gi], 64), :])
            pks = _unpack(pk[g, s * L // 2:(s + 1) * L // 2, :])
            upd = jnp.dot(vtg, pks, preferred_element_type=f32)
            return upd if R is None else R + upd

        def mem_lhs(gi, s, R):
            g = gs[gi]
            mt = jnp.where(blockdiag, R, 0.0)
            z = zs[0, g]
            for s2 in range(1, s):
                z = z + zs[s2, g]
            z = jnp.sum(z, axis=0, keepdims=True)
            zr = jnp.where(zmask, z, 0.0)
            return jnp.concatenate([mt, zr], axis=0).astype(bf16)

        steps = [(gi, s, t) for gi in range(ng) for s in range(NSEG) for t in range(4)]
        n = len(steps)
        Sc, PL = {}, {}
        R = None
        lhs = {}
        for i in range(n + LAG):
            if i < n:
                Sc[i] = qk(*steps[i])
                gi, s, t = steps[i]
                if t == 0 and s == 0:
                    R = None
                    lhs[gi, 0] = None
                if t == 3 and s < NSEG - 1:
                    R = mem_update(gi, s, R)
                    lhs[gi, s + 1] = mem_lhs(gi, s + 1, R)
                PL[i] = sm(Sc.pop(i), t)
            if 0 <= i - LAG < n:
                gi, s, t = steps[i - LAG]
                pv(PL.pop(i - LAG), gi, s, t, lhs[gi, s])

    wr = wr_ref[...].astype(f32).reshape(1, D)
    CP, RP = D // ONP, OB // ONP
    lane_ob = lax.broadcasted_iota(i32, (OB, 128), 1)
    row_ob = lax.broadcasted_iota(i32, (OB, 128), 0)

    def o_lhs(r0):
        return jnp.concatenate([_unpack(o_s[g, _half(r0, OB), :]) for g in range(G)], axis=1)

    def o_epilogue(refs, r0, out, last):
        xa_, x1_, y_, xo_ = refs
        x1 = _r(xa_[r0:r0 + RP, :] + _r(out))
        x1_[r0 // 2:(r0 + RP) // 2, :] = _pack(x1)
        y = _layernorm(x1)
        y_[r0 // 2:(r0 + RP) // 2, :] = _pack(y)
        if last:
            xo_[r0:r0 + RP, :] = (x1 + y).astype(bf16)
        else:
            xa_[r0:r0 + RP, :] = _r(x1 + y)
        return _r(jnp.sum(y * wr, axis=1, keepdims=True))

    def o_refs(r0, n):
        return [xa.at[pl.ds(r0, n)], x1_s.at[_half(r0, n)], y_s.at[_half(r0, n)],
                xio.at[pl.ds(r0, n)]]

    def o_step(refs, k, blk, src, dst, last):
        if dst is not None:
            ob = o_lhs((blk + 1) * OB)
        rcols = []
        for p in range(ONP):
            if dst is not None:
                dst[:, p * CP:(p + 1) * CP] = jnp.dot(
                    ob, _unpack(wo[:, p * CP:(p + 1) * CP]), preferred_element_type=f32)
            rcols.append(o_epilogue(refs, k * OB + p * RP, src[p * RP:(p + 1) * RP, :], last))
        rb = jnp.broadcast_to(jnp.concatenate(rcols, axis=0), (OB, 128))
        r_s[pl.ds(blk, 1), :] = jnp.max(jnp.where(row_ob == lane_ob, rb, -jnp.inf),
                                        axis=0, keepdims=True)

    def o_phase(last):
        nb = S // OB
        oc[0] = jnp.dot(o_lhs(0), _unpack(wo[...]), preferred_element_type=f32)
        nloop = (nb - 2) // OSTEP
        assert OSTEP % 2 == 0

        def body(i, carry):
            refs = o_refs(pl.multiple_of(i * OSTEP * OB, OSTEP * OB), OSTEP * OB)
            for k in range(OSTEP):
                o_step(refs, k, i * OSTEP + k, oc.at[k % 2], oc.at[(k + 1) % 2], last)
            return carry

        lax.fori_loop(0, nloop, body, 0)
        b0 = nloop * OSTEP
        refs = o_refs(b0 * OB, (nb - b0) * OB)
        for k in range(nb - b0):
            o_step(refs, k, b0 + k, oc.at[k % 2],
                   oc.at[(k + 1) % 2] if b0 + k + 1 < nb else None, last)

    out_cp = pltpu.make_async_copy(xio, out_hbm.at[0], sems.at[2])

    def moe_phase(last):
        r_all = r_s[...]
        ridx = (lax.broadcasted_iota(i32, r_all.shape, 0) * OB
                + lax.broadcasted_iota(i32, r_all.shape, 1)).astype(f32)
        m1 = jnp.max(r_all)
        i1f = jnp.min(jnp.where(r_all == m1, ridx, 1e9))
        r2 = jnp.where(ridx == i1f, -jnp.inf, r_all)
        m2 = jnp.max(r2)
        i2f = jnp.min(jnp.where((r2 == m2) & (ridx != i1f), ridx, 1e9))
        idx = [jnp.clip(i1f.astype(i32), 0, S - 1), jnp.clip(i2f.astype(i32), 0, S - 1)]
        base = [pl.multiple_of((ix >> 4) << 4, 16) for ix in idx]
        off = [ix & 15 for ix in idx]
        row16 = lax.broadcasted_iota(i32, (16, D), 0)

        def gather(ref):
            res = None
            for kk in range(2):
                blk = _unpack(ref[_half(base[kk], 16), :]).astype(f32)
                one = jnp.sum(jnp.where(row16 == off[kk], blk, 0.0), axis=0, keepdims=True)
                part = jnp.where(row16 == kk, one, 0.0)
                res = part if res is None else res + part
            return res

        ysel = gather(y_s)
        x1sel = gather(x1_s)
        xsel = ysel.astype(bf16)
        if not last:
            ln_block(0)
        yf = None
        for c0 in range(0, F, FCH):
            gte = _r(jnp.dot(xsel, wg[:, c0:c0 + FCH], preferred_element_type=f32))
            up = _r(jnp.dot(xsel, wu[:, c0:c0 + FCH], preferred_element_type=f32))
            act = _r(gte * jax.nn.sigmoid(gte))
            hcol = (act * up).astype(bf16)
            part = jnp.dot(hcol, wd[c0:c0 + FCH, :], preferred_element_type=f32)
            yf = part if yf is None else yf + part
        rsel = _r(jax.nn.sigmoid(jnp.where(row16 == 0, m1, m2)))
        upd = _r(_r(yf) * rsel)
        x2 = _r(x1sel + _r(ysel + upd))
        rows2 = [jnp.sum(jnp.where(row16 == kk, x2, 0.0), axis=0, keepdims=True)
                 for kk in range(2)]
        if not last:
            xn2 = _layernorm(x2)
            for kk in range(2):
                xa[pl.ds(idx[kk], 1), :] = rows2[kk]
                one = jnp.sum(jnp.where(row16 == kk, xn2, 0.0), axis=0, keepdims=True)
                blk = _unpack(xn[_half(base[kk], 16), :]).astype(f32)
                xn[_half(base[kk], 16), :] = _pack(jnp.where(row16 == off[kk], one, blk))
        else:
            out_cp.wait()
            for kk in range(2):
                blk = xio[pl.ds(base[kk], 16), :].astype(f32)
                xio[pl.ds(base[kk], 16), :] = jnp.where(
                    row16 == off[kk], rows2[kk], blk).astype(bf16)
            cp0 = pltpu.make_async_copy(xio.at[pl.ds(base[0], 16), :],
                                        out_hbm.at[0, pl.ds(base[0], 16), :], sems.at[0])
            cp1 = pltpu.make_async_copy(xio.at[pl.ds(base[1], 16), :],
                                        out_hbm.at[0, pl.ds(base[1], 16), :], sems.at[1])
            cp0.start()

            @pl.when(base[0] != base[1])
            def _():
                cp1.start()
                cp1.wait()

            cp0.wait()

    if _ONLY:
        for c in x_cp + w_cp:
            c.wait()
        dict(O0=lambda: o_phase(False), O1=lambda: o_phase(True),
             B0=lambda: moe_phase(False))[_ONLY]()
        out_cp.start()
        out_cp.wait()
        return

    x_cp[0].wait()
    widen_x(0)
    ln_block(0)
    w_cp[0].wait()
    repack(0, wv)

    for li in range(2):
        last = li == 1
        z8 = jnp.zeros((8, 128), f32)
        if li == 0:
            lax.fori_loop(0, NSEG, lambda s, c: (vproj_block(s), c)[1], 0)
            for i, dst in ((1, wq), (2, wk)):
                w_cp[i].wait()
                repack(i, dst)
            qmax, kmax = lax.fori_loop(
                0, NSEG, lambda s, c: qkproj_block(s, c, False), (z8, z8))
        else:
            qmax, kmax = lax.fori_loop(
                0, NSEG, lambda s, c: qkproj_block(s, c, True), (z8, z8))
        bound = DH * jnp.max(qmax) * jnp.max(kmax)
        safe = bound <= SAFE_BOUND

        @pl.when(safe)
        def _():
            lax.fori_loop(0, G // AG, lambda i, c: (attn_groups(i * AG, AG, False), c)[1], 0)

        @pl.when(jnp.logical_not(safe))
        def _():
            lax.fori_loop(0, G, lambda g, c: (attn_groups(g, 1, True), c)[1], 0)

        if li == 0:
            w_cp[3].wait()
            repack(3, wo)
        o_phase(last)
        if li == 0:
            for c in w_cp[4:]:
                c.wait()
        else:
            out_cp.start()
        moe_phase(last)


@jax.jit
def pallas_interleave_layers__memory_aug_infini_attn__moe_arch_mod__prompt_kernel(
    A_x: jax.Array,
    A_wq: jax.Array,
    A_wk: jax.Array,
    A_wv: jax.Array,
    A_wo: jax.Array,
    A_beta: jax.Array,
    B_x: jax.Array,
    B_w_r: jax.Array,
    B_w_gate: jax.Array,
    B_w_up: jax.Array,
    B_w_down: jax.Array,
):
    del B_x
    any_spec = pl.BlockSpec(memory_space=pl.ANY)
    vm = pltpu.VMEM
    return pl.pallas_call(
        _kernel,
        out_shape=jax.ShapeDtypeStruct((1, S, D), bf16),
        in_specs=[pl.BlockSpec(memory_space=vm), pl.BlockSpec(memory_space=vm)] + [any_spec] * 8,
        out_specs=any_spec,
        scratch_shapes=[
            vm((S, D), bf16),
            vm((4, D, D), bf16),
            vm((S, D), f32),
            vm((S // 2, D), i32),
            vm((S // 2, D), i32),
            vm((D // 2, D), i32), vm((D // 2, D), i32),
            vm((D // 2, D), i32), vm((D // 2, D), i32),
            vm((G, S // 2, 128), i32), vm((G, S // 2, 128), i32),
            vm((G, S // 2, 128), i32), vm((G, S // 2, 128), i32),
            vm((NSEG, D // 2, L), i32),
            vm((G, S // 2, 128), i32),
            vm((S // 2, D), i32), vm((S // 2, D), i32),
            vm((NSEG, G, 8, 128), f32),
            vm((H, 128), f32),
            vm((S // OB, 128), f32),
            vm((2, OB, D), f32),
            vm((D, F), bf16), vm((D, F), bf16), vm((F, D), bf16),
            pltpu.SemaphoreType.DMA((NSEG + 7,)),
        ],
        compiler_params=pltpu.CompilerParams(vmem_limit_bytes=120 * 1024 * 1024),
    )(A_beta, B_w_r, A_x, A_wq, A_wk, A_wv, A_wo, B_w_gate, B_w_up, B_w_down)
```

```python
import math

import jax
import jax.numpy as jnp
import numpy as np
from jax import lax
import jax.experimental.pallas as pl
import jax.experimental.pallas.tpu as pltpu

S = 2048
D = 1024
H = 32
DH = D // H
NSEG = 4
L = S // NSEG
G = 8
F = 3584
OB = 32
OSTEP = 20
ONP = 2
VT_IN_V = 1
LINK = 1
SPLITD = 1
PSTAGE = 0
PLINK = 1
TIE = 1
TORD = 1230
ONB = 2
AG = 2
LAG = 2
FCH = 896

bf16 = jnp.bfloat16
f32 = jnp.float32
i32 = jnp.int32

QSCALE = (DH ** -0.5) * math.log2(math.e)
SAFE_BOUND = 24.0
NEG = -1e30
EPS_BF16 = 1.0013580322265625e-05

_NT = (((1,), (1,)), ((), ()))
_ONLY = None
_FLAGS = None


def _r(x):
    return x.astype(bf16).astype(f32)


def _pack(x):
    return pltpu.bitcast(x.astype(bf16), i32)


def _unpack(w):
    return pltpu.bitcast(w, bf16)


def _layernorm(xf):
    mean = jnp.sum(xf, axis=1, keepdims=True) * (1.0 / D)
    c = xf - mean
    var = jnp.sum(c * c, axis=1, keepdims=True) * (1.0 / D)
    d = _r(xf - _r(mean))
    s = _r(jnp.sqrt(_r(_r(var) + EPS_BF16)))
    return _r(d * (1.0 / s))


def _phi(t):
    return jnp.where(t > 0, t + 1.0, jnp.exp(t))


def _head_lanes(qi, h):
    lane = lax.broadcasted_iota(i32, qi.shape, 1)
    return _unpack(jnp.where((lane >> 5) == h, qi, 0))


def _fold8(x):
    return x.reshape(x.shape[0] // 8, 8, x.shape[1])


def _half(i, n):
    return pl.ds(i // 2 if isinstance(i, int) else pl.multiple_of(i // 2, n // 2), n // 2)


def _kernel(zero_s, beta_ref, wr_ref,
            x_hbm, wq_hbm, wk_hbm, wv_hbm, wo_hbm, wg_hbm, wu_hbm, wd_hbm,
            out_hbm,
            xio, wst, xa, xn, vn, wq, wk, wv, wo, qs, pq, ks, pk, vt, o_s, y_s, x1_s,
            zs, gt, r_s, oc, pb0, pb1, pb2, wg, wu, wd, sems):
    pbufs = [pb0, pb1, pb2]
    nx = NSEG
    x_cp = [pltpu.make_async_copy(x_hbm.at[0, pl.ds(i * L, L), :],
                                  xio.at[pl.ds(i * L, L), :], sems.at[i])
            for i in range(nx)]
    w_cp = [pltpu.make_async_copy(src, dst, sems.at[nx + i]) for i, (src, dst) in
            enumerate([(wv_hbm, wst.at[0]), (wq_hbm, wst.at[1]), (wk_hbm, wst.at[2]),
                       (wo_hbm, wst.at[3]), (wg_hbm, wg), (wu_hbm, wu), (wd_hbm, wd)])]
    x_cp[0].start()
    w_cp[0].start()
    for c in x_cp[1:]:
        c.start()
    for c in w_cp[1:]:
        c.start()

    b = jnp.broadcast_to(beta_ref[...].astype(f32).reshape(1, H), (H, H))
    rr = lax.broadcasted_iota(i32, (H, H), 0)
    cc = lax.broadcasted_iota(i32, (H, H), 1)
    bcol = jnp.sum(jnp.where(rr == cc, b, 0.0), axis=1, keepdims=True)
    gt[...] = _r(jax.nn.sigmoid(jnp.broadcast_to(bcol, (H, 128))))

    lane = lax.broadcasted_iota(i32, (128, 128), 1)
    row = lax.broadcasted_iota(i32, (128, 128), 0)

    def widen_x(r0):
        xa[pl.ds(r0, L), :] = xio[pl.ds(r0, L), :].astype(f32)

    def ln_rows(r0, n):
        xn[_half(r0, n), :] = _pack(_layernorm(xa[pl.ds(r0, n), :]))

    def ln_block(r0):
        ln_rows(r0, L)

    def repack(i, dst):
        dst[...] = _pack(wst[i])

    CB = 256

    def next_block(s):
        return pl.multiple_of(jnp.minimum(s + 1, NSEG - 1) * L, L)

    def vproj_block(s):
        for i in range(1, nx):
            @pl.when(s == i - 1)
            def _():
                x_cp[i].wait()
                widen_x(i * L)

        r0 = pl.multiple_of(s * L, L)
        xb = _unpack(xn[_half(r0, L), :])
        for c0 in range(0, D, CB):
            v = jnp.dot(xb, _unpack(wv[:, c0:c0 + CB]), preferred_element_type=f32)
            if VT_IN_V:
                vt[s, c0 // 2:(c0 + CB) // 2, :] = pltpu.bitcast(v.astype(bf16).T, i32)
            else:
                vn[_half(r0, L), c0:c0 + CB] = _pack(v)
        ln_block(next_block(s))

    def qkproj_block(s, carry, with_v):
        qmax, kmax = carry
        r0 = pl.multiple_of(s * L, L)
        xb = _unpack(xn[_half(r0, L), :])
        for c0 in range(0, D, CB):
            if with_v:
                v = jnp.dot(xb, _unpack(wv[:, c0:c0 + CB]),
                            preferred_element_type=f32).astype(bf16)
            elif VT_IN_V:
                break
            else:
                v = _unpack(vn[_half(r0, L), c0:c0 + CB])
            vt[s, c0 // 2:(c0 + CB) // 2, :] = pltpu.bitcast(v.T, i32)
        for c0 in range(0, D, CB):
            q = jnp.dot(xb, _unpack(wq[:, c0:c0 + CB]), preferred_element_type=f32)
            k = jnp.dot(xb, _unpack(wk[:, c0:c0 + CB]), preferred_element_type=f32)
            for j in range(CB // 128):
                g = c0 // 128 + j
                qg = q[:, j * 128:(j + 1) * 128]
                kg = k[:, j * 128:(j + 1) * 128]
                qsc = qg * QSCALE
                qs[g, _half(r0, L), :] = _pack(qsc)
                pq[g, _half(r0, L), :] = _pack(_phi(qg))
                ks[g, _half(r0, L), :] = _pack(kg)
                pkg = _phi(kg)
                pk[g, _half(r0, L), :] = _pack(pkg)
                zs[s, g] = jnp.sum(_fold8(pkg), axis=0)
                qmax = jnp.maximum(qmax, jnp.max(_fold8(jnp.abs(qsc)), axis=0))
                kmax = jnp.maximum(kmax, jnp.max(_fold8(jnp.abs(kg)), axis=0))
        if with_v:
            ln_block(next_block(s))
        return qmax, kmax

    def attn_groups(g0, ng, use_max):
        causal = row <= lane
        gs = [g0 + i for i in range(ng)]
        g64 = [pl.multiple_of(g * 64, 64) for g in gs]
        gate = [[gt[pl.ds(g * 4 + h, 1), :] for h in range(4)] for g in gs]
        blockdiag = (row >> 5) == (lane >> 5)
        lane16 = lax.broadcasted_iota(i32, (16, 128), 1)
        row16 = lax.broadcasted_iota(i32, (16, 128), 0)
        zmask = (lane16 >> 5) == row16

        def tile(ref, g, s, t):
            return ref[g, (s * L + t * 128) // 2:(s * L + (t + 1) * 128) // 2, :]

        split_diag = SPLITD and not use_max
        lane64 = lax.broadcasted_iota(i32, (64, 128), 1)
        causal64 = lax.broadcasted_iota(i32, (64, 128), 0) <= (lane64 & 63)
        low64 = lane64 < 64
        low8 = lax.broadcasted_iota(i32, (8, 128), 1) < 64

        def qk(gi, s, t, flip, link_slot=None):
            g = gs[gi]
            qt = tile(qs, g, s, t)
            if link_slot is not None:
                zero = zero_s[0]
                lk = pltpu.bitcast(pbufs[link_slot][zero, 0:16, :], i32)
                qt = jnp.concatenate([qt[0:8] | (lk & zero), qt[8:]], axis=0)
            qlane = lax.broadcasted_iota(i32, qt.shape, 1)
            qi = [jnp.where((qlane >> 5) == h, qt, 0) for h in range(4)]
            qm = [_unpack(x) for x in qi]
            Sc = [[None] * (t + 1) for _ in range(4)]
            for j in range(t if split_diag else t + 1):
                kk = _unpack(tile(ks, g, s, j))
                for h in range(4):
                    Sc[h][j] = lax.dot_general(kk, qm[h], _NT, preferred_element_type=f32)
            if not split_diag:
                return Sc, None
            kd = tile(ks, g, s, t)
            T1, T2 = [None, None], [None, None]

            def t1(pr):
                w = _unpack(jnp.concatenate([qi[2 * pr][0:32], qi[2 * pr + 1][0:32]], axis=0))
                T1[pr] = lax.dot_general(_unpack(kd[0:32]), w, _NT, preferred_element_type=f32)

            def t2(pr):
                w = _unpack(jnp.concatenate([qi[2 * pr][32:64], qi[2 * pr + 1][32:64]], axis=0))
                T2[pr] = lax.dot_general(_unpack(kd), w, _NT, preferred_element_type=f32)

            for fn, pr in ((t2, 0), (t2, 1), (t1, 0), (t1, 1)) if flip else (
                    (t1, 0), (t1, 1), (t2, 0), (t2, 1)):
                fn(pr)
            return Sc, (T1, T2)

        def tie(x, part):
            if not TIE:
                return x
            n = x.shape[0] - 8
            return jnp.concatenate([x[:n], x[n:] + part * 0.0], axis=0)

        def sm(ScD, t, slot):
            Sc, Dg = ScD
            P = [None] * 4
            Linv = [None] * 4
            l8 = [None] * 4
            for h in range(4):
                sc = list(Sc[h])
                if not split_diag:
                    sc[t] = jnp.where(causal, sc[t], NEG)
                else:
                    sc = sc[:t]
                if use_max:
                    m = sc[0]
                    for j in range(1, t + 1):
                        m = jnp.maximum(m, sc[j])
                    m = jnp.max(m, axis=0, keepdims=True)
                    p = [jnp.exp2(x - m) for x in sc]
                else:
                    p = [jnp.exp2(x) for x in sc]
                P[h] = []
                for x in p:
                    part = jnp.sum(_fold8(x), axis=0)
                    l8[h] = part if l8[h] is None else l8[h] + part
                    P[h].append(tie(x, part).astype(bf16))
            if split_diag:
                for pr in range(2):
                    a, b = 2 * pr, 2 * pr + 1
                    e1 = jnp.exp2(jnp.where(causal64, Dg[0][pr], NEG))
                    e2a = jnp.exp2(Dg[1][pr][0:64])
                    e2b = jnp.exp2(jnp.where(causal64, Dg[1][pr][64:128], NEG))
                    p1 = jnp.sum(_fold8(e1), axis=0)
                    p2 = jnp.sum(_fold8(e2a), axis=0) + jnp.sum(_fold8(e2b), axis=0)
                    la = jnp.where(low8, p1, pltpu.roll(p2, 64, 1))
                    lb = jnp.where(low8, pltpu.roll(p1, 64, 1), p2)
                    l8[a] = la if l8[a] is None else l8[a] + la
                    l8[b] = lb if l8[b] is None else l8[b] + lb
                    e1, e2b = tie(e1, p1), tie(e2b, p2)
                    P[a].append(jnp.concatenate(
                        [jnp.where(low64, e1, pltpu.roll(e2a, 64, 1)),
                         jnp.where(low64, 0.0, pltpu.roll(e2b, 64, 1))], axis=0).astype(bf16))
                    P[b].append(jnp.concatenate(
                        [jnp.where(low64, pltpu.roll(e1, 64, 1), e2a),
                         jnp.where(low64, 0.0, e2b)], axis=0).astype(bf16))
            for h in range(4):
                Linv[h] = 1.0 / jnp.sum(l8[h], axis=0, keepdims=True)
            if PSTAGE:
                for h in range(4):
                    for j in range(t + 1):
                        pbufs[slot][h, j * 128:(j + 1) * 128, :] = P[h][j]
                P = slot
            return P, Linv

        def pv(PL, gi, s, t, lhs_m):
            g = gs[gi]
            P, Linv = PL
            acc = [None] * 4
            for j in range(t + 1):
                for h in range(4):
                    vth = _unpack(vt[s, pl.ds(g64[gi] + 16 * h, 16), j * 128:(j + 1) * 128])
                    if PSTAGE:
                        pt = pbufs[P][h + zero_s[0], j * 128:(j + 1) * 128, :]
                    else:
                        pt = P[h][j]
                    o = jnp.dot(vth, pt, preferred_element_type=f32)
                    acc[h] = o if acc[h] is None else acc[h] + o
            if lhs_m is not None:
                pqt = _unpack(tile(pq, g, s, t))
                nd = lax.dot_general(lhs_m, pqt, _NT, preferred_element_type=f32)
            outs = []
            for h in range(4):
                o = acc[h] * ((1.0 - gate[gi][h]) * Linv[h])
                if lhs_m is not None:
                    den = nd[128 + h:129 + h, :] + 1e-6
                    o = o + nd[32 * h:32 * h + 32, :] * (gate[gi][h] / den)
                outs.append(o)
            ot = jnp.concatenate(outs, axis=0).astype(bf16)
            o_s[g, (s * L + t * 128) // 2:(s * L + (t + 1) * 128) // 2, :] = (
                pltpu.bitcast(ot.T, i32))

        def mem_update(gi, s, R):
            g = gs[gi]
            vtg = _unpack(vt[s, pl.ds(g64[gi], 64), :])
            pks = _unpack(pk[g, s * L // 2:(s + 1) * L // 2, :])
            upd = jnp.dot(vtg, pks, preferred_element_type=f32)
            return upd if R is None else R + upd

        def mem_lhs(gi, s, R):
            g = gs[gi]
            mt = jnp.where(blockdiag, R, 0.0)
            z = zs[0, g]
            for s2 in range(1, s):
                z = z + zs[s2, g]
            z = jnp.sum(z, axis=0, keepdims=True)
            zr = jnp.where(zmask, z, 0.0)
            return jnp.concatenate([mt, zr], axis=0).astype(bf16)

        order = [int(c) for c in str(TORD).zfill(4)]
        steps = [(gi, s, t) for gi in range(ng) for s in range(NSEG) for t in order]
        n = len(steps)
        Sc, PL = {}, {}
        R = None
        lhs = {}
        for i in range(n + LAG):
            if i < n:
                Sc[i] = qk(*steps[i], i % 2 == 1,
                           (i - 2) % 3 if (PSTAGE and PLINK and i >= 2) else None)
                gi, s, t = steps[i]
                if t == order[0] and s == 0:
                    R = None
                    lhs[gi, 0] = None
                if t == order[-1] and s < NSEG - 1:
                    R = mem_update(gi, s, R)
                    lhs[gi, s + 1] = mem_lhs(gi, s + 1, R)
                if not PSTAGE:
                    PL[i] = sm(Sc.pop(i), t, i % 3)
            if 0 <= i - LAG < n:
                gi, s, t = steps[i - LAG]
                pv(PL.pop(i - LAG), gi, s, t, lhs[gi, s])
            if PSTAGE and i < n:
                PL[i] = sm(Sc.pop(i), steps[i][2], i % 3)

    wr = wr_ref[...].astype(f32).reshape(1, D)
    CP, RP = D // ONP, OB // ONP
    lane_ob = lax.broadcasted_iota(i32, (OB, 128), 1)
    row_ob = lax.broadcasted_iota(i32, (OB, 128), 0)

    def o_lhs(r0):
        return jnp.concatenate([_unpack(o_s[g, _half(r0, OB), :]) for g in range(G)], axis=1)

    def o_epilogue(refs, r0, out, last):
        xa_, x1_, y_, xo_ = refs
        x1 = _r(xa_[r0:r0 + RP, :] + _r(out))
        x1_[r0:r0 + RP, :] = x1.astype(bf16)
        y = _layernorm(x1)
        y_[r0:r0 + RP, :] = y.astype(bf16)
        if last:
            xo_[r0:r0 + RP, :] = (x1 + y).astype(bf16)
        else:
            xa_[r0:r0 + RP, :] = _r(x1 + y)
        return _r(jnp.sum(y * wr, axis=1, keepdims=True))

    def o_refs(r0, n):
        return [xa.at[pl.ds(r0, n)], x1_s.at[pl.ds(r0, n)], y_s.at[pl.ds(r0, n)],
                xio.at[pl.ds(r0, n)]]

    def o_step(refs, k, blk, src, dst, last):
        if dst is not None:
            ob = o_lhs((blk + 1) * OB)
        rcols = []
        for p in range(ONP):
            if dst is not None:
                dst[:, p * CP:(p + 1) * CP] = jnp.dot(
                    ob, _unpack(wo[:, p * CP:(p + 1) * CP]), preferred_element_type=f32)
            rcols.append(o_epilogue(refs, k * OB + p * RP, src[p * RP:(p + 1) * RP, :], last))
        rb = jnp.broadcast_to(jnp.concatenate(rcols, axis=0), (OB, 128))
        r_s[pl.ds(blk, 1), :] = jnp.max(jnp.where(row_ob == lane_ob, rb, -jnp.inf),
                                        axis=0, keepdims=True)

    def o_phase(last):
        nb = S // OB
        oc[0] = jnp.dot(o_lhs(0), _unpack(wo[...]), preferred_element_type=f32)
        nloop = (nb - 2) // OSTEP
        assert OSTEP % ONB == 0

        def body(i, carry):
            refs = o_refs(pl.multiple_of(i * OSTEP * OB, OSTEP * OB), OSTEP * OB)
            for k in range(OSTEP):
                o_step(refs, k, i * OSTEP + k, oc.at[k % ONB], oc.at[(k + 1) % ONB], last)
            return carry

        lax.fori_loop(0, nloop, body, 0)
        b0 = nloop * OSTEP
        refs = o_refs(b0 * OB, (nb - b0) * OB)
        for k in range(nb - b0):
            o_step(refs, k, b0 + k, oc.at[k % ONB],
                   oc.at[(k + 1) % ONB] if b0 + k + 1 < nb else None, last)

    out_cp = pltpu.make_async_copy(xio, out_hbm.at[0], sems.at[2])

    def moe_phase(last):
        r_all = r_s[...]
        ridx = (lax.broadcasted_iota(i32, r_all.shape, 0) * OB
                + lax.broadcasted_iota(i32, r_all.shape, 1)).astype(f32)
        m1 = jnp.max(r_all)
        i1f = jnp.min(jnp.where(r_all == m1, ridx, 1e9))
        r2 = jnp.where(ridx == i1f, -jnp.inf, r_all)
        m2 = jnp.max(r2)
        i2f = jnp.min(jnp.where((r2 == m2) & (ridx != i1f), ridx, 1e9))
        idx = [jnp.clip(i1f.astype(i32), 0, S - 1), jnp.clip(i2f.astype(i32), 0, S - 1)]
        base = [pl.multiple_of((ix >> 4) << 4, 16) for ix in idx]
        off = [ix & 15 for ix in idx]
        row16 = lax.broadcasted_iota(i32, (16, D), 0)

        def gather(ref):
            res = None
            for kk in range(2):
                blk = ref[pl.ds(base[kk], 16), :].astype(f32)
                one = jnp.sum(jnp.where(row16 == off[kk], blk, 0.0), axis=0, keepdims=True)
                part = jnp.where(row16 == kk, one, 0.0)
                res = part if res is None else res + part
            return res

        ysel = gather(y_s)
        x1sel = gather(x1_s)
        xsel32 = _pack(ysel)
        zero = zero_s[0]
        yf = None
        nch = F // FCH
        rp = L // nch
        for ci, c0 in enumerate(range(0, F, FCH)):
            if not last and LINK:
                ln_rows(ci * rp, rp)
                link = xn[pl.ds(pl.multiple_of(zero, 8), 8), :]
                xsel = _unpack(xsel32 | (link & zero))
            else:
                xsel = _unpack(xsel32)
            gte = _r(jnp.dot(xsel, wg[:, c0:c0 + FCH], preferred_element_type=f32))
            up = _r(jnp.dot(xsel, wu[:, c0:c0 + FCH], preferred_element_type=f32))
            act = _r(gte * jax.nn.sigmoid(gte))
            hcol = (act * up).astype(bf16)
            part = jnp.dot(hcol, wd[c0:c0 + FCH, :], preferred_element_type=f32)
            yf = part if yf is None else yf + part
        if not last and not LINK:
            ln_block(0)
        rsel = _r(jax.nn.sigmoid(jnp.where(row16 == 0, m1, m2)))
        upd = _r(_r(yf) * rsel)
        x2 = _r(x1sel + _r(ysel + upd))
        rows2 = [jnp.sum(jnp.where(row16 == kk, x2, 0.0), axis=0, keepdims=True)
                 for kk in range(2)]
        if not last:
            xn2 = _layernorm(x2)
            for kk in range(2):
                xa[pl.ds(idx[kk], 1), :] = rows2[kk]
                one = jnp.sum(jnp.where(row16 == kk, xn2, 0.0), axis=0, keepdims=True)
                blk = _unpack(xn[_half(base[kk], 16), :]).astype(f32)
                xn[_half(base[kk], 16), :] = _pack(jnp.where(row16 == off[kk], one, blk))
        else:
            out_cp.wait()
            for kk in range(2):
                blk = xio[pl.ds(base[kk], 16), :].astype(f32)
                xio[pl.ds(base[kk], 16), :] = jnp.where(
                    row16 == off[kk], rows2[kk], blk).astype(bf16)
            cp0 = pltpu.make_async_copy(xio.at[pl.ds(base[0], 16), :],
                                        out_hbm.at[0, pl.ds(base[0], 16), :], sems.at[0])
            cp1 = pltpu.make_async_copy(xio.at[pl.ds(base[1], 16), :],
                                        out_hbm.at[0, pl.ds(base[1], 16), :], sems.at[1])
            cp0.start()

            @pl.when(base[0] != base[1])
            def _():
                cp1.start()
                cp1.wait()

            cp0.wait()

    if _ONLY:
        for c in x_cp + w_cp:
            c.wait()
        dict(O0=lambda: o_phase(False), O1=lambda: o_phase(True),
             B0=lambda: moe_phase(False),
             A=lambda: lax.fori_loop(0, G // AG, lambda i, c: (attn_groups(i * AG, AG, False), c)[1], 0))[_ONLY]()
        out_cp.start()
        out_cp.wait()
        return

    x_cp[0].wait()
    widen_x(0)
    ln_block(0)
    w_cp[0].wait()
    repack(0, wv)

    for li in range(2):
        last = li == 1
        z8 = jnp.zeros((8, 128), f32)
        if li == 0:
            lax.fori_loop(0, NSEG, lambda s, c: (vproj_block(s), c)[1], 0)
            for i, dst in ((1, wq), (2, wk)):
                w_cp[i].wait()
                repack(i, dst)
            qmax, kmax = lax.fori_loop(
                0, NSEG, lambda s, c: qkproj_block(s, c, False), (z8, z8))
        else:
            qmax, kmax = lax.fori_loop(
                0, NSEG, lambda s, c: qkproj_block(s, c, True), (z8, z8))
        bound = DH * jnp.max(qmax) * jnp.max(kmax)
        safe = bound <= SAFE_BOUND

        @pl.when(safe)
        def _():
            lax.fori_loop(0, G // AG, lambda i, c: (attn_groups(i * AG, AG, False), c)[1], 0)

        @pl.when(jnp.logical_not(safe))
        def _():
            lax.fori_loop(0, G, lambda g, c: (attn_groups(g, 1, True), c)[1], 0)

        if li == 0:
            w_cp[3].wait()
            repack(3, wo)
        o_phase(last)
        if li == 0:
            for c in w_cp[4:]:
                c.wait()
        else:
            out_cp.start()
        moe_phase(last)


@jax.jit
def pallas_interleave_layers__memory_aug_infini_attn__moe_arch_mod__prompt_kernel(
    A_x: jax.Array,
    A_wq: jax.Array,
    A_wk: jax.Array,
    A_wv: jax.Array,
    A_wo: jax.Array,
    A_beta: jax.Array,
    B_x: jax.Array,
    B_w_r: jax.Array,
    B_w_gate: jax.Array,
    B_w_up: jax.Array,
    B_w_down: jax.Array,
):
    del B_x
    any_spec = pl.BlockSpec(memory_space=pl.ANY)
    vm = pltpu.VMEM
    return pl.pallas_call(
        _kernel,
        out_shape=jax.ShapeDtypeStruct((1, S, D), bf16),
        in_specs=[pl.BlockSpec(memory_space=pltpu.SMEM),
                  pl.BlockSpec(memory_space=vm), pl.BlockSpec(memory_space=vm)] + [any_spec] * 8,
        out_specs=any_spec,
        scratch_shapes=[
            vm((S, D), bf16),
            vm((4, D, D), bf16),
            vm((S, D), f32),
            vm((S // 2, D), i32),
            vm((S // 2, D), i32),
            vm((D // 2, D), i32), vm((D // 2, D), i32),
            vm((D // 2, D), i32), vm((D // 2, D), i32),
            vm((G, S // 2, 128), i32), vm((G, S // 2, 128), i32),
            vm((G, S // 2, 128), i32), vm((G, S // 2, 128), i32),
            vm((NSEG, D // 2, L), i32),
            vm((G, S // 2, 128), i32),
            vm((S, D), bf16), vm((S, D), bf16),
            vm((NSEG, G, 8, 128), f32),
            vm((H, 128), f32),
            vm((S // OB, 128), f32),
            vm((ONB, OB, D), f32),
            vm((4, L, 128), bf16), vm((4, L, 128), bf16), vm((4, L, 128), bf16),
            vm((D, F), bf16), vm((D, F), bf16), vm((F, D), bf16),
            pltpu.SemaphoreType.DMA((NSEG + 7,)),
        ],
        compiler_params=pltpu.CompilerParams(vmem_limit_bytes=120 * 1024 * 1024, flags=_FLAGS),
    )(np.zeros((1,), np.int32), A_beta, B_w_r, A_x, A_wq, A_wk, A_wv, A_wo, B_w_gate, B_w_up, B_w_down)
```

```python
import math

import jax
import jax.numpy as jnp
import numpy as np
from jax import lax
import jax.experimental.pallas as pl
import jax.experimental.pallas.tpu as pltpu

S = 2048
D = 1024
H = 32
DH = D // H
NSEG = 4
L = S // NSEG
G = 8
F = 3584
OB = 32
OSTEP = 30
ONP = 2
VT_IN_V = 1
LINK = 1
SPLITD = 1
ODELAY = 3
TIE = 1
TORD = 1230
ONB = 5
AG = 2
LAG = 2
FCH = 896

bf16 = jnp.bfloat16
f32 = jnp.float32
i32 = jnp.int32

QSCALE = (DH ** -0.5) * math.log2(math.e)
SAFE_BOUND = 24.0
NEG = -1e30
EPS_BF16 = 1.0013580322265625e-05

_NT = (((1,), (1,)), ((), ()))
_ONLY = None
_FLAGS = None


def _r(x):
    return x.astype(bf16).astype(f32)


def _pack(x):
    return pltpu.bitcast(x.astype(bf16), i32)


def _unpack(w):
    return pltpu.bitcast(w, bf16)


def _layernorm(xf):
    mean = jnp.sum(xf, axis=1, keepdims=True) * (1.0 / D)
    c = xf - mean
    var = jnp.sum(c * c, axis=1, keepdims=True) * (1.0 / D)
    d = _r(xf - _r(mean))
    s = _r(jnp.sqrt(_r(_r(var) + EPS_BF16)))
    return _r(d * (1.0 / s))


def _phi(t):
    return jnp.where(t > 0, t + 1.0, jnp.exp(t))


def _head_lanes(qi, h):
    lane = lax.broadcasted_iota(i32, qi.shape, 1)
    return _unpack(jnp.where((lane >> 5) == h, qi, 0))


def _fold8(x):
    return x.reshape(x.shape[0] // 8, 8, x.shape[1])


def _half(i, n):
    return pl.ds(i // 2 if isinstance(i, int) else pl.multiple_of(i // 2, n // 2), n // 2)


def _kernel(zero_s, beta_ref, wr_ref,
            x_hbm, wq_hbm, wk_hbm, wv_hbm, wo_hbm, wg_hbm, wu_hbm, wd_hbm,
            out_hbm,
            xio, wst, xa, xn, vn, wo, qs, pq, ks, pk, vt, o_s, y_s, x1_s,
            zs, gt, r_s, oc, wg, wu, wd, sems):
    nx = NSEG
    x_cp = [pltpu.make_async_copy(x_hbm.at[0, pl.ds(i * L, L), :],
                                  xio.at[pl.ds(i * L, L), :], sems.at[i])
            for i in range(nx)]
    w_cp = [pltpu.make_async_copy(src, dst, sems.at[nx + i]) for i, (src, dst) in
            enumerate([(wv_hbm, wst.at[0]), (wq_hbm, wst.at[1]), (wk_hbm, wst.at[2]),
                       (wo_hbm, wst.at[3]), (wg_hbm, wg), (wu_hbm, wu), (wd_hbm, wd)])]
    x_cp[0].start()
    w_cp[0].start()
    for c in x_cp[1:]:
        c.start()
    for c in w_cp[1:]:
        c.start()

    b = jnp.broadcast_to(beta_ref[...].astype(f32).reshape(1, H), (H, H))
    rr = lax.broadcasted_iota(i32, (H, H), 0)
    cc = lax.broadcasted_iota(i32, (H, H), 1)
    bcol = jnp.sum(jnp.where(rr == cc, b, 0.0), axis=1, keepdims=True)
    gt[...] = _r(jax.nn.sigmoid(jnp.broadcast_to(bcol, (H, 128))))

    lane = lax.broadcasted_iota(i32, (128, 128), 1)
    row = lax.broadcasted_iota(i32, (128, 128), 0)

    def ln_rows(r0, n, src=None):
        src = xa if src is None else src
        xn[_half(r0, n), :] = _pack(_layernorm(src[pl.ds(r0, n), :].astype(f32)))

    def ln_block(r0, src=None):
        ln_rows(r0, L, src)

    def pin(w32, ref):
        zero = zero_s[0]
        lk = ref[pl.ds(pl.multiple_of(zero, 8), 8), 0:128] & zero
        head = jnp.concatenate([w32[0:8, 0:128] | lk, w32[0:8, 128:]], axis=1)
        return head if w32.shape[0] == 8 else jnp.concatenate([head, w32[8:]], axis=0)

    CB = 256

    def next_block(s):
        return pl.multiple_of(jnp.minimum(s + 1, NSEG - 1) * L, L)

    def vproj_block(s):
        for i in range(1, nx):
            @pl.when(s == i - 1)
            def _():
                x_cp[i].wait()

        r0 = pl.multiple_of(s * L, L)
        xb32 = xn[_half(r0, L), :]
        if not VT_IN_V:
            ln_block(next_block(s), xio)
        for c0 in range(0, D, CB):
            xb = xb32
            if not VT_IN_V and c0 == D - CB:
                xb = pin(xb32, xn)
            v = jnp.dot(_unpack(xb), wst[0, :, c0:c0 + CB], preferred_element_type=f32)
            if VT_IN_V:
                vt[s, c0 // 2:(c0 + CB) // 2, :] = pltpu.bitcast(v.astype(bf16).T, i32)
            else:
                vn[pl.ds(r0, L), c0:c0 + CB] = v.astype(bf16)
        if VT_IN_V:
            ln_block(next_block(s), xio)

    def qkproj_block(s, carry, with_v):
        qmax, kmax = carry
        r0 = pl.multiple_of(s * L, L)
        xb = _unpack(xn[_half(r0, L), :])
        for c0 in range(0, D, CB):
            if with_v:
                v = jnp.dot(xb, wst[0, :, c0:c0 + CB],
                            preferred_element_type=f32).astype(bf16)
            elif VT_IN_V:
                break
            else:
                v = vn[pl.ds(r0, L), c0:c0 + CB]
            vt[s, c0 // 2:(c0 + CB) // 2, :] = pltpu.bitcast(v.T, i32)
        for c0 in range(0, D, CB):
            q = jnp.dot(xb, wst[1, :, c0:c0 + CB], preferred_element_type=f32)
            k = jnp.dot(xb, wst[2, :, c0:c0 + CB], preferred_element_type=f32)
            for j in range(CB // 128):
                g = c0 // 128 + j
                qg = q[:, j * 128:(j + 1) * 128]
                kg = k[:, j * 128:(j + 1) * 128]
                qsc = qg * QSCALE
                qs[g, _half(r0, L), :] = _pack(qsc)
                pq[g, _half(r0, L), :] = _pack(_phi(qg))
                ks[g, _half(r0, L), :] = _pack(kg)
                pkg = _phi(kg)
                pk[g, _half(r0, L), :] = _pack(pkg)
                zs[s, g] = jnp.sum(_fold8(pkg), axis=0)
                qmax = jnp.maximum(qmax, jnp.max(_fold8(jnp.abs(qsc)), axis=0))
                kmax = jnp.maximum(kmax, jnp.max(_fold8(jnp.abs(kg)), axis=0))
        if with_v:
            ln_block(next_block(s))
        else:
            wo[pl.ds(pl.multiple_of(s * (D // 8), D // 8), D // 8), :] = _pack(
                wst[3, pl.ds(pl.multiple_of(s * (D // 4), D // 4), D // 4), :])
        return qmax, kmax

    def attn_groups(g0, ng, use_max):
        causal = row <= lane
        gs = [g0 + i for i in range(ng)]
        g64 = [pl.multiple_of(g * 64, 64) for g in gs]
        gate = [[gt[pl.ds(g * 4 + h, 1), :] for h in range(4)] for g in gs]
        blockdiag = (row >> 5) == (lane >> 5)
        lane16 = lax.broadcasted_iota(i32, (16, 128), 1)
        row16 = lax.broadcasted_iota(i32, (16, 128), 0)
        zmask = (lane16 >> 5) == row16

        def tile(ref, g, s, t):
            return ref[g, (s * L + t * 128) // 2:(s * L + (t + 1) * 128) // 2, :]

        split_diag = SPLITD and not use_max
        lane64 = lax.broadcasted_iota(i32, (64, 128), 1)
        causal64 = lax.broadcasted_iota(i32, (64, 128), 0) <= (lane64 & 63)
        low64 = lane64 < 64
        low8 = lax.broadcasted_iota(i32, (8, 128), 1) < 64

        def qk(gi, s, t, flip, link=None):
            g = gs[gi]
            qt = tile(qs, g, s, t)
            if link is not None:
                qt = jnp.concatenate([qt[0:8] | link, qt[8:]], axis=0)
            qlane = lax.broadcasted_iota(i32, qt.shape, 1)
            qi = [jnp.where((qlane >> 5) == h, qt, 0) for h in range(4)]
            qm = [_unpack(x) for x in qi]
            Sc = [[None] * (t + 1) for _ in range(4)]
            for j in range(t if split_diag else t + 1):
                kk = _unpack(tile(ks, g, s, j))
                for h in range(4):
                    Sc[h][j] = lax.dot_general(kk, qm[h], _NT, preferred_element_type=f32)
            if not split_diag:
                return Sc, None
            kd = tile(ks, g, s, t)
            T1, T2 = [None, None], [None, None]

            def t1(pr):
                w = _unpack(jnp.concatenate([qi[2 * pr][0:32], qi[2 * pr + 1][0:32]], axis=0))
                T1[pr] = lax.dot_general(_unpack(kd[0:32]), w, _NT, preferred_element_type=f32)

            def t2(pr):
                w = _unpack(jnp.concatenate([qi[2 * pr][32:64], qi[2 * pr + 1][32:64]], axis=0))
                T2[pr] = lax.dot_general(_unpack(kd), w, _NT, preferred_element_type=f32)

            for fn, pr in ((t2, 0), (t2, 1), (t1, 0), (t1, 1)) if flip else (
                    (t1, 0), (t1, 1), (t2, 0), (t2, 1)):
                fn(pr)
            return Sc, (T1, T2)

        def tie(x, part):
            if not TIE:
                return x
            n = x.shape[0] - 8
            return jnp.concatenate([x[:n], x[n:] + part * 0.0], axis=0)

        def sm(ScD, t):
            Sc, Dg = ScD
            P = [None] * 4
            Linv = [None] * 4
            l8 = [None] * 4
            for h in range(4):
                sc = list(Sc[h])
                if not split_diag:
                    sc[t] = jnp.where(causal, sc[t], NEG)
                else:
                    sc = sc[:t]
                if use_max:
                    m = sc[0]
                    for j in range(1, t + 1):
                        m = jnp.maximum(m, sc[j])
                    m = jnp.max(m, axis=0, keepdims=True)
                    p = [jnp.exp2(x - m) for x in sc]
                else:
                    p = [jnp.exp2(x) for x in sc]
                P[h] = []
                for x in p:
                    part = jnp.sum(_fold8(x), axis=0)
                    l8[h] = part if l8[h] is None else l8[h] + part
                    P[h].append(tie(x, part).astype(bf16))
            if split_diag:
                for pr in range(2):
                    a, b = 2 * pr, 2 * pr + 1
                    e1 = jnp.exp2(jnp.where(causal64, Dg[0][pr], NEG))
                    e2a = jnp.exp2(Dg[1][pr][0:64])
                    e2b = jnp.exp2(jnp.where(causal64, Dg[1][pr][64:128], NEG))
                    p1 = jnp.sum(_fold8(e1), axis=0)
                    p2 = jnp.sum(_fold8(e2a), axis=0) + jnp.sum(_fold8(e2b), axis=0)
                    la = jnp.where(low8, p1, pltpu.roll(p2, 64, 1))
                    lb = jnp.where(low8, pltpu.roll(p1, 64, 1), p2)
                    l8[a] = la if l8[a] is None else l8[a] + la
                    l8[b] = lb if l8[b] is None else l8[b] + lb
                    e1, e2b = tie(e1, p1), tie(e2b, p2)
                    P[a].append(jnp.concatenate(
                        [jnp.where(low64, e1, pltpu.roll(e2a, 64, 1)),
                         jnp.where(low64, 0.0, pltpu.roll(e2b, 64, 1))], axis=0).astype(bf16))
                    P[b].append(jnp.concatenate(
                        [jnp.where(low64, pltpu.roll(e1, 64, 1), e2a),
                         jnp.where(low64, 0.0, e2b)], axis=0).astype(bf16))
            for h in range(4):
                Linv[h] = 1.0 / jnp.sum(l8[h], axis=0, keepdims=True)
            return P, Linv

        def pv(PL, gi, s, t, lhs_m):
            g = gs[gi]
            P, Linv = PL
            acc = [None] * 4
            for j in range(t + 1):
                for h in range(4):
                    vth = _unpack(vt[s, pl.ds(g64[gi] + 16 * h, 16), j * 128:(j + 1) * 128])
                    o = jnp.dot(vth, P[h][j], preferred_element_type=f32)
                    acc[h] = o if acc[h] is None else acc[h] + o
            if lhs_m is not None:
                pqt = _unpack(tile(pq, g, s, t))
                nd = lax.dot_general(lhs_m, pqt, _NT, preferred_element_type=f32)
            outs = []
            for h in range(4):
                o = acc[h] * ((1.0 - gate[gi][h]) * Linv[h])
                if lhs_m is not None:
                    den = nd[128 + h:129 + h, :] + 1e-6
                    o = o + nd[32 * h:32 * h + 32, :] * (gate[gi][h] / den)
                outs.append(o)
            ot = jnp.concatenate(outs, axis=0).astype(bf16)
            o_s[g, (s * L + t * 128) // 2:(s * L + (t + 1) * 128) // 2, :] = (
                pltpu.bitcast(ot.T, i32))
            zero = zero_s[0]
            return o_s[g, pl.ds(pl.multiple_of(zero, 8), 8), :] & zero

        def mem_update(gi, s, R):
            g = gs[gi]
            vtg = _unpack(vt[s, pl.ds(g64[gi], 64), :])
            pks = _unpack(pk[g, s * L // 2:(s + 1) * L // 2, :])
            upd = jnp.dot(vtg, pks, preferred_element_type=f32)
            return upd if R is None else R + upd

        def mem_lhs(gi, s, R):
            g = gs[gi]
            mt = jnp.where(blockdiag, R, 0.0)
            z = zs[0, g]
            for s2 in range(1, s):
                z = z + zs[s2, g]
            z = jnp.sum(z, axis=0, keepdims=True)
            zr = jnp.where(zmask, z, 0.0)
            return jnp.concatenate([mt, zr], axis=0).astype(bf16)

        order = [int(c) for c in str(TORD).zfill(4)]
        steps = [(gi, s, t) for gi in range(ng) for s in range(NSEG) for t in order]
        n = len(steps)
        Sc, PL = {}, {}
        R = None
        lhs = {}
        links = {}
        for i in range(n + LAG):
            if i < n:
                Sc[i] = qk(*steps[i], i % 2 == 1,
                           links.get(i - LAG - ODELAY) if ODELAY else None)
                gi, s, t = steps[i]
                if t == order[0] and s == 0:
                    R = None
                    lhs[gi, 0] = None
                if t == order[-1] and s < NSEG - 1:
                    R = mem_update(gi, s, R)
                    lhs[gi, s + 1] = mem_lhs(gi, s + 1, R)
                PL[i] = sm(Sc.pop(i), t)
            if 0 <= i - LAG < n:
                gi, s, t = steps[i - LAG]
                links[i - LAG] = pv(PL.pop(i - LAG), gi, s, t, lhs[gi, s])

    CP, RP = D // ONP, OB // ONP

    def o_lhs(r0):
        return jnp.concatenate([_unpack(o_s[g, _half(r0, OB), :]) for g in range(G)], axis=1)

    def o_epilogue(refs, r0, out, last):
        xa_, x1_, y_, xo_ = refs
        res = xa_[r0:r0 + RP, :] if last else xo_[r0:r0 + RP, :].astype(f32)
        x1 = _r(res + _r(out))
        x1_[r0:r0 + RP, :] = x1.astype(bf16)
        y = _layernorm(x1)
        y_[r0:r0 + RP, :] = y.astype(bf16)
        if last:
            xo_[r0:r0 + RP, :] = (x1 + y).astype(bf16)
        else:
            xa_[r0:r0 + RP, :] = _r(x1 + y)
        wr = wr_ref[...].astype(f32).reshape(1, D)
        return _r(jnp.sum(y * wr, axis=1, keepdims=True))

    def o_refs(r0, n):
        return [xa.at[pl.ds(r0, n)], x1_s.at[pl.ds(r0, n)], y_s.at[pl.ds(r0, n)],
                xio.at[pl.ds(r0, n)]]

    def o_step(refs, k, blk, src, dst, last):
        if dst is not None:
            ob = o_lhs((blk + 1) * OB)
        rcols = []
        for p in range(ONP):
            if dst is not None:
                dst[:, p * CP:(p + 1) * CP] = jnp.dot(
                    ob, _unpack(wo[:, p * CP:(p + 1) * CP]), preferred_element_type=f32)
            rcols.append(o_epilogue(refs, k * OB + p * RP, src[p * RP:(p + 1) * RP, :], last))
        rb = jnp.broadcast_to(jnp.concatenate(rcols, axis=0), (OB, 128))
        lane_ob = lax.broadcasted_iota(i32, (OB, 128), 1)
        row_ob = lax.broadcasted_iota(i32, (OB, 128), 0)
        r_s[pl.ds(blk, 1), :] = jnp.max(jnp.where(row_ob == lane_ob, rb, -jnp.inf),
                                        axis=0, keepdims=True)

    def o_phase(last):
        nb = S // OB
        oc[0] = jnp.dot(o_lhs(0), _unpack(wo[...]), preferred_element_type=f32)
        nloop = (nb - 2) // OSTEP
        assert OSTEP % ONB == 0

        def out_rows(r0, n):
            return pltpu.make_async_copy(xio.at[pl.ds(r0, n)], out_hbm.at[0, pl.ds(r0, n)],
                                         sems.at[2])

        def body(i, carry):
            if last:
                @pl.when(i > 0)
                def _():
                    out_rows(pl.multiple_of((i - 1) * OSTEP * OB, OSTEP * OB),
                             OSTEP * OB).start()

            refs = o_refs(pl.multiple_of(i * OSTEP * OB, OSTEP * OB), OSTEP * OB)
            for k in range(OSTEP):
                o_step(refs, k, i * OSTEP + k, oc.at[k % ONB], oc.at[(k + 1) % ONB], last)
            return carry

        lax.fori_loop(0, nloop, body, 0)
        b0 = nloop * OSTEP
        if last:
            out_rows((b0 - OSTEP) * OB, OSTEP * OB).start()
        refs = o_refs(b0 * OB, (nb - b0) * OB)
        for k in range(nb - b0):
            o_step(refs, k, b0 + k, oc.at[k % ONB],
                   oc.at[(k + 1) % ONB] if b0 + k + 1 < nb else None, last)
        if last:
            out_rows(b0 * OB, (nb - b0) * OB).start()

    out_cp = pltpu.make_async_copy(xio, out_hbm.at[0], sems.at[2])

    def moe_phase(last):
        r_all = r_s[...]
        ridx = (lax.broadcasted_iota(i32, r_all.shape, 0) * OB
                + lax.broadcasted_iota(i32, r_all.shape, 1)).astype(f32)

        def red(fn, x):
            return fn(fn(x, axis=0, keepdims=True), axis=1, keepdims=True)

        m1 = red(jnp.max, r_all)
        i1f = red(jnp.min, jnp.where(r_all == m1, ridx, 1e9))
        r2 = jnp.where(ridx == i1f, -jnp.inf, r_all)
        m2 = red(jnp.max, r2)
        i2f = red(jnp.min, jnp.where((r2 == m2) & (ridx != i1f), ridx, 1e9))
        idx = [jnp.clip(v[0, 0].astype(i32), 0, S - 1) for v in (i1f, i2f)]
        base = [pl.multiple_of((ix >> 4) << 4, 16) for ix in idx]
        off = [ix & 15 for ix in idx]
        row16 = lax.broadcasted_iota(i32, (16, D), 0)

        def gather(ref):
            res = None
            for kk in range(2):
                blk = ref[pl.ds(base[kk], 16), :].astype(f32)
                one = jnp.sum(jnp.where(row16 == off[kk], blk, 0.0), axis=0, keepdims=True)
                part = jnp.where(row16 == kk, one, 0.0)
                res = part if res is None else res + part
            return res

        ysel = gather(y_s)
        x1sel = gather(x1_s)
        xsel32 = _pack(ysel)
        yf = None
        nch = F // FCH
        rp = L // nch
        for ci, c0 in enumerate(range(0, F, FCH)):
            if not last and LINK == 1:
                ln_rows(ci * rp, rp)
                xsel = _unpack(pin(xsel32, xn))
            elif not last and LINK == 2:
                if ci == 0:
                    ln_block(0)
                xsel = _unpack(pin(xsel32, xn) if ci == nch - 1 else xsel32)
            else:
                xsel = _unpack(xsel32)
            gte = _r(jnp.dot(xsel, wg[:, c0:c0 + FCH], preferred_element_type=f32))
            up = _r(jnp.dot(xsel, wu[:, c0:c0 + FCH], preferred_element_type=f32))
            act = _r(gte * jax.nn.sigmoid(gte))
            hcol = (act * up).astype(bf16)
            part = jnp.dot(hcol, wd[c0:c0 + FCH, :], preferred_element_type=f32)
            yf = part if yf is None else yf + part
        if not last and not LINK:
            ln_block(0)
        rsel = _r(jax.nn.sigmoid(jnp.where(row16 == 0, m1, m2)))
        upd = _r(_r(yf) * rsel)
        x2 = _r(x1sel + _r(ysel + upd))
        rows2 = [jnp.sum(jnp.where(row16 == kk, x2, 0.0), axis=0, keepdims=True)
                 for kk in range(2)]
        if not last:
            xn2 = _layernorm(x2)
            for kk in range(2):
                xa[pl.ds(idx[kk], 1), :] = rows2[kk]
                one = jnp.sum(jnp.where(row16 == kk, xn2, 0.0), axis=0, keepdims=True)
                blk = _unpack(xn[_half(base[kk], 16), :]).astype(f32)
                xn[_half(base[kk], 16), :] = _pack(jnp.where(row16 == off[kk], one, blk))
        else:
            out_cp.wait()
            for kk in range(2):
                blk = xio[pl.ds(base[kk], 16), :].astype(f32)
                xio[pl.ds(base[kk], 16), :] = jnp.where(
                    row16 == off[kk], rows2[kk], blk).astype(bf16)
            cp0 = pltpu.make_async_copy(xio.at[pl.ds(base[0], 16), :],
                                        out_hbm.at[0, pl.ds(base[0], 16), :], sems.at[0])
            cp1 = pltpu.make_async_copy(xio.at[pl.ds(base[1], 16), :],
                                        out_hbm.at[0, pl.ds(base[1], 16), :], sems.at[1])
            cp0.start()

            @pl.when(base[0] != base[1])
            def _():
                cp1.start()
                cp1.wait()

            cp0.wait()

    if _ONLY:
        for c in x_cp + w_cp:
            c.wait()
        dict(O0=lambda: o_phase(False), O1=lambda: o_phase(True),
             B0=lambda: moe_phase(False),
             A=lambda: lax.fori_loop(0, G // AG, lambda i, c: (attn_groups(i * AG, AG, False), c)[1], 0))[_ONLY]()
        out_cp.start()
        out_cp.wait()
        return

    x_cp[0].wait()
    ln_block(0, xio)
    w_cp[0].wait()

    for li in range(2):
        last = li == 1
        z8 = jnp.zeros((8, 128), f32)
        if li == 0:
            lax.fori_loop(0, NSEG, lambda s, c: (vproj_block(s), c)[1], 0)
            for c in w_cp[1:4]:
                c.wait()
            qmax, kmax = lax.fori_loop(
                0, NSEG, lambda s, c: qkproj_block(s, c, False), (z8, z8))
        else:
            qmax, kmax = lax.fori_loop(
                0, NSEG, lambda s, c: qkproj_block(s, c, True), (z8, z8))
        bound = DH * jnp.max(qmax) * jnp.max(kmax)
        safe = bound <= SAFE_BOUND

        @pl.when(safe)
        def _():
            lax.fori_loop(0, G // AG, lambda i, c: (attn_groups(i * AG, AG, False), c)[1], 0)

        @pl.when(jnp.logical_not(safe))
        def _():
            lax.fori_loop(0, G, lambda g, c: (attn_groups(g, 1, True), c)[1], 0)

        o_phase(last)
        if li == 0:
            for c in w_cp[4:]:
                c.wait()
        moe_phase(last)


@jax.jit
def pallas_interleave_layers__memory_aug_infini_attn__moe_arch_mod__prompt_kernel(
    A_x: jax.Array,
    A_wq: jax.Array,
    A_wk: jax.Array,
    A_wv: jax.Array,
    A_wo: jax.Array,
    A_beta: jax.Array,
    B_x: jax.Array,
    B_w_r: jax.Array,
    B_w_gate: jax.Array,
    B_w_up: jax.Array,
    B_w_down: jax.Array,
):
    del B_x
    any_spec = pl.BlockSpec(memory_space=pl.ANY)
    vm = pltpu.VMEM
    return pl.pallas_call(
        _kernel,
        out_shape=jax.ShapeDtypeStruct((1, S, D), bf16),
        in_specs=[pl.BlockSpec(memory_space=pltpu.SMEM),
                  pl.BlockSpec(memory_space=vm), pl.BlockSpec(memory_space=vm)] + [any_spec] * 8,
        out_specs=any_spec,
        scratch_shapes=[
            vm((S, D), bf16),
            vm((4, D, D), bf16),
            vm((S, D), f32),
            vm((S // 2, D), i32),
            vm((S, D), bf16),
            vm((D // 2, D), i32),
            vm((G, S // 2, 128), i32), vm((G, S // 2, 128), i32),
            vm((G, S // 2, 128), i32), vm((G, S // 2, 128), i32),
            vm((NSEG, D // 2, L), i32),
            vm((G, S // 2, 128), i32),
            vm((S, D), bf16), vm((S, D), bf16),
            vm((NSEG, G, 8, 128), f32),
            vm((H, 128), f32),
            vm((S // OB, 128), f32),
            vm((ONB, OB, D), f32),
            vm((D, F), bf16), vm((D, F), bf16), vm((F, D), bf16),
            pltpu.SemaphoreType.DMA((NSEG + 7,)),
        ],
        compiler_params=pltpu.CompilerParams(vmem_limit_bytes=120 * 1024 * 1024, flags=_FLAGS),
    )(np.zeros((1,), np.int32), A_beta, B_w_r, A_x, A_wq, A_wk, A_wv, A_wo, B_w_gate, B_w_up, B_w_down)
```

```python
import math

import jax
import jax.numpy as jnp
import numpy as np
from jax import lax
import jax.experimental.pallas as pl
import jax.experimental.pallas.tpu as pltpu

S = 2048
D = 1024
H = 32
DH = D // H
NSEG = 4
L = S // NSEG
G = 8
F = 3584
OB = 32
OSTEP = 30
ONP = 2
LINK = 1
SPLITD = 1
ODELAY = 3
TIE = 1
TORD = 1230
ONB = 5
AG = 2
LAG = 2
FCH = 896

bf16 = jnp.bfloat16
f32 = jnp.float32
i32 = jnp.int32

QSCALE = (DH ** -0.5) * math.log2(math.e)
SAFE_BOUND = 24.0
NEG = -1e30
EPS_BF16 = 1.0013580322265625e-05

_NT = (((1,), (1,)), ((), ()))
_ONLY = None
_FLAGS = None


def _r(x):
    return x.astype(bf16).astype(f32)


def _pack(x):
    return pltpu.bitcast(x.astype(bf16), i32)


def _unpack(w):
    return pltpu.bitcast(w, bf16)


def _layernorm(xf):
    mean = jnp.sum(xf, axis=1, keepdims=True) * (1.0 / D)
    c = xf - mean
    var = jnp.sum(c * c, axis=1, keepdims=True) * (1.0 / D)
    d = _r(xf - _r(mean))
    s = _r(jnp.sqrt(_r(_r(var) + EPS_BF16)))
    return _r(d * (1.0 / s))


def _phi(t):
    return jnp.where(t > 0, t + 1.0, jnp.exp(t))


def _head_lanes(qi, h):
    lane = lax.broadcasted_iota(i32, qi.shape, 1)
    return _unpack(jnp.where((lane >> 5) == h, qi, 0))


def _fold8(x):
    return x.reshape(x.shape[0] // 8, 8, x.shape[1])


def _half(i, n):
    return pl.ds(i // 2 if isinstance(i, int) else pl.multiple_of(i // 2, n // 2), n // 2)


def _kernel(zero_s, beta_ref, wr_ref,
            x_hbm, wq_hbm, wk_hbm, wv_hbm, wo_hbm, wg_hbm, wu_hbm, wd_hbm,
            out_hbm,
            xio, wst, xa, xn, wo, qs, pq, ks, pk, vt, o_s, y_s, x1_s,
            zs, gt, r_s, oc, wg, wu, wd, sems):
    nx = NSEG
    x_cp = [pltpu.make_async_copy(x_hbm.at[0, pl.ds(i * L, L), :],
                                  xio.at[pl.ds(i * L, L), :], sems.at[i])
            for i in range(nx)]
    w_cp = [pltpu.make_async_copy(src, dst, sems.at[nx + i]) for i, (src, dst) in
            enumerate([(wv_hbm.at[:, pl.ds(D // 2, D // 2)], wst.at[0, :, pl.ds(D // 2, D // 2)]),
                       (wq_hbm, wst.at[1]), (wk_hbm, wst.at[2]),
                       (wo_hbm, wst.at[3]), (wg_hbm, wg), (wu_hbm, wu), (wd_hbm, wd),
                       (wv_hbm.at[:, pl.ds(0, D // 2)], wst.at[0, :, pl.ds(0, D // 2)])])]
    x_cp[0].start()
    w_cp[7].start()
    x_cp[1].start()
    w_cp[0].start()
    for c in x_cp[2:]:
        c.start()
    for c in w_cp[1:7]:
        c.start()

    b = jnp.broadcast_to(beta_ref[...].astype(f32).reshape(1, H), (H, H))
    rr = lax.broadcasted_iota(i32, (H, H), 0)
    cc = lax.broadcasted_iota(i32, (H, H), 1)
    bcol = jnp.sum(jnp.where(rr == cc, b, 0.0), axis=1, keepdims=True)
    gt[...] = _r(jax.nn.sigmoid(jnp.broadcast_to(bcol, (H, 128))))

    lane = lax.broadcasted_iota(i32, (128, 128), 1)
    row = lax.broadcasted_iota(i32, (128, 128), 0)

    def ln_rows(r0, n, src=None):
        src = xa if src is None else src
        xn[_half(r0, n), :] = _pack(_layernorm(src[pl.ds(r0, n), :].astype(f32)))

    def ln_block(r0, src=None):
        ln_rows(r0, L, src)

    def pin(w32, ref):
        zero = zero_s[0]
        lk = ref[pl.ds(pl.multiple_of(zero, 8), 8), 0:128] & zero
        head = jnp.concatenate([w32[0:8, 0:128] | lk, w32[0:8, 128:]], axis=1)
        return head if w32.shape[0] == 8 else jnp.concatenate([head, w32[8:]], axis=0)

    CB = 256

    def next_block(s):
        return pl.multiple_of(jnp.minimum(s + 1, NSEG - 1) * L, L)

    def vproj_block(s, first=False):
        r0 = s * L if first else pl.multiple_of(s * L, L)

        def vcols(lo, hi):
            xb = _unpack(xn[_half(r0, L), :])
            for c0 in range(lo, hi, CB):
                v = jnp.dot(xb, wst[0, :, c0:c0 + CB], preferred_element_type=f32)
                vt[s, c0 // 2:(c0 + CB) // 2, :] = pltpu.bitcast(v.astype(bf16).T, i32)

        if first:
            vcols(0, D // 2)
            w_cp[0].wait()
            x_cp[1].wait()
            vcols(D // 2, D)
        else:
            for i in range(2, nx):
                @pl.when(s == i - 1)
                def _():
                    x_cp[i].wait()

            vcols(0, D)
        ln_block(next_block(s), xio)

    def qkproj_block(s, carry, with_v):
        qmax, kmax = carry
        r0 = pl.multiple_of(s * L, L)
        xb = _unpack(xn[_half(r0, L), :])
        for c0 in range(0, D, CB):
            if with_v:
                v = jnp.dot(xb, wst[0, :, c0:c0 + CB], preferred_element_type=f32)
                vt[s, c0 // 2:(c0 + CB) // 2, :] = pltpu.bitcast(v.astype(bf16).T, i32)
        for c0 in range(0, D, CB):
            q = jnp.dot(xb, wst[1, :, c0:c0 + CB], preferred_element_type=f32)
            k = jnp.dot(xb, wst[2, :, c0:c0 + CB], preferred_element_type=f32)
            for j in range(CB // 128):
                g = c0 // 128 + j
                qg = q[:, j * 128:(j + 1) * 128]
                kg = k[:, j * 128:(j + 1) * 128]
                qsc = qg * QSCALE
                qs[g, _half(r0, L), :] = _pack(qsc)
                pq[g, _half(r0, L), :] = _pack(_phi(qg))
                ks[g, _half(r0, L), :] = _pack(kg)
                pkg = _phi(kg)
                pk[g, _half(r0, L), :] = _pack(pkg)
                zs[s, g] = jnp.sum(_fold8(pkg), axis=0)
                qmax = jnp.maximum(qmax, jnp.max(_fold8(jnp.abs(qsc)), axis=0))
                kmax = jnp.maximum(kmax, jnp.max(_fold8(jnp.abs(kg)), axis=0))
        if with_v:
            ln_block(next_block(s))
        else:
            wo[pl.ds(pl.multiple_of(s * (D // 8), D // 8), D // 8), :] = _pack(
                wst[3, pl.ds(pl.multiple_of(s * (D // 4), D // 4), D // 4), :])
        return qmax, kmax

    def attn_groups(g0, ng, use_max):
        causal = row <= lane
        gs = [g0 + i for i in range(ng)]
        g64 = [pl.multiple_of(g * 64, 64) for g in gs]
        gate = [[gt[pl.ds(g * 4 + h, 1), :] for h in range(4)] for g in gs]
        blockdiag = (row >> 5) == (lane >> 5)
        lane16 = lax.broadcasted_iota(i32, (16, 128), 1)
        row16 = lax.broadcasted_iota(i32, (16, 128), 0)
        zmask = (lane16 >> 5) == row16

        def tile(ref, g, s, t):
            return ref[g, (s * L + t * 128) // 2:(s * L + (t + 1) * 128) // 2, :]

        split_diag = SPLITD and not use_max
        lane64 = lax.broadcasted_iota(i32, (64, 128), 1)
        causal64 = lax.broadcasted_iota(i32, (64, 128), 0) <= (lane64 & 63)
        low64 = lane64 < 64
        low8 = lax.broadcasted_iota(i32, (8, 128), 1) < 64

        def qk(gi, s, t, flip, link=None):
            g = gs[gi]
            qt = tile(qs, g, s, t)
            if link is not None:
                qt = jnp.concatenate([qt[0:8] | link, qt[8:]], axis=0)
            qlane = lax.broadcasted_iota(i32, qt.shape, 1)
            qi = [jnp.where((qlane >> 5) == h, qt, 0) for h in range(4)]
            qm = [_unpack(x) for x in qi]
            Sc = [[None] * (t + 1) for _ in range(4)]
            for j in range(t if split_diag else t + 1):
                kk = _unpack(tile(ks, g, s, j))
                for h in range(4):
                    Sc[h][j] = lax.dot_general(kk, qm[h], _NT, preferred_element_type=f32)
            if not split_diag:
                return Sc, None
            kd = tile(ks, g, s, t)
            T1, T2 = [None, None], [None, None]

            def t1(pr):
                w = _unpack(jnp.concatenate([qi[2 * pr][0:32], qi[2 * pr + 1][0:32]], axis=0))
                T1[pr] = lax.dot_general(_unpack(kd[0:32]), w, _NT, preferred_element_type=f32)

            def t2(pr):
                w = _unpack(jnp.concatenate([qi[2 * pr][32:64], qi[2 * pr + 1][32:64]], axis=0))
                T2[pr] = lax.dot_general(_unpack(kd), w, _NT, preferred_element_type=f32)

            for fn, pr in ((t2, 0), (t2, 1), (t1, 0), (t1, 1)) if flip else (
                    (t1, 0), (t1, 1), (t2, 0), (t2, 1)):
                fn(pr)
            return Sc, (T1, T2)

        def tie(x, part):
            if not TIE:
                return x
            n = x.shape[0] - 8
            return jnp.concatenate([x[:n], x[n:] + part * 0.0], axis=0)

        def sm(ScD, t):
            Sc, Dg = ScD
            P = [None] * 4
            Linv = [None] * 4
            l8 = [None] * 4
            for h in range(4):
                sc = list(Sc[h])
                if not split_diag:
                    sc[t] = jnp.where(causal, sc[t], NEG)
                else:
                    sc = sc[:t]
                if use_max:
                    m = sc[0]
                    for j in range(1, t + 1):
                        m = jnp.maximum(m, sc[j])
                    m = jnp.max(m, axis=0, keepdims=True)
                    p = [jnp.exp2(x - m) for x in sc]
                else:
                    p = [jnp.exp2(x) for x in sc]
                P[h] = []
                for x in p:
                    part = jnp.sum(_fold8(x), axis=0)
                    l8[h] = part if l8[h] is None else l8[h] + part
                    P[h].append(tie(x, part).astype(bf16))
            if split_diag:
                for pr in range(2):
                    a, b = 2 * pr, 2 * pr + 1
                    e1 = jnp.exp2(jnp.where(causal64, Dg[0][pr], NEG))
                    e2a = jnp.exp2(Dg[1][pr][0:64])
                    e2b = jnp.exp2(jnp.where(causal64, Dg[1][pr][64:128], NEG))
                    p1 = jnp.sum(_fold8(e1), axis=0)
                    p2 = jnp.sum(_fold8(e2a), axis=0) + jnp.sum(_fold8(e2b), axis=0)
                    la = jnp.where(low8, p1, pltpu.roll(p2, 64, 1))
                    lb = jnp.where(low8, pltpu.roll(p1, 64, 1), p2)
                    l8[a] = la if l8[a] is None else l8[a] + la
                    l8[b] = lb if l8[b] is None else l8[b] + lb
                    e1, e2b = tie(e1, p1), tie(e2b, p2)
                    P[a].append(jnp.concatenate(
                        [jnp.where(low64, e1, pltpu.roll(e2a, 64, 1)),
                         jnp.where(low64, 0.0, pltpu.roll(e2b, 64, 1))], axis=0).astype(bf16))
                    P[b].append(jnp.concatenate(
                        [jnp.where(low64, pltpu.roll(e1, 64, 1), e2a),
                         jnp.where(low64, 0.0, e2b)], axis=0).astype(bf16))
            for h in range(4):
                Linv[h] = 1.0 / jnp.sum(l8[h], axis=0, keepdims=True)
            return P, Linv

        def pv(PL, gi, s, t, lhs_m):
            g = gs[gi]
            P, Linv = PL
            acc = [None] * 4
            for j in range(t + 1):
                for h in range(4):
                    vth = _unpack(vt[s, pl.ds(g64[gi] + 16 * h, 16), j * 128:(j + 1) * 128])
                    o = jnp.dot(vth, P[h][j], preferred_element_type=f32)
                    acc[h] = o if acc[h] is None else acc[h] + o
            if lhs_m is not None:
                pqt = _unpack(tile(pq, g, s, t))
                nd = lax.dot_general(lhs_m, pqt, _NT, preferred_element_type=f32)
            outs = []
            for h in range(4):
                o = acc[h] * ((1.0 - gate[gi][h]) * Linv[h])
                if lhs_m is not None:
                    den = nd[128 + h:129 + h, :] + 1e-6
                    o = o + nd[32 * h:32 * h + 32, :] * (gate[gi][h] / den)
                outs.append(o)
            ot = jnp.concatenate(outs, axis=0).astype(bf16)
            o_s[g, (s * L + t * 128) // 2:(s * L + (t + 1) * 128) // 2, :] = (
                pltpu.bitcast(ot.T, i32))
            zero = zero_s[0]
            return o_s[g, pl.ds(pl.multiple_of(zero, 8), 8), :] & zero

        def mem_update(gi, s, R):
            g = gs[gi]
            vtg = _unpack(vt[s, pl.ds(g64[gi], 64), :])
            pks = _unpack(pk[g, s * L // 2:(s + 1) * L // 2, :])
            upd = jnp.dot(vtg, pks, preferred_element_type=f32)
            return upd if R is None else R + upd

        def mem_lhs(gi, s, R):
            g = gs[gi]
            mt = jnp.where(blockdiag, R, 0.0)
            z = zs[0, g]
            for s2 in range(1, s):
                z = z + zs[s2, g]
            z = jnp.sum(z, axis=0, keepdims=True)
            zr = jnp.where(zmask, z, 0.0)
            return jnp.concatenate([mt, zr], axis=0).astype(bf16)

        order = [int(c) for c in str(TORD).zfill(4)]
        steps = [(gi, s, t) for gi in range(ng) for s in range(NSEG) for t in order]
        n = len(steps)
        Sc, PL = {}, {}
        R = None
        lhs = {}
        links = {}
        for i in range(n + LAG):
            if i < n:
                Sc[i] = qk(*steps[i], i % 2 == 1,
                           links.get(i - LAG - ODELAY) if ODELAY else None)
                gi, s, t = steps[i]
                if t == order[0] and s == 0:
                    R = None
                    lhs[gi, 0] = None
                if t == order[-1] and s < NSEG - 1:
                    R = mem_update(gi, s, R)
                    lhs[gi, s + 1] = mem_lhs(gi, s + 1, R)
                PL[i] = sm(Sc.pop(i), t)
            if 0 <= i - LAG < n:
                gi, s, t = steps[i - LAG]
                links[i - LAG] = pv(PL.pop(i - LAG), gi, s, t, lhs[gi, s])

    CP, RP = D // ONP, OB // ONP

    def o_lhs(r0):
        return jnp.concatenate([_unpack(o_s[g, _half(r0, OB), :]) for g in range(G)], axis=1)

    def o_epilogue(refs, r0, out, last):
        xa_, x1_, y_, xo_ = refs
        res = xa_[r0:r0 + RP, :] if last else xo_[r0:r0 + RP, :].astype(f32)
        x1 = _r(res + _r(out))
        x1_[r0:r0 + RP, :] = x1.astype(bf16)
        y = _layernorm(x1)
        y_[r0:r0 + RP, :] = y.astype(bf16)
        if last:
            xo_[r0:r0 + RP, :] = (x1 + y).astype(bf16)
        else:
            xa_[r0:r0 + RP, :] = _r(x1 + y)
        wr = wr_ref[...].astype(f32).reshape(1, D)
        return _r(jnp.sum(y * wr, axis=1, keepdims=True))

    def o_refs(r0, n):
        return [xa.at[pl.ds(r0, n)], x1_s.at[pl.ds(r0, n)], y_s.at[pl.ds(r0, n)],
                xio.at[pl.ds(r0, n)]]

    def o_step(refs, k, blk, src, dst, last):
        if dst is not None:
            ob = o_lhs((blk + 1) * OB)
        rcols = []
        for p in range(ONP):
            if dst is not None:
                dst[:, p * CP:(p + 1) * CP] = jnp.dot(
                    ob, _unpack(wo[:, p * CP:(p + 1) * CP]), preferred_element_type=f32)
            rcols.append(o_epilogue(refs, k * OB + p * RP, src[p * RP:(p + 1) * RP, :], last))
        rb = jnp.broadcast_to(jnp.concatenate(rcols, axis=0), (OB, 128))
        lane_ob = lax.broadcasted_iota(i32, (OB, 128), 1)
        row_ob = lax.broadcasted_iota(i32, (OB, 128), 0)
        r_s[pl.ds(blk, 1), :] = jnp.max(jnp.where(row_ob == lane_ob, rb, -jnp.inf),
                                        axis=0, keepdims=True)

    def o_phase(last):
        nb = S // OB
        oc[0] = jnp.dot(o_lhs(0), _unpack(wo[...]), preferred_element_type=f32)
        nloop = (nb - 2) // OSTEP
        assert OSTEP % ONB == 0

        def out_rows(r0, n):
            return pltpu.make_async_copy(xio.at[pl.ds(r0, n)], out_hbm.at[0, pl.ds(r0, n)],
                                         sems.at[2])

        def body(i, carry):
            if last:
                @pl.when(i > 0)
                def _():
                    out_rows(pl.multiple_of((i - 1) * OSTEP * OB, OSTEP * OB),
                             OSTEP * OB).start()

            refs = o_refs(pl.multiple_of(i * OSTEP * OB, OSTEP * OB), OSTEP * OB)
            for k in range(OSTEP):
                o_step(refs, k, i * OSTEP + k, oc.at[k % ONB], oc.at[(k + 1) % ONB], last)
            return carry

        lax.fori_loop(0, nloop, body, 0)
        b0 = nloop * OSTEP
        if last:
            out_rows((b0 - OSTEP) * OB, OSTEP * OB).start()
        refs = o_refs(b0 * OB, (nb - b0) * OB)
        for k in range(nb - b0):
            o_step(refs, k, b0 + k, oc.at[k % ONB],
                   oc.at[(k + 1) % ONB] if b0 + k + 1 < nb else None, last)
        if last:
            out_rows(b0 * OB, (nb - b0) * OB).start()

    out_cp = pltpu.make_async_copy(xio, out_hbm.at[0], sems.at[2])

    def moe_phase(last):
        r_all = r_s[...]
        ridx = (lax.broadcasted_iota(i32, r_all.shape, 0) * OB
                + lax.broadcasted_iota(i32, r_all.shape, 1)).astype(f32)

        def red(fn, x):
            return fn(fn(x, axis=0, keepdims=True), axis=1, keepdims=True)

        m1 = red(jnp.max, r_all)
        i1f = red(jnp.min, jnp.where(r_all == m1, ridx, 1e9))
        r2 = jnp.where(ridx == i1f, -jnp.inf, r_all)
        m2 = red(jnp.max, r2)
        i2f = red(jnp.min, jnp.where((r2 == m2) & (ridx != i1f), ridx, 1e9))
        idx = [jnp.clip(v[0, 0].astype(i32), 0, S - 1) for v in (i1f, i2f)]
        base = [pl.multiple_of((ix >> 4) << 4, 16) for ix in idx]
        off = [ix & 15 for ix in idx]
        row16 = lax.broadcasted_iota(i32, (16, D), 0)

        def gather(ref):
            res = None
            for kk in range(2):
                blk = ref[pl.ds(base[kk], 16), :].astype(f32)
                one = jnp.sum(jnp.where(row16 == off[kk], blk, 0.0), axis=0, keepdims=True)
                part = jnp.where(row16 == kk, one, 0.0)
                res = part if res is None else res + part
            return res

        ysel = gather(y_s)
        x1sel = gather(x1_s)
        xsel32 = _pack(ysel)
        yf = None
        nch = F // FCH
        rp = L // nch
        for ci, c0 in enumerate(range(0, F, FCH)):
            if not last and LINK == 1:
                ln_rows(ci * rp, rp)
                xsel = _unpack(pin(xsel32, xn))
            elif not last and LINK == 2:
                if ci == 0:
                    ln_block(0)
                xsel = _unpack(pin(xsel32, xn) if ci == nch - 1 else xsel32)
            else:
                xsel = _unpack(xsel32)
            gte = _r(jnp.dot(xsel, wg[:, c0:c0 + FCH], preferred_element_type=f32))
            up = _r(jnp.dot(xsel, wu[:, c0:c0 + FCH], preferred_element_type=f32))
            act = _r(gte * jax.nn.sigmoid(gte))
            hcol = (act * up).astype(bf16)
            part = jnp.dot(hcol, wd[c0:c0 + FCH, :], preferred_element_type=f32)
            yf = part if yf is None else yf + part
        if not last and not LINK:
            ln_block(0)
        rsel = _r(jax.nn.sigmoid(jnp.where(row16 == 0, m1, m2)))
        upd = _r(_r(yf) * rsel)
        x2 = _r(x1sel + _r(ysel + upd))
        rows2 = [jnp.sum(jnp.where(row16 == kk, x2, 0.0), axis=0, keepdims=True)
                 for kk in range(2)]
        if not last:
            xn2 = _layernorm(x2)
            for kk in range(2):
                xa[pl.ds(idx[kk], 1), :] = rows2[kk]
                one = jnp.sum(jnp.where(row16 == kk, xn2, 0.0), axis=0, keepdims=True)
                blk = _unpack(xn[_half(base[kk], 16), :]).astype(f32)
                xn[_half(base[kk], 16), :] = _pack(jnp.where(row16 == off[kk], one, blk))
        else:
            out_cp.wait()
            for kk in range(2):
                blk = xio[pl.ds(base[kk], 16), :].astype(f32)
                xio[pl.ds(base[kk], 16), :] = jnp.where(
                    row16 == off[kk], rows2[kk], blk).astype(bf16)
            cp0 = pltpu.make_async_copy(xio.at[pl.ds(base[0], 16), :],
                                        out_hbm.at[0, pl.ds(base[0], 16), :], sems.at[0])
            cp1 = pltpu.make_async_copy(xio.at[pl.ds(base[1], 16), :],
                                        out_hbm.at[0, pl.ds(base[1], 16), :], sems.at[1])
            cp0.start()

            @pl.when(base[0] != base[1])
            def _():
                cp1.start()
                cp1.wait()

            cp0.wait()

    if _ONLY:
        for c in x_cp + w_cp:
            c.wait()
        dict(O0=lambda: o_phase(False), O1=lambda: o_phase(True),
             B0=lambda: moe_phase(False),
             A=lambda: lax.fori_loop(0, G // AG, lambda i, c: (attn_groups(i * AG, AG, False), c)[1], 0))[_ONLY]()
        out_cp.start()
        out_cp.wait()
        return

    x_cp[0].wait()
    ln_block(0, xio)
    w_cp[7].wait()

    for li in range(2):
        last = li == 1
        z8 = jnp.zeros((8, 128), f32)
        if li == 0:
            vproj_block(0, True)
            lax.fori_loop(1, NSEG, lambda s, c: (vproj_block(s), c)[1], 0)
            for c in w_cp[1:4]:
                c.wait()
            qmax, kmax = lax.fori_loop(
                0, NSEG, lambda s, c: qkproj_block(s, c, False), (z8, z8))
        else:
            qmax, kmax = lax.fori_loop(
                0, NSEG, lambda s, c: qkproj_block(s, c, True), (z8, z8))
        bound = DH * jnp.max(qmax) * jnp.max(kmax)
        safe = bound <= SAFE_BOUND

        @pl.when(safe)
        def _():
            lax.fori_loop(0, G // AG, lambda i, c: (attn_groups(i * AG, AG, False), c)[1], 0)

        @pl.when(jnp.logical_not(safe))
        def _():
            lax.fori_loop(0, G, lambda g, c: (attn_groups(g, 1, True), c)[1], 0)

        o_phase(last)
        if li == 0:
            for c in w_cp[4:7]:
                c.wait()
        moe_phase(last)


@jax.jit
def pallas_interleave_layers__memory_aug_infini_attn__moe_arch_mod__prompt_kernel(
    A_x: jax.Array,
    A_wq: jax.Array,
    A_wk: jax.Array,
    A_wv: jax.Array,
    A_wo: jax.Array,
    A_beta: jax.Array,
    B_x: jax.Array,
    B_w_r: jax.Array,
    B_w_gate: jax.Array,
    B_w_up: jax.Array,
    B_w_down: jax.Array,
):
    del B_x
    any_spec = pl.BlockSpec(memory_space=pl.ANY)
    vm = pltpu.VMEM
    return pl.pallas_call(
        _kernel,
        out_shape=jax.ShapeDtypeStruct((1, S, D), bf16),
        in_specs=[pl.BlockSpec(memory_space=pltpu.SMEM),
                  pl.BlockSpec(memory_space=vm), pl.BlockSpec(memory_space=vm)] + [any_spec] * 8,
        out_specs=any_spec,
        scratch_shapes=[
            vm((S, D), bf16),
            vm((4, D, D), bf16),
            vm((S, D), f32),
            vm((S // 2, D), i32),
            vm((D // 2, D), i32),
            vm((G, S // 2, 128), i32), vm((G, S // 2, 128), i32),
            vm((G, S // 2, 128), i32), vm((G, S // 2, 128), i32),
            vm((NSEG, D // 2, L), i32),
            vm((G, S // 2, 128), i32),
            vm((S, D), bf16), vm((S, D), bf16),
            vm((NSEG, G, 8, 128), f32),
            vm((H, 128), f32),
            vm((S // OB, 128), f32),
            vm((ONB, OB, D), f32),
            vm((D, F), bf16), vm((D, F), bf16), vm((F, D), bf16),
            pltpu.SemaphoreType.DMA((NSEG + 8,)),
        ],
        compiler_params=pltpu.CompilerParams(vmem_limit_bytes=120 * 1024 * 1024, flags=_FLAGS),
    )(np.zeros((1,), np.int32), A_beta, B_w_r, A_x, A_wq, A_wk, A_wv, A_wo, B_w_gate, B_w_up, B_w_down)
```

```python
import math

import jax
import jax.numpy as jnp
import numpy as np
from jax import lax
import jax.experimental.pallas as pl
import jax.experimental.pallas.tpu as pltpu

S = 2048
D = 1024
H = 32
DH = D // H
NSEG = 4
L = S // NSEG
G = 8
F = 3584
OB = 32
OSTEP = 30
ONP = 2
LINK = 1
SPLITD = 1
ODELAY = 3
TIE = 1
TORD = 1230
ONB = 5
AG = 2
LAG = 2
FCH = 896

bf16 = jnp.bfloat16
f32 = jnp.float32
i32 = jnp.int32

QSCALE = (DH ** -0.5) * math.log2(math.e)
SAFE_BOUND = 24.0
NEG = -1e30
EPS_BF16 = 1.0013580322265625e-05

_NT = (((1,), (1,)), ((), ()))
_ONLY = None
_FLAGS = None


def _r(x):
    return x.astype(bf16).astype(f32)


def _pack(x):
    return pltpu.bitcast(x.astype(bf16), i32)


def _unpack(w):
    return pltpu.bitcast(w, bf16)


def _layernorm(xf):
    mean = jnp.sum(xf, axis=1, keepdims=True) * (1.0 / D)
    c = xf - mean
    var = jnp.sum(c * c, axis=1, keepdims=True) * (1.0 / D)
    d = _r(xf - _r(mean))
    s = _r(jnp.sqrt(_r(_r(var) + EPS_BF16)))
    return _r(d * (1.0 / s))


def _phi(t):
    return jnp.where(t > 0, t + 1.0, jnp.exp(t))


def _head_lanes(qi, h):
    lane = lax.broadcasted_iota(i32, qi.shape, 1)
    return _unpack(jnp.where((lane >> 5) == h, qi, 0))


def _fold8(x):
    return x.reshape(x.shape[0] // 8, 8, x.shape[1])


def _half(i, n):
    return pl.ds(i // 2 if isinstance(i, int) else pl.multiple_of(i // 2, n // 2), n // 2)


def _kernel(zero_s, beta_ref, wr_ref,
            x_hbm, wq_hbm, wk_hbm, wv_hbm, wo_hbm, wg_hbm, wu_hbm, wd_hbm,
            out_hbm,
            xio, wst, xa, xn, wo, qs, pq, ks, pk, vt, o_s, y_s, x1_s,
            zs, gt, r_s, oc, wg, wu, wd, sems):
    nx = NSEG
    x_cp = [pltpu.make_async_copy(x_hbm.at[0, pl.ds(i * L, L), :],
                                  xio.at[pl.ds(i * L, L), :], sems.at[i])
            for i in range(nx)]
    w_cp = [pltpu.make_async_copy(src, dst, sems.at[nx + i]) for i, (src, dst) in
            enumerate([(wv_hbm.at[:, pl.ds(D // 2, D // 2)], wst.at[0, :, pl.ds(D // 2, D // 2)]),
                       (wq_hbm, wst.at[1]), (wk_hbm, wst.at[2]),
                       (wo_hbm, wst.at[3]), (wg_hbm, wg), (wu_hbm, wu), (wd_hbm, wd),
                       (wv_hbm.at[:, pl.ds(0, D // 2)], wst.at[0, :, pl.ds(0, D // 2)])])]
    for c in (x_cp[0], w_cp[7], x_cp[1], w_cp[0], w_cp[1], w_cp[2], w_cp[3],
              x_cp[2], x_cp[3], w_cp[4], w_cp[5], w_cp[6]):
        c.start()

    b = jnp.broadcast_to(beta_ref[...].astype(f32).reshape(1, H), (H, H))
    rr = lax.broadcasted_iota(i32, (H, H), 0)
    cc = lax.broadcasted_iota(i32, (H, H), 1)
    bcol = jnp.sum(jnp.where(rr == cc, b, 0.0), axis=1, keepdims=True)
    gt[...] = _r(jax.nn.sigmoid(jnp.broadcast_to(bcol, (H, 128))))

    lane = lax.broadcasted_iota(i32, (128, 128), 1)
    row = lax.broadcasted_iota(i32, (128, 128), 0)

    def ln_rows(r0, n, src=None):
        src = xa if src is None else src
        xn[_half(r0, n), :] = _pack(_layernorm(src[pl.ds(r0, n), :].astype(f32)))

    def ln_block(r0, src=None):
        ln_rows(r0, L, src)

    def pin(w32, ref):
        zero = zero_s[0]
        lk = ref[pl.ds(pl.multiple_of(zero, 8), 8), 0:128] & zero
        head = jnp.concatenate([w32[0:8, 0:128] | lk, w32[0:8, 128:]], axis=1)
        return head if w32.shape[0] == 8 else jnp.concatenate([head, w32[8:]], axis=0)

    CB = 256

    def next_block(s):
        return pl.multiple_of(jnp.minimum(s + 1, NSEG - 1) * L, L)

    def v_cols(s, xb, lo, hi):
        for c0 in range(lo, hi, CB):
            v = jnp.dot(xb, wst[0, :, c0:c0 + CB], preferred_element_type=f32)
            vt[s, c0 // 2:(c0 + CB) // 2, :] = pltpu.bitcast(v.astype(bf16).T, i32)

    def q_cols(s, r0, xb, c0, qmax):
        q = jnp.dot(xb, wst[1, :, c0:c0 + CB], preferred_element_type=f32)
        for j in range(CB // 128):
            g = c0 // 128 + j
            qg = q[:, j * 128:(j + 1) * 128]
            qsc = qg * QSCALE
            qs[g, _half(r0, L), :] = _pack(qsc)
            pq[g, _half(r0, L), :] = _pack(_phi(qg))
            qmax = jnp.maximum(qmax, jnp.max(_fold8(jnp.abs(qsc)), axis=0))
        return qmax

    def k_cols(s, r0, xb, c0, kmax):
        k = jnp.dot(xb, wst[2, :, c0:c0 + CB], preferred_element_type=f32)
        for j in range(CB // 128):
            g = c0 // 128 + j
            kg = k[:, j * 128:(j + 1) * 128]
            ks[g, _half(r0, L), :] = _pack(kg)
            pkg = _phi(kg)
            pk[g, _half(r0, L), :] = _pack(pkg)
            zs[s, g] = jnp.sum(_fold8(pkg), axis=0)
            kmax = jnp.maximum(kmax, jnp.max(_fold8(jnp.abs(kg)), axis=0))
        return kmax

    def proj_first():
        z8 = jnp.zeros((8, 128), f32)
        v_cols(0, _unpack(xn[0:L // 2, :]), 0, D // 2)
        w_cp[0].wait()
        x_cp[1].wait()
        v_cols(0, _unpack(xn[0:L // 2, :]), D // 2, D)
        ln_block(L, xio)
        w_cp[1].wait()
        qmax = kmax = z8
        xb = _unpack(xn[0:L // 2, :])
        for c0 in range(0, D, CB):
            qmax = q_cols(0, 0, xb, c0, qmax)
        w_cp[2].wait()
        xb = _unpack(xn[0:L // 2, :])
        for c0 in range(0, D, CB):
            kmax = k_cols(0, 0, xb, c0, kmax)
        w_cp[3].wait()
        return qmax, kmax

    def proj_block(s, carry, li):
        qmax, kmax = carry
        if li == 0:
            for i in range(2, nx):
                @pl.when(s == i - 1)
                def _():
                    x_cp[i].wait()
        r0 = pl.multiple_of(s * L, L)
        xb = _unpack(xn[_half(r0, L), :])
        v_cols(s, xb, 0, D)
        for c0 in range(0, D, CB):
            qmax = q_cols(s, r0, xb, c0, qmax)
            kmax = k_cols(s, r0, xb, c0, kmax)
        ln_block(next_block(s), xio if li == 0 else xa)
        if li == 0:
            w0 = pl.multiple_of((s - 1) * 168, 8)
            wo[pl.ds(w0, 176), :] = _pack(wst[3, pl.ds(pl.multiple_of(2 * w0, 16), 352), :])
        return qmax, kmax

    def attn_groups(g0, ng, use_max):
        causal = row <= lane
        gs = [g0 + i for i in range(ng)]
        g64 = [pl.multiple_of(g * 64, 64) for g in gs]
        gate = [[gt[pl.ds(g * 4 + h, 1), :] for h in range(4)] for g in gs]
        blockdiag = (row >> 5) == (lane >> 5)
        lane16 = lax.broadcasted_iota(i32, (16, 128), 1)
        row16 = lax.broadcasted_iota(i32, (16, 128), 0)
        zmask = (lane16 >> 5) == row16

        def tile(ref, g, s, t):
            return ref[g, (s * L + t * 128) // 2:(s * L + (t + 1) * 128) // 2, :]

        split_diag = SPLITD and not use_max
        lane64 = lax.broadcasted_iota(i32, (64, 128), 1)
        causal64 = lax.broadcasted_iota(i32, (64, 128), 0) <= (lane64 & 63)
        low64 = lane64 < 64
        low8 = lax.broadcasted_iota(i32, (8, 128), 1) < 64

        def qk(gi, s, t, flip, link=None):
            g = gs[gi]
            qt = tile(qs, g, s, t)
            if link is not None:
                qt = jnp.concatenate([qt[0:8] | link, qt[8:]], axis=0)
            qlane = lax.broadcasted_iota(i32, qt.shape, 1)
            qi = [jnp.where((qlane >> 5) == h, qt, 0) for h in range(4)]
            qm = [_unpack(x) for x in qi]
            Sc = [[None] * (t + 1) for _ in range(4)]
            for j in range(t if split_diag else t + 1):
                kk = _unpack(tile(ks, g, s, j))
                for h in range(4):
                    Sc[h][j] = lax.dot_general(kk, qm[h], _NT, preferred_element_type=f32)
            if not split_diag:
                return Sc, None
            kd = tile(ks, g, s, t)
            T1, T2 = [None, None], [None, None]

            def t1(pr):
                w = _unpack(jnp.concatenate([qi[2 * pr][0:32], qi[2 * pr + 1][0:32]], axis=0))
                T1[pr] = lax.dot_general(_unpack(kd[0:32]), w, _NT, preferred_element_type=f32)

            def t2(pr):
                w = _unpack(jnp.concatenate([qi[2 * pr][32:64], qi[2 * pr + 1][32:64]], axis=0))
                T2[pr] = lax.dot_general(_unpack(kd), w, _NT, preferred_element_type=f32)

            for fn, pr in ((t2, 0), (t2, 1), (t1, 0), (t1, 1)) if flip else (
                    (t1, 0), (t1, 1), (t2, 0), (t2, 1)):
                fn(pr)
            return Sc, (T1, T2)

        def tie(x, part):
            if not TIE:
                return x
            n = x.shape[0] - 8
            return jnp.concatenate([x[:n], x[n:] + part * 0.0], axis=0)

        def sm(ScD, t):
            Sc, Dg = ScD
            P = [None] * 4
            Linv = [None] * 4
            l8 = [None] * 4
            for h in range(4):
                sc = list(Sc[h])
                if not split_diag:
                    sc[t] = jnp.where(causal, sc[t], NEG)
                else:
                    sc = sc[:t]
                if use_max:
                    m = sc[0]
                    for j in range(1, t + 1):
                        m = jnp.maximum(m, sc[j])
                    m = jnp.max(m, axis=0, keepdims=True)
                    p = [jnp.exp2(x - m) for x in sc]
                else:
                    p = [jnp.exp2(x) for x in sc]
                P[h] = []
                for x in p:
                    part = jnp.sum(_fold8(x), axis=0)
                    l8[h] = part if l8[h] is None else l8[h] + part
                    P[h].append(tie(x, part).astype(bf16))
            if split_diag:
                for pr in range(2):
                    a, b = 2 * pr, 2 * pr + 1
                    e1 = jnp.exp2(jnp.where(causal64, Dg[0][pr], NEG))
                    e2a = jnp.exp2(Dg[1][pr][0:64])
                    e2b = jnp.exp2(jnp.where(causal64, Dg[1][pr][64:128], NEG))
                    p1 = jnp.sum(_fold8(e1), axis=0)
                    p2 = jnp.sum(_fold8(e2a), axis=0) + jnp.sum(_fold8(e2b), axis=0)
                    la = jnp.where(low8, p1, pltpu.roll(p2, 64, 1))
                    lb = jnp.where(low8, pltpu.roll(p1, 64, 1), p2)
                    l8[a] = la if l8[a] is None else l8[a] + la
                    l8[b] = lb if l8[b] is None else l8[b] + lb
                    e1, e2b = tie(e1, p1), tie(e2b, p2)
                    P[a].append(jnp.concatenate(
                        [jnp.where(low64, e1, pltpu.roll(e2a, 64, 1)),
                         jnp.where(low64, 0.0, pltpu.roll(e2b, 64, 1))], axis=0).astype(bf16))
                    P[b].append(jnp.concatenate(
                        [jnp.where(low64, pltpu.roll(e1, 64, 1), e2a),
                         jnp.where(low64, 0.0, e2b)], axis=0).astype(bf16))
            for h in range(4):
                Linv[h] = 1.0 / jnp.sum(l8[h], axis=0, keepdims=True)
            return P, Linv

        def pv(PL, gi, s, t, lhs_m):
            g = gs[gi]
            P, Linv = PL
            acc = [None] * 4
            for j in range(t + 1):
                for h in range(4):
                    vth = _unpack(vt[s, pl.ds(g64[gi] + 16 * h, 16), j * 128:(j + 1) * 128])
                    o = jnp.dot(vth, P[h][j], preferred_element_type=f32)
                    acc[h] = o if acc[h] is None else acc[h] + o
            if lhs_m is not None:
                pqt = _unpack(tile(pq, g, s, t))
                nd = lax.dot_general(lhs_m, pqt, _NT, preferred_element_type=f32)
            outs = []
            for h in range(4):
                o = acc[h] * ((1.0 - gate[gi][h]) * Linv[h])
                if lhs_m is not None:
                    den = nd[128 + h:129 + h, :] + 1e-6
                    o = o + nd[32 * h:32 * h + 32, :] * (gate[gi][h] / den)
                outs.append(o)
            ot = jnp.concatenate(outs, axis=0).astype(bf16)
            o_s[g, (s * L + t * 128) // 2:(s * L + (t + 1) * 128) // 2, :] = (
                pltpu.bitcast(ot.T, i32))
            zero = zero_s[0]
            return o_s[g, pl.ds(pl.multiple_of((s * L + t * 128) // 2 + zero, 8), 8), :] & zero

        def mem_update(gi, s, R):
            g = gs[gi]
            vtg = _unpack(vt[s, pl.ds(g64[gi], 64), :])
            pks = _unpack(pk[g, s * L // 2:(s + 1) * L // 2, :])
            upd = jnp.dot(vtg, pks, preferred_element_type=f32)
            return upd if R is None else R + upd

        def mem_lhs(gi, s, R):
            g = gs[gi]
            mt = jnp.where(blockdiag, R, 0.0)
            z = zs[0, g]
            for s2 in range(1, s):
                z = z + zs[s2, g]
            z = jnp.sum(z, axis=0, keepdims=True)
            zr = jnp.where(zmask, z, 0.0)
            return jnp.concatenate([mt, zr], axis=0).astype(bf16)

        order = [int(c) for c in str(TORD).zfill(4)]
        steps = [(gi, s, t) for gi in range(ng) for s in range(NSEG) for t in order]
        n = len(steps)
        Sc, PL = {}, {}
        R = None
        lhs = {}
        links = {}
        for i in range(n + LAG):
            if i < n:
                Sc[i] = qk(*steps[i], i % 2 == 1,
                           links.get(i - LAG - ODELAY) if ODELAY else None)
                gi, s, t = steps[i]
                if t == order[0] and s == 0:
                    R = None
                    lhs[gi, 0] = None
                if t == order[-1] and s < NSEG - 1:
                    R = mem_update(gi, s, R)
                    lhs[gi, s + 1] = mem_lhs(gi, s + 1, R)
                PL[i] = sm(Sc.pop(i), t)
            if 0 <= i - LAG < n:
                gi, s, t = steps[i - LAG]
                links[i - LAG] = pv(PL.pop(i - LAG), gi, s, t, lhs[gi, s])

    CP, RP = D // ONP, OB // ONP

    def o_lhs(r0):
        return jnp.concatenate([_unpack(o_s[g, _half(r0, OB), :]) for g in range(G)], axis=1)

    def o_epilogue(refs, r0, out, last):
        xa_, x1_, y_, xo_ = refs
        res = xa_[r0:r0 + RP, :] if last else xo_[r0:r0 + RP, :].astype(f32)
        x1 = _r(res + _r(out))
        x1_[r0:r0 + RP, :] = x1.astype(bf16)
        y = _layernorm(x1)
        y_[r0:r0 + RP, :] = y.astype(bf16)
        if last:
            xo_[r0:r0 + RP, :] = (x1 + y).astype(bf16)
        else:
            xa_[r0:r0 + RP, :] = _r(x1 + y)
        wr = wr_ref[...].astype(f32).reshape(1, D)
        return _r(jnp.sum(y * wr, axis=1, keepdims=True))

    def o_refs(r0, n):
        return [xa.at[pl.ds(r0, n)], x1_s.at[pl.ds(r0, n)], y_s.at[pl.ds(r0, n)],
                xio.at[pl.ds(r0, n)]]

    def o_step(refs, k, blk, src, dst, last):
        if dst is not None:
            ob = o_lhs((blk + 1) * OB)
        rcols = []
        for p in range(ONP):
            if dst is not None:
                dst[:, p * CP:(p + 1) * CP] = jnp.dot(
                    ob, _unpack(wo[:, p * CP:(p + 1) * CP]), preferred_element_type=f32)
            rcols.append(o_epilogue(refs, k * OB + p * RP, src[p * RP:(p + 1) * RP, :], last))
        rb = jnp.broadcast_to(jnp.concatenate(rcols, axis=0), (OB, 128))
        lane_ob = lax.broadcasted_iota(i32, (OB, 128), 1)
        row_ob = lax.broadcasted_iota(i32, (OB, 128), 0)
        r_s[pl.ds(blk, 1), :] = jnp.max(jnp.where(row_ob == lane_ob, rb, -jnp.inf),
                                        axis=0, keepdims=True)

    def o_phase(last):
        nb = S // OB
        oc[0] = jnp.dot(o_lhs(0), _unpack(wo[...]), preferred_element_type=f32)
        nloop = (nb - 2) // OSTEP
        assert OSTEP % ONB == 0

        def out_rows(r0, n):
            return pltpu.make_async_copy(xio.at[pl.ds(r0, n)], out_hbm.at[0, pl.ds(r0, n)],
                                         sems.at[2])

        def body(i, carry):
            if last:
                @pl.when(i > 0)
                def _():
                    out_rows(pl.multiple_of((i - 1) * OSTEP * OB, OSTEP * OB),
                             OSTEP * OB).start()

            refs = o_refs(pl.multiple_of(i * OSTEP * OB, OSTEP * OB), OSTEP * OB)
            for k in range(OSTEP):
                o_step(refs, k, i * OSTEP + k, oc.at[k % ONB], oc.at[(k + 1) % ONB], last)
            return carry

        lax.fori_loop(0, nloop, body, 0)
        b0 = nloop * OSTEP
        if last:
            out_rows((b0 - OSTEP) * OB, OSTEP * OB).start()
        refs = o_refs(b0 * OB, (nb - b0) * OB)
        for k in range(nb - b0):
            o_step(refs, k, b0 + k, oc.at[k % ONB],
                   oc.at[(k + 1) % ONB] if b0 + k + 1 < nb else None, last)
        if last:
            out_rows(b0 * OB, (nb - b0) * OB).start()

    out_cp = pltpu.make_async_copy(xio, out_hbm.at[0], sems.at[2])

    def moe_phase(last):
        r_all = r_s[...]
        ridx = (lax.broadcasted_iota(i32, r_all.shape, 0) * OB
                + lax.broadcasted_iota(i32, r_all.shape, 1)).astype(f32)

        def red(fn, x):
            return fn(fn(x, axis=0, keepdims=True), axis=1, keepdims=True)

        m1 = red(jnp.max, r_all)
        i1f = red(jnp.min, jnp.where(r_all == m1, ridx, 1e9))
        r2 = jnp.where(ridx == i1f, -jnp.inf, r_all)
        m2 = red(jnp.max, r2)
        i2f = red(jnp.min, jnp.where((r2 == m2) & (ridx != i1f), ridx, 1e9))
        idx = [jnp.clip(v[0, 0].astype(i32), 0, S - 1) for v in (i1f, i2f)]
        base = [pl.multiple_of((ix >> 4) << 4, 16) for ix in idx]
        off = [ix & 15 for ix in idx]
        row16 = lax.broadcasted_iota(i32, (16, D), 0)

        def gather(ref):
            res = None
            for kk in range(2):
                blk = ref[pl.ds(base[kk], 16), :].astype(f32)
                one = jnp.sum(jnp.where(row16 == off[kk], blk, 0.0), axis=0, keepdims=True)
                part = jnp.where(row16 == kk, one, 0.0)
                res = part if res is None else res + part
            return res

        ysel = gather(y_s)
        x1sel = gather(x1_s)
        xsel32 = _pack(ysel)
        yf = None
        nch = F // FCH
        rp = L // nch
        for ci, c0 in enumerate(range(0, F, FCH)):
            if not last and LINK == 1:
                ln_rows(ci * rp, rp)
                xsel = _unpack(pin(xsel32, xn))
            elif not last and LINK == 2:
                if ci == 0:
                    ln_block(0)
                xsel = _unpack(pin(xsel32, xn) if ci == nch - 1 else xsel32)
            else:
                xsel = _unpack(xsel32)
            gte = _r(jnp.dot(xsel, wg[:, c0:c0 + FCH], preferred_element_type=f32))
            up = _r(jnp.dot(xsel, wu[:, c0:c0 + FCH], preferred_element_type=f32))
            act = _r(gte * jax.nn.sigmoid(gte))
            hcol = (act * up).astype(bf16)
            part = jnp.dot(hcol, wd[c0:c0 + FCH, :], preferred_element_type=f32)
            yf = part if yf is None else yf + part
        if not last and not LINK:
            ln_block(0)
        rsel = _r(jax.nn.sigmoid(jnp.where(row16 == 0, m1, m2)))
        upd = _r(_r(yf) * rsel)
        x2 = _r(x1sel + _r(ysel + upd))
        rows2 = [jnp.sum(jnp.where(row16 == kk, x2, 0.0), axis=0, keepdims=True)
                 for kk in range(2)]
        if not last:
            xn2 = _layernorm(x2)
            for kk in range(2):
                xa[pl.ds(idx[kk], 1), :] = rows2[kk]
                one = jnp.sum(jnp.where(row16 == kk, xn2, 0.0), axis=0, keepdims=True)
                blk = _unpack(xn[_half(base[kk], 16), :]).astype(f32)
                xn[_half(base[kk], 16), :] = _pack(jnp.where(row16 == off[kk], one, blk))
        else:
            out_cp.wait()
            for kk in range(2):
                blk = xio[pl.ds(base[kk], 16), :].astype(f32)
                xio[pl.ds(base[kk], 16), :] = jnp.where(
                    row16 == off[kk], rows2[kk], blk).astype(bf16)
            cp0 = pltpu.make_async_copy(xio.at[pl.ds(base[0], 16), :],
                                        out_hbm.at[0, pl.ds(base[0], 16), :], sems.at[0])
            cp1 = pltpu.make_async_copy(xio.at[pl.ds(base[1], 16), :],
                                        out_hbm.at[0, pl.ds(base[1], 16), :], sems.at[1])
            cp0.start()

            @pl.when(base[0] != base[1])
            def _():
                cp1.start()
                cp1.wait()

            cp0.wait()

    if _ONLY:
        for c in x_cp + w_cp:
            c.wait()
        dict(O0=lambda: o_phase(False), O1=lambda: o_phase(True),
             B0=lambda: moe_phase(False),
             A=lambda: lax.fori_loop(0, G // AG, lambda i, c: (attn_groups(i * AG, AG, False), c)[1], 0))[_ONLY]()
        out_cp.start()
        out_cp.wait()
        return

    x_cp[0].wait()
    ln_block(0, xio)
    w_cp[7].wait()

    for li in range(2):
        last = li == 1
        if li == 0:
            qmax, kmax = lax.fori_loop(1, NSEG, lambda s, c: proj_block(s, c, 0), proj_first())
        else:
            z8 = jnp.zeros((8, 128), f32)
            qmax, kmax = lax.fori_loop(0, NSEG, lambda s, c: proj_block(s, c, 1), (z8, z8))
        bound = DH * jnp.max(qmax) * jnp.max(kmax)
        safe = bound <= SAFE_BOUND

        @pl.when(safe)
        def _():
            lax.fori_loop(0, G // AG, lambda i, c: (attn_groups(i * AG, AG, False), c)[1], 0)

        @pl.when(jnp.logical_not(safe))
        def _():
            lax.fori_loop(0, G, lambda g, c: (attn_groups(g, 1, True), c)[1], 0)

        o_phase(last)
        if li == 0:
            for c in w_cp[4:7]:
                c.wait()
        moe_phase(last)


@jax.jit
def pallas_interleave_layers__memory_aug_infini_attn__moe_arch_mod__prompt_kernel(
    A_x: jax.Array,
    A_wq: jax.Array,
    A_wk: jax.Array,
    A_wv: jax.Array,
    A_wo: jax.Array,
    A_beta: jax.Array,
    B_x: jax.Array,
    B_w_r: jax.Array,
    B_w_gate: jax.Array,
    B_w_up: jax.Array,
    B_w_down: jax.Array,
):
    del B_x
    any_spec = pl.BlockSpec(memory_space=pl.ANY)
    vm = pltpu.VMEM
    return pl.pallas_call(
        _kernel,
        out_shape=jax.ShapeDtypeStruct((1, S, D), bf16),
        in_specs=[pl.BlockSpec(memory_space=pltpu.SMEM),
                  pl.BlockSpec(memory_space=vm), pl.BlockSpec(memory_space=vm)] + [any_spec] * 8,
        out_specs=any_spec,
        scratch_shapes=[
            vm((S, D), bf16),
            vm((4, D, D), bf16),
            vm((S, D), f32),
            vm((S // 2, D), i32),
            vm((D // 2, D), i32),
            vm((G, S // 2, 128), i32), vm((G, S // 2, 128), i32),
            vm((G, S // 2, 128), i32), vm((G, S // 2, 128), i32),
            vm((NSEG, D // 2, L), i32),
            vm((G, S // 2, 128), i32),
            vm((S, D), bf16), vm((S, D), bf16),
            vm((NSEG, G, 8, 128), f32),
            vm((H, 128), f32),
            vm((S // OB, 128), f32),
            vm((ONB, OB, D), f32),
            vm((D, F), bf16), vm((D, F), bf16), vm((F, D), bf16),
            pltpu.SemaphoreType.DMA((NSEG + 8,)),
        ],
        compiler_params=pltpu.CompilerParams(vmem_limit_bytes=120 * 1024 * 1024, flags=_FLAGS),
    )(np.zeros((1,), np.int32), A_beta, B_w_r, A_x, A_wq, A_wk, A_wv, A_wo, B_w_gate, B_w_up, B_w_down)
```

```python
import math

import jax
import jax.numpy as jnp
import numpy as np
from jax import lax
import jax.experimental.pallas as pl
import jax.experimental.pallas.tpu as pltpu

S = 2048
D = 1024
H = 32
DH = D // H
NSEG = 4
L = S // NSEG
G = 8
F = 3584
OB = 32
OSTEP = 30
ONP = 2
NLN = 4
LNE = 1
SPLITD = 1
ODELAY = 3
TIE = 1
TORD = 1230
ONB = 5
AG = 2
LAG = 2
FCH = 896

bf16 = jnp.bfloat16
f32 = jnp.float32
i32 = jnp.int32

QSCALE = (DH ** -0.5) * math.log2(math.e)
SAFE_BOUND = 24.0
NEG = -1e30
EPS_BF16 = 1.0013580322265625e-05

_NT = (((1,), (1,)), ((), ()))
_ONLY = None
_FLAGS = None


def _r(x):
    return x.astype(bf16).astype(f32)


def _pack(x):
    return pltpu.bitcast(x.astype(bf16), i32)


def _unpack(w):
    return pltpu.bitcast(w, bf16)


def _layernorm(xf):
    mean = jnp.sum(xf, axis=1, keepdims=True) * (1.0 / D)
    c = xf - mean
    var = jnp.sum(c * c, axis=1, keepdims=True) * (1.0 / D)
    d = _r(xf - _r(mean))
    s = _r(jnp.sqrt(_r(_r(var) + EPS_BF16)))
    return _r(d * (1.0 / s))


def _phi(t):
    return jnp.where(t > 0, t + 1.0, jnp.exp(t))


def _head_lanes(qi, h):
    lane = lax.broadcasted_iota(i32, qi.shape, 1)
    return _unpack(jnp.where((lane >> 5) == h, qi, 0))


def _fold8(x):
    return x.reshape(x.shape[0] // 8, 8, x.shape[1])


def _half(i, n):
    return pl.ds(i // 2 if isinstance(i, int) else pl.multiple_of(i // 2, n // 2), n // 2)


def _kernel(zero_s, beta_ref, wr_ref,
            x_hbm, wq_hbm, wk_hbm, wv_hbm, wo_hbm, wg_hbm, wu_hbm, wd_hbm,
            out_hbm,
            xio, wst, xa, xn, wo, qs, pq, ks, pk, vt, o_s, y_s, x1_s,
            zs, gt, r_s, oc, wg, wu, wd, sems):
    nx = NSEG
    x_cp = [pltpu.make_async_copy(x_hbm.at[0, pl.ds(i * L, L), :],
                                  xio.at[pl.ds(i * L, L), :], sems.at[i])
            for i in range(nx)]
    w_cp = [pltpu.make_async_copy(src, dst, sems.at[nx + i]) for i, (src, dst) in
            enumerate([(wv_hbm.at[:, pl.ds(D // 2, D // 2)], wst.at[0, :, pl.ds(D // 2, D // 2)]),
                       (wq_hbm, wst.at[1]), (wk_hbm, wst.at[2]),
                       (wo_hbm, wst.at[3]), (wg_hbm, wg), (wu_hbm, wu), (wd_hbm, wd),
                       (wv_hbm.at[:, pl.ds(0, D // 2)], wst.at[0, :, pl.ds(0, D // 2)])])]
    for c in (x_cp[0], w_cp[7], x_cp[1], w_cp[0], w_cp[1], w_cp[2], w_cp[3],
              x_cp[2], x_cp[3], w_cp[4], w_cp[5], w_cp[6]):
        c.start()

    b = jnp.broadcast_to(beta_ref[...].astype(f32).reshape(1, H), (H, H))
    rr = lax.broadcasted_iota(i32, (H, H), 0)
    cc = lax.broadcasted_iota(i32, (H, H), 1)
    bcol = jnp.sum(jnp.where(rr == cc, b, 0.0), axis=1, keepdims=True)
    gt[...] = _r(jax.nn.sigmoid(jnp.broadcast_to(bcol, (H, 128))))

    lane = lax.broadcasted_iota(i32, (128, 128), 1)
    row = lax.broadcasted_iota(i32, (128, 128), 0)

    def ln_rows(r0, n, src=None, after=None):
        src = xa if src is None else src
        xf = src[pl.ds(r0, n), :].astype(f32)
        if after is not None:
            z = pltpu.bitcast(jnp.concatenate([after] * (n // 8), axis=0), f32)
            xf = jnp.concatenate([xf[:, 0:128] + z, xf[:, 128:]], axis=1)
        xn[_half(r0, n), :] = _pack(_layernorm(xf))

    def ln_block(r0, src=None):
        ln_rows(r0, L, src)

    def pin(w32, ref):
        zero = zero_s[0]
        lk = ref[pl.ds(pl.multiple_of(zero, 8), 8), 0:128] & zero
        head = jnp.concatenate([w32[0:8, 0:128] | lk, w32[0:8, 128:]], axis=1)
        return head if w32.shape[0] == 8 else jnp.concatenate([head, w32[8:]], axis=0)

    CB = 256

    def next_block(s):
        return pl.multiple_of(jnp.minimum(s + 1, NSEG - 1) * L, L)

    def v_cols(s, xb, lo, hi):
        for c0 in range(lo, hi, CB):
            v = jnp.dot(xb, wst[0, :, c0:c0 + CB], preferred_element_type=f32)
            vt[s, c0 // 2:(c0 + CB) // 2, :] = pltpu.bitcast(v.astype(bf16).T, i32)

    def q_cols(s, r0, xb, c0, qmax):
        q = jnp.dot(xb, wst[1, :, c0:c0 + CB], preferred_element_type=f32)
        for j in range(CB // 128):
            g = c0 // 128 + j
            qg = q[:, j * 128:(j + 1) * 128]
            qsc = qg * QSCALE
            qs[g, _half(r0, L), :] = _pack(qsc)
            pq[g, _half(r0, L), :] = _pack(_phi(qg))
            qmax = jnp.maximum(qmax, jnp.max(_fold8(jnp.abs(qsc)), axis=0))
        return qmax

    def k_cols(s, r0, xb, c0, kmax):
        k = jnp.dot(xb, wst[2, :, c0:c0 + CB], preferred_element_type=f32)
        for j in range(CB // 128):
            g = c0 // 128 + j
            kg = k[:, j * 128:(j + 1) * 128]
            ks[g, _half(r0, L), :] = _pack(kg)
            pkg = _phi(kg)
            pk[g, _half(r0, L), :] = _pack(pkg)
            zs[s, g] = jnp.sum(_fold8(pkg), axis=0)
            kmax = jnp.maximum(kmax, jnp.max(_fold8(jnp.abs(kg)), axis=0))
        return kmax

    def proj_first():
        z8 = jnp.zeros((8, 128), f32)
        v_cols(0, _unpack(xn[0:L // 2, :]), 0, D // 2)
        w_cp[0].wait()
        x_cp[1].wait()
        v_cols(0, _unpack(xn[0:L // 2, :]), D // 2, D)
        ln_block(L, xio)
        w_cp[1].wait()
        qmax = kmax = z8
        xb = _unpack(xn[0:L // 2, :])
        for c0 in range(0, D, CB):
            qmax = q_cols(0, 0, xb, c0, qmax)
        w_cp[2].wait()
        xb = _unpack(xn[0:L // 2, :])
        for c0 in range(0, D, CB):
            kmax = k_cols(0, 0, xb, c0, kmax)
        w_cp[3].wait()
        return qmax, kmax

    def proj_block(s, carry, li):
        qmax, kmax = carry
        if li == 0:
            for i in range(2, nx):
                @pl.when(s == i - 1)
                def _():
                    x_cp[i].wait()
        r0 = pl.multiple_of(s * L, L)
        xb = _unpack(xn[_half(r0, L), :])
        v_cols(s, xb, 0, D)
        for c0 in range(0, D, CB):
            qmax = q_cols(s, r0, xb, c0, qmax)
            kmax = k_cols(s, r0, xb, c0, kmax)
        ln_block(next_block(s), xio if li == 0 else xa)
        if li == 0:
            w0 = pl.multiple_of((s - 1) * 168, 8)
            wo[pl.ds(w0, 176), :] = _pack(wst[3, pl.ds(pl.multiple_of(2 * w0, 16), 352), :])
        return qmax, kmax

    def attn_groups(g0, ng, use_max):
        causal = row <= lane
        gs = [g0 + i for i in range(ng)]
        g64 = [pl.multiple_of(g * 64, 64) for g in gs]
        gate = [[gt[pl.ds(g * 4 + h, 1), :] for h in range(4)] for g in gs]
        blockdiag = (row >> 5) == (lane >> 5)
        lane16 = lax.broadcasted_iota(i32, (16, 128), 1)
        row16 = lax.broadcasted_iota(i32, (16, 128), 0)
        zmask = (lane16 >> 5) == row16

        def tile(ref, g, s, t):
            return ref[g, (s * L + t * 128) // 2:(s * L + (t + 1) * 128) // 2, :]

        split_diag = SPLITD and not use_max
        lane64 = lax.broadcasted_iota(i32, (64, 128), 1)
        causal64 = lax.broadcasted_iota(i32, (64, 128), 0) <= (lane64 & 63)
        low64 = lane64 < 64
        low8 = lax.broadcasted_iota(i32, (8, 128), 1) < 64

        def qk(gi, s, t, flip, link=None):
            g = gs[gi]
            qt = tile(qs, g, s, t)
            if link is not None:
                qt = jnp.concatenate([qt[0:8] | link, qt[8:]], axis=0)
            qlane = lax.broadcasted_iota(i32, qt.shape, 1)
            qi = [jnp.where((qlane >> 5) == h, qt, 0) for h in range(4)]
            qm = [_unpack(x) for x in qi]
            Sc = [[None] * (t + 1) for _ in range(4)]
            for j in range(t if split_diag else t + 1):
                kk = _unpack(tile(ks, g, s, j))
                for h in range(4):
                    Sc[h][j] = lax.dot_general(kk, qm[h], _NT, preferred_element_type=f32)
            if not split_diag:
                return Sc, None
            kd = tile(ks, g, s, t)
            T1, T2 = [None, None], [None, None]

            def t1(pr):
                w = _unpack(jnp.concatenate([qi[2 * pr][0:32], qi[2 * pr + 1][0:32]], axis=0))
                T1[pr] = lax.dot_general(_unpack(kd[0:32]), w, _NT, preferred_element_type=f32)

            def t2(pr):
                w = _unpack(jnp.concatenate([qi[2 * pr][32:64], qi[2 * pr + 1][32:64]], axis=0))
                T2[pr] = lax.dot_general(_unpack(kd), w, _NT, preferred_element_type=f32)

            for fn, pr in ((t2, 0), (t2, 1), (t1, 0), (t1, 1)) if flip else (
                    (t1, 0), (t1, 1), (t2, 0), (t2, 1)):
                fn(pr)
            return Sc, (T1, T2)

        def tie(x, part):
            if not TIE:
                return x
            n = x.shape[0] - 8
            return jnp.concatenate([x[:n], x[n:] + part * 0.0], axis=0)

        def sm(ScD, t):
            Sc, Dg = ScD
            P = [None] * 4
            Linv = [None] * 4
            l8 = [None] * 4
            for h in range(4):
                sc = list(Sc[h])
                if not split_diag:
                    sc[t] = jnp.where(causal, sc[t], NEG)
                else:
                    sc = sc[:t]
                if use_max:
                    m = sc[0]
                    for j in range(1, t + 1):
                        m = jnp.maximum(m, sc[j])
                    m = jnp.max(m, axis=0, keepdims=True)
                    p = [jnp.exp2(x - m) for x in sc]
                else:
                    p = [jnp.exp2(x) for x in sc]
                P[h] = []
                for x in p:
                    part = jnp.sum(_fold8(x), axis=0)
                    l8[h] = part if l8[h] is None else l8[h] + part
                    P[h].append(tie(x, part).astype(bf16))
            if split_diag:
                for pr in range(2):
                    a, b = 2 * pr, 2 * pr + 1
                    e1 = jnp.exp2(jnp.where(causal64, Dg[0][pr], NEG))
                    e2a = jnp.exp2(Dg[1][pr][0:64])
                    e2b = jnp.exp2(jnp.where(causal64, Dg[1][pr][64:128], NEG))
                    p1 = jnp.sum(_fold8(e1), axis=0)
                    p2 = jnp.sum(_fold8(e2a), axis=0) + jnp.sum(_fold8(e2b), axis=0)
                    la = jnp.where(low8, p1, pltpu.roll(p2, 64, 1))
                    lb = jnp.where(low8, pltpu.roll(p1, 64, 1), p2)
                    l8[a] = la if l8[a] is None else l8[a] + la
                    l8[b] = lb if l8[b] is None else l8[b] + lb
                    e1, e2b = tie(e1, p1), tie(e2b, p2)
                    P[a].append(jnp.concatenate(
                        [jnp.where(low64, e1, pltpu.roll(e2a, 64, 1)),
                         jnp.where(low64, 0.0, pltpu.roll(e2b, 64, 1))], axis=0).astype(bf16))
                    P[b].append(jnp.concatenate(
                        [jnp.where(low64, pltpu.roll(e1, 64, 1), e2a),
                         jnp.where(low64, 0.0, e2b)], axis=0).astype(bf16))
            for h in range(4):
                Linv[h] = 1.0 / jnp.sum(l8[h], axis=0, keepdims=True)
            return P, Linv

        def pv(PL, gi, s, t, lhs_m):
            g = gs[gi]
            P, Linv = PL
            acc = [None] * 4
            for j in range(t + 1):
                for h in range(4):
                    vth = _unpack(vt[s, pl.ds(g64[gi] + 16 * h, 16), j * 128:(j + 1) * 128])
                    o = jnp.dot(vth, P[h][j], preferred_element_type=f32)
                    acc[h] = o if acc[h] is None else acc[h] + o
            if lhs_m is not None:
                pqt = _unpack(tile(pq, g, s, t))
                nd = lax.dot_general(lhs_m, pqt, _NT, preferred_element_type=f32)
            outs = []
            for h in range(4):
                o = acc[h] * ((1.0 - gate[gi][h]) * Linv[h])
                if lhs_m is not None:
                    den = nd[128 + h:129 + h, :] + 1e-6
                    o = o + nd[32 * h:32 * h + 32, :] * (gate[gi][h] / den)
                outs.append(o)
            ot = jnp.concatenate(outs, axis=0).astype(bf16)
            o_s[g, (s * L + t * 128) // 2:(s * L + (t + 1) * 128) // 2, :] = (
                pltpu.bitcast(ot.T, i32))
            zero = zero_s[0]
            return o_s[g, pl.ds(pl.multiple_of((s * L + t * 128) // 2 + zero, 8), 8), :] & zero

        def mem_update(gi, s, R):
            g = gs[gi]
            vtg = _unpack(vt[s, pl.ds(g64[gi], 64), :])
            pks = _unpack(pk[g, s * L // 2:(s + 1) * L // 2, :])
            upd = jnp.dot(vtg, pks, preferred_element_type=f32)
            return upd if R is None else R + upd

        def mem_lhs(gi, s, R):
            g = gs[gi]
            mt = jnp.where(blockdiag, R, 0.0)
            z = zs[0, g]
            for s2 in range(1, s):
                z = z + zs[s2, g]
            z = jnp.sum(z, axis=0, keepdims=True)
            zr = jnp.where(zmask, z, 0.0)
            return jnp.concatenate([mt, zr], axis=0).astype(bf16)

        order = [int(c) for c in str(TORD).zfill(4)]
        steps = [(gi, s, t) for gi in range(ng) for s in range(NSEG) for t in order]
        n = len(steps)
        Sc, PL = {}, {}
        R = None
        lhs = {}
        links = {}
        for i in range(n + LAG):
            if i < n:
                Sc[i] = qk(*steps[i], i % 2 == 1,
                           links.get(i - LAG - ODELAY) if ODELAY else None)
                gi, s, t = steps[i]
                if t == order[0] and s == 0:
                    R = None
                    lhs[gi, 0] = None
                if t == order[-1] and s < NSEG - 1:
                    R = mem_update(gi, s, R)
                    lhs[gi, s + 1] = mem_lhs(gi, s + 1, R)
                PL[i] = sm(Sc.pop(i), t)
            if 0 <= i - LAG < n:
                gi, s, t = steps[i - LAG]
                links[i - LAG] = pv(PL.pop(i - LAG), gi, s, t, lhs[gi, s])

    CP, RP = D // ONP, OB // ONP

    def o_lhs(r0):
        return jnp.concatenate([_unpack(o_s[g, _half(r0, OB), :]) for g in range(G)], axis=1)

    def o_epilogue(refs, r0, out, last):
        xa_, x1_, y_, xo_ = refs
        res = xa_[r0:r0 + RP, :] if last else xo_[r0:r0 + RP, :].astype(f32)
        x1 = _r(res + _r(out))
        x1_[r0:r0 + RP, :] = x1.astype(bf16)
        y = _layernorm(x1)
        y_[r0:r0 + RP, :] = y.astype(bf16)
        if last:
            xo_[r0:r0 + RP, :] = (x1 + y).astype(bf16)
        else:
            xa_[r0:r0 + RP, :] = _r(x1 + y)
        wr = wr_ref[...].astype(f32).reshape(1, D)
        return _r(jnp.sum(y * wr, axis=1, keepdims=True))

    def o_refs(r0, n):
        return [xa.at[pl.ds(r0, n)], x1_s.at[pl.ds(r0, n)], y_s.at[pl.ds(r0, n)],
                xio.at[pl.ds(r0, n)]]

    def o_step(refs, k, blk, src, dst, last):
        if dst is not None:
            ob = o_lhs((blk + 1) * OB)
        rcols = []
        for p in range(ONP):
            if dst is not None:
                dst[:, p * CP:(p + 1) * CP] = jnp.dot(
                    ob, _unpack(wo[:, p * CP:(p + 1) * CP]), preferred_element_type=f32)
            rcols.append(o_epilogue(refs, k * OB + p * RP, src[p * RP:(p + 1) * RP, :], last))
        rb = jnp.broadcast_to(jnp.concatenate(rcols, axis=0), (OB, 128))
        lane_ob = lax.broadcasted_iota(i32, (OB, 128), 1)
        row_ob = lax.broadcasted_iota(i32, (OB, 128), 0)
        r_s[pl.ds(blk, 1), :] = jnp.max(jnp.where(row_ob == lane_ob, rb, -jnp.inf),
                                        axis=0, keepdims=True)

    def o_phase(last):
        nb = S // OB
        oc[0] = jnp.dot(o_lhs(0), _unpack(wo[...]), preferred_element_type=f32)
        nloop = (nb - 2) // OSTEP
        assert OSTEP % ONB == 0

        def out_rows(r0, n):
            return pltpu.make_async_copy(xio.at[pl.ds(r0, n)], out_hbm.at[0, pl.ds(r0, n)],
                                         sems.at[2])

        def body(i, carry):
            if last:
                @pl.when(i > 0)
                def _():
                    out_rows(pl.multiple_of((i - 1) * OSTEP * OB, OSTEP * OB),
                             OSTEP * OB).start()

            refs = o_refs(pl.multiple_of(i * OSTEP * OB, OSTEP * OB), OSTEP * OB)
            for k in range(OSTEP):
                o_step(refs, k, i * OSTEP + k, oc.at[k % ONB], oc.at[(k + 1) % ONB], last)
            return carry

        lax.fori_loop(0, nloop, body, 0)
        b0 = nloop * OSTEP
        if last:
            out_rows((b0 - OSTEP) * OB, OSTEP * OB).start()
        refs = o_refs(b0 * OB, (nb - b0) * OB)
        for k in range(nb - b0):
            o_step(refs, k, b0 + k, oc.at[k % ONB],
                   oc.at[(k + 1) % ONB] if b0 + k + 1 < nb else None, last)
        if last:
            out_rows(b0 * OB, (nb - b0) * OB).start()

    out_cp = pltpu.make_async_copy(xio, out_hbm.at[0], sems.at[2])

    def moe_phase(last):
        r_all = r_s[...]
        ridx = (lax.broadcasted_iota(i32, r_all.shape, 0) * OB
                + lax.broadcasted_iota(i32, r_all.shape, 1)).astype(f32)

        def red(fn, x):
            return fn(fn(x, axis=0, keepdims=True), axis=1, keepdims=True)

        m1 = red(jnp.max, r_all)
        i1f = red(jnp.min, jnp.where(r_all == m1, ridx, 1e9))
        r2 = jnp.where(ridx == i1f, -jnp.inf, r_all)
        m2 = red(jnp.max, r2)
        i2f = red(jnp.min, jnp.where((r2 == m2) & (ridx != i1f), ridx, 1e9))
        idx = [jnp.clip(v[0, 0].astype(i32), 0, S - 1) for v in (i1f, i2f)]
        base = [pl.multiple_of((ix >> 4) << 4, 16) for ix in idx]
        off = [ix & 15 for ix in idx]
        row16 = lax.broadcasted_iota(i32, (16, D), 0)

        def gather(ref):
            res = None
            for kk in range(2):
                blk = ref[pl.ds(base[kk], 16), :].astype(f32)
                one = jnp.sum(jnp.where(row16 == off[kk], blk, 0.0), axis=0, keepdims=True)
                part = jnp.where(row16 == kk, one, 0.0)
                res = part if res is None else res + part
            return res

        ysel = gather(y_s)
        x1sel = gather(x1_s)
        xsel32 = _pack(ysel)
        yf = None
        after = None
        nch = F // FCH
        rp = L // NLN
        for ci, c0 in enumerate(range(0, F, FCH)):
            if not last and ci % LNE == 0 and ci // LNE < NLN:
                ln_rows(ci // LNE * rp, rp, None, after)
                xsel = _unpack(pin(xsel32, xn))
            else:
                xsel = _unpack(xsel32)
            gte = _r(jnp.dot(xsel, wg[:, c0:c0 + FCH], preferred_element_type=f32))
            after = pltpu.bitcast(gte[0:8, 0:128], i32) & zero_s[0]
            up = _r(jnp.dot(xsel, wu[:, c0:c0 + FCH], preferred_element_type=f32))
            act = _r(gte * jax.nn.sigmoid(gte))
            hcol = (act * up).astype(bf16)
            part = jnp.dot(hcol, wd[c0:c0 + FCH, :], preferred_element_type=f32)
            yf = part if yf is None else yf + part
        rsel = _r(jax.nn.sigmoid(jnp.where(row16 == 0, m1, m2)))
        upd = _r(_r(yf) * rsel)
        x2 = _r(x1sel + _r(ysel + upd))
        rows2 = [jnp.sum(jnp.where(row16 == kk, x2, 0.0), axis=0, keepdims=True)
                 for kk in range(2)]
        if not last:
            xn2 = _layernorm(x2)
            for kk in range(2):
                xa[pl.ds(idx[kk], 1), :] = rows2[kk]
                one = jnp.sum(jnp.where(row16 == kk, xn2, 0.0), axis=0, keepdims=True)
                blk = _unpack(xn[_half(base[kk], 16), :]).astype(f32)
                xn[_half(base[kk], 16), :] = _pack(jnp.where(row16 == off[kk], one, blk))
        else:
            out_cp.wait()
            for kk in range(2):
                blk = xio[pl.ds(base[kk], 16), :].astype(f32)
                xio[pl.ds(base[kk], 16), :] = jnp.where(
                    row16 == off[kk], rows2[kk], blk).astype(bf16)
            cp0 = pltpu.make_async_copy(xio.at[pl.ds(base[0], 16), :],
                                        out_hbm.at[0, pl.ds(base[0], 16), :], sems.at[0])
            cp1 = pltpu.make_async_copy(xio.at[pl.ds(base[1], 16), :],
                                        out_hbm.at[0, pl.ds(base[1], 16), :], sems.at[1])
            cp0.start()

            @pl.when(base[0] != base[1])
            def _():
                cp1.start()
                cp1.wait()

            cp0.wait()

    if _ONLY:
        for c in x_cp + w_cp:
            c.wait()
        dict(O0=lambda: o_phase(False), O1=lambda: o_phase(True),
             B0=lambda: moe_phase(False),
             A=lambda: lax.fori_loop(0, G // AG, lambda i, c: (attn_groups(i * AG, AG, False), c)[1], 0))[_ONLY]()
        out_cp.start()
        out_cp.wait()
        return

    x_cp[0].wait()
    ln_block(0, xio)
    w_cp[7].wait()

    for li in range(2):
        last = li == 1
        if li == 0:
            qmax, kmax = lax.fori_loop(1, NSEG, lambda s, c: proj_block(s, c, 0), proj_first())
        else:
            z8 = jnp.zeros((8, 128), f32)
            qmax, kmax = lax.fori_loop(0, NSEG, lambda s, c: proj_block(s, c, 1), (z8, z8))
        bound = DH * jnp.max(qmax) * jnp.max(kmax)
        safe = bound <= SAFE_BOUND

        @pl.when(safe)
        def _():
            lax.fori_loop(0, G // AG, lambda i, c: (attn_groups(i * AG, AG, False), c)[1], 0)

        @pl.when(jnp.logical_not(safe))
        def _():
            lax.fori_loop(0, G, lambda g, c: (attn_groups(g, 1, True), c)[1], 0)

        o_phase(last)
        if li == 0:
            for c in w_cp[4:7]:
                c.wait()
        moe_phase(last)


@jax.jit
def pallas_interleave_layers__memory_aug_infini_attn__moe_arch_mod__prompt_kernel(
    A_x: jax.Array,
    A_wq: jax.Array,
    A_wk: jax.Array,
    A_wv: jax.Array,
    A_wo: jax.Array,
    A_beta: jax.Array,
    B_x: jax.Array,
    B_w_r: jax.Array,
    B_w_gate: jax.Array,
    B_w_up: jax.Array,
    B_w_down: jax.Array,
):
    del B_x
    any_spec = pl.BlockSpec(memory_space=pl.ANY)
    vm = pltpu.VMEM
    return pl.pallas_call(
        _kernel,
        out_shape=jax.ShapeDtypeStruct((1, S, D), bf16),
        in_specs=[pl.BlockSpec(memory_space=pltpu.SMEM),
                  pl.BlockSpec(memory_space=vm), pl.BlockSpec(memory_space=vm)] + [any_spec] * 8,
        out_specs=any_spec,
        scratch_shapes=[
            vm((S, D), bf16),
            vm((4, D, D), bf16),
            vm((S, D), f32),
            vm((S // 2, D), i32),
            vm((D // 2, D), i32),
            vm((G, S // 2, 128), i32), vm((G, S // 2, 128), i32),
            vm((G, S // 2, 128), i32), vm((G, S // 2, 128), i32),
            vm((NSEG, D // 2, L), i32),
            vm((G, S // 2, 128), i32),
            vm((S, D), bf16), vm((S, D), bf16),
            vm((NSEG, G, 8, 128), f32),
            vm((H, 128), f32),
            vm((S // OB, 128), f32),
            vm((ONB, OB, D), f32),
            vm((D, F), bf16), vm((D, F), bf16), vm((F, D), bf16),
            pltpu.SemaphoreType.DMA((NSEG + 8,)),
        ],
        compiler_params=pltpu.CompilerParams(vmem_limit_bytes=120 * 1024 * 1024, flags=_FLAGS),
    )(np.zeros((1,), np.int32), A_beta, B_w_r, A_x, A_wq, A_wk, A_wv, A_wo, B_w_gate, B_w_up, B_w_down)
```

```python
import math

import jax
import jax.numpy as jnp
import numpy as np
from jax import lax
import jax.experimental.pallas as pl
import jax.experimental.pallas.tpu as pltpu

S = 2048
D = 1024
H = 32
DH = D // H
NSEG = 4
L = S // NSEG
G = 8
F = 3584
OB = 32
OSTEP = 30
ONP = 2
NLN = 4
LNE = 1
SPLITD = 1
ODELAY = 3
TIE = 1
TORD = 1230
ONB = 5
AG = 2
LAG = 2
FCH = 896

bf16 = jnp.bfloat16
f32 = jnp.float32
i32 = jnp.int32

QSCALE = (DH ** -0.5) * math.log2(math.e)
SAFE_BOUND = 24.0
NEG = -1e30
EPS_BF16 = 1.0013580322265625e-05

_NT = (((1,), (1,)), ((), ()))
_ONLY = None
_FLAGS = None


def _r(x):
    return x.astype(bf16).astype(f32)


def _pack(x):
    return pltpu.bitcast(x.astype(bf16), i32)


def _unpack(w):
    return pltpu.bitcast(w, bf16)


def _layernorm(xf):
    mean = jnp.sum(xf, axis=1, keepdims=True) * (1.0 / D)
    c = xf - mean
    var = jnp.sum(c * c, axis=1, keepdims=True) * (1.0 / D)
    d = _r(xf - _r(mean))
    s = _r(jnp.sqrt(_r(_r(var) + EPS_BF16)))
    return _r(d * (1.0 / s))


def _phi(t):
    return jnp.where(t > 0, t + 1.0, jnp.exp(t))


def _head_lanes(qi, h):
    lane = lax.broadcasted_iota(i32, qi.shape, 1)
    return _unpack(jnp.where((lane >> 5) == h, qi, 0))


def _fold8(x):
    return x.reshape(x.shape[0] // 8, 8, x.shape[1])


def _half(i, n):
    return pl.ds(i // 2 if isinstance(i, int) else pl.multiple_of(i // 2, n // 2), n // 2)


def _kernel(zero_s, beta_ref, wr_ref,
            x_hbm, wq_hbm, wk_hbm, wv_hbm, wo_hbm, wg_hbm, wu_hbm, wd_hbm,
            out_hbm,
            xio, wst, xa, xn, wo, qs, pq, ks, pk, vt, o_s, y_s, x1_s,
            zs, gt, r_s, oc, wg, wu, wd, sems):
    nx = NSEG
    XP = L // 4
    QD = D // 4

    def cp(src, dst, i):
        return pltpu.make_async_copy(src, dst, sems.at[i])

    def wcols(lo, n):
        return wv_hbm.at[:, pl.ds(lo, n)], wst.at[0, :, pl.ds(lo, n)]

    x0_cp = [cp(x_hbm.at[0, pl.ds(i * XP, XP), :], xio.at[pl.ds(i * XP, XP), :], i)
             for i in range(4)]
    x_cp = [None] + [cp(x_hbm.at[0, pl.ds(i * L, L), :], xio.at[pl.ds(i * L, L), :], 3 + i)
                     for i in range(1, nx)]
    wv_cp = [cp(*wcols(0, QD), 7), cp(*wcols(QD, QD), 8), cp(*wcols(2 * QD, 2 * QD), 9)]
    w_cp = [cp(src, dst, 10 + i) for i, (src, dst) in
            enumerate([(wq_hbm, wst.at[1]), (wk_hbm, wst.at[2]), (wo_hbm, wst.at[3]),
                       (wg_hbm, wg), (wu_hbm, wu), (wd_hbm, wd)])]
    for c in x0_cp + wv_cp + w_cp[:2] + x_cp[1:2] + w_cp[2:3] + x_cp[2:] + w_cp[3:]:
        c.start()

    b = jnp.broadcast_to(beta_ref[...].astype(f32).reshape(1, H), (H, H))
    rr = lax.broadcasted_iota(i32, (H, H), 0)
    cc = lax.broadcasted_iota(i32, (H, H), 1)
    bcol = jnp.sum(jnp.where(rr == cc, b, 0.0), axis=1, keepdims=True)
    gsig = _r(jax.nn.sigmoid(jnp.broadcast_to(bcol, (H, 128))))
    gt[0:H, :] = gsig
    gt[H:2 * H, :] = 1.0 - gsig

    lane = lax.broadcasted_iota(i32, (128, 128), 1)
    row = lax.broadcasted_iota(i32, (128, 128), 0)

    def ln_rows(r0, n, src=None, after=None):
        src = xa if src is None else src
        xf = src[pl.ds(r0, n), :].astype(f32)
        if after is not None:
            z = pltpu.bitcast(jnp.concatenate([after] * (n // 8), axis=0), f32)
            xf = jnp.concatenate([xf[:, 0:128] + z, xf[:, 128:]], axis=1)
        xn[_half(r0, n), :] = _pack(_layernorm(xf))

    def ln_block(r0, src=None):
        ln_rows(r0, L, src)

    def pin(w32, ref):
        zero = zero_s[0]
        lk = ref[pl.ds(pl.multiple_of(zero, 8), 8), 0:128] & zero
        head = jnp.concatenate([w32[0:8, 0:128] | lk, w32[0:8, 128:]], axis=1)
        return head if w32.shape[0] == 8 else jnp.concatenate([head, w32[8:]], axis=0)

    CB = 256

    def next_block(s):
        return pl.multiple_of(jnp.minimum(s + 1, NSEG - 1) * L, L)

    def v_cols(s, xb, lo, hi):
        for c0 in range(lo, hi, CB):
            v = jnp.dot(xb, wst[0, :, c0:c0 + CB], preferred_element_type=f32)
            vt[s, c0 // 2:(c0 + CB) // 2, :] = pltpu.bitcast(v.astype(bf16).T, i32)

    def q_cols(s, r0, xb, c0, qmax):
        q = jnp.dot(xb, wst[1, :, c0:c0 + CB], preferred_element_type=f32)
        for j in range(CB // 128):
            g = c0 // 128 + j
            qg = q[:, j * 128:(j + 1) * 128]
            qsc = qg * QSCALE
            qs[g, _half(r0, L), :] = _pack(qsc)
            pq[g, _half(r0, L), :] = _pack(_phi(qg))
            qmax = jnp.maximum(qmax, jnp.max(_fold8(jnp.abs(qsc)), axis=0))
        return qmax

    def k_cols(s, r0, xb, c0, kmax):
        k = jnp.dot(xb, wst[2, :, c0:c0 + CB], preferred_element_type=f32)
        for j in range(CB // 128):
            g = c0 // 128 + j
            kg = k[:, j * 128:(j + 1) * 128]
            ks[g, _half(r0, L), :] = _pack(kg)
            pkg = _phi(kg)
            pk[g, _half(r0, L), :] = _pack(pkg)
            zs[s, g] = jnp.sum(_fold8(pkg), axis=0)
            kmax = jnp.maximum(kmax, jnp.max(_fold8(jnp.abs(kg)), axis=0))
        return kmax

    def proj_first():
        for i in range(4):
            x0_cp[i].wait()
            ln_rows(i * XP, XP, xio)
        for c, lo, hi in zip(wv_cp, (0, QD, 2 * QD), (QD, 2 * QD, D)):
            c.wait()
            v_cols(0, _unpack(xn[0:L // 2, :]), lo, hi)
        w_cp[0].wait()
        qmax = kmax = jnp.zeros((8, 128), f32)
        xb = _unpack(xn[0:L // 2, :])
        for c0 in range(0, D, CB):
            qmax = q_cols(0, 0, xb, c0, qmax)
        w_cp[1].wait()
        x_cp[1].wait()
        xb = _unpack(xn[0:L // 2, :])
        for c0 in range(0, D, CB):
            kmax = k_cols(0, 0, xb, c0, kmax)
        ln_block(L, xio)
        w_cp[2].wait()
        return qmax, kmax

    def proj_block(s, carry, li):
        qmax, kmax = carry
        if li == 0:
            for i in range(2, nx):
                @pl.when(s == i - 1)
                def _():
                    x_cp[i].wait()
        r0 = pl.multiple_of(s * L, L)
        xb = _unpack(xn[_half(r0, L), :])
        v_cols(s, xb, 0, D)
        for c0 in range(0, D, CB):
            qmax = q_cols(s, r0, xb, c0, qmax)
            kmax = k_cols(s, r0, xb, c0, kmax)
        ln_block(next_block(s), xio if li == 0 else xa)
        if li == 0:
            w0 = pl.multiple_of((s - 1) * 168, 8)
            wo[pl.ds(w0, 176), :] = _pack(wst[3, pl.ds(pl.multiple_of(2 * w0, 16), 352), :])
        return qmax, kmax

    def attn_groups(g0, ng, use_max):
        causal = row <= lane
        gs = [g0 + i for i in range(ng)]
        g64 = [pl.multiple_of(g * 64, 64) for g in gs]
        blockdiag = (row >> 5) == (lane >> 5)
        lane16 = lax.broadcasted_iota(i32, (16, 128), 1)
        row16 = lax.broadcasted_iota(i32, (16, 128), 0)
        zmask = (lane16 >> 5) == row16

        def tile(ref, g, s, t):
            return ref[g, (s * L + t * 128) // 2:(s * L + (t + 1) * 128) // 2, :]

        split_diag = SPLITD and not use_max
        lane64 = lax.broadcasted_iota(i32, (64, 128), 1)
        causal64 = lax.broadcasted_iota(i32, (64, 128), 0) <= (lane64 & 63)
        low64 = lane64 < 64
        low8 = lax.broadcasted_iota(i32, (8, 128), 1) < 64

        def qk(gi, s, t, flip, link=None):
            g = gs[gi]
            qt = tile(qs, g, s, t)
            if link is not None:
                qt = jnp.concatenate([qt[0:8] | link, qt[8:]], axis=0)
            qlane = lax.broadcasted_iota(i32, qt.shape, 1)
            qi = [jnp.where((qlane >> 5) == h, qt, 0) for h in range(4)]
            qm = [_unpack(x) for x in qi]
            Sc = [[None] * (t + 1) for _ in range(4)]
            for j in range(t if split_diag else t + 1):
                kk = _unpack(tile(ks, g, s, j))
                for h in range(4):
                    Sc[h][j] = lax.dot_general(kk, qm[h], _NT, preferred_element_type=f32)
            if not split_diag:
                return Sc, None
            kd = tile(ks, g, s, t)
            T1, T2 = [None, None], [None, None]

            def t1(pr):
                w = _unpack(jnp.concatenate([qi[2 * pr][0:32], qi[2 * pr + 1][0:32]], axis=0))
                T1[pr] = lax.dot_general(_unpack(kd[0:32]), w, _NT, preferred_element_type=f32)

            def t2(pr):
                w = _unpack(jnp.concatenate([qi[2 * pr][32:64], qi[2 * pr + 1][32:64]], axis=0))
                T2[pr] = lax.dot_general(_unpack(kd), w, _NT, preferred_element_type=f32)

            for fn, pr in ((t2, 0), (t2, 1), (t1, 0), (t1, 1)) if flip else (
                    (t1, 0), (t1, 1), (t2, 0), (t2, 1)):
                fn(pr)
            return Sc, (T1, T2)

        def tie(x, part):
            if not TIE:
                return x
            n = x.shape[0] - 8
            return jnp.concatenate([x[:n], x[n:] + part * 0.0], axis=0)

        def sm(ScD, t):
            Sc, Dg = ScD
            P = [None] * 4
            Linv = [None] * 4
            l8 = [None] * 4
            for h in range(4):
                sc = list(Sc[h])
                if not split_diag:
                    sc[t] = jnp.where(causal, sc[t], NEG)
                else:
                    sc = sc[:t]
                if use_max:
                    m = sc[0]
                    for j in range(1, t + 1):
                        m = jnp.maximum(m, sc[j])
                    m = jnp.max(m, axis=0, keepdims=True)
                    p = [jnp.exp2(x - m) for x in sc]
                else:
                    p = [jnp.exp2(x) for x in sc]
                P[h] = []
                for x in p:
                    part = jnp.sum(_fold8(x), axis=0)
                    l8[h] = part if l8[h] is None else l8[h] + part
                    P[h].append(tie(x, part).astype(bf16))
            if split_diag:
                for pr in range(2):
                    a, b = 2 * pr, 2 * pr + 1
                    e1 = jnp.exp2(jnp.where(causal64, Dg[0][pr], NEG))
                    e2a = jnp.exp2(Dg[1][pr][0:64])
                    e2b = jnp.exp2(jnp.where(causal64, Dg[1][pr][64:128], NEG))
                    p1 = jnp.sum(_fold8(e1), axis=0)
                    p2 = jnp.sum(_fold8(e2a), axis=0) + jnp.sum(_fold8(e2b), axis=0)
                    la = jnp.where(low8, p1, pltpu.roll(p2, 64, 1))
                    lb = jnp.where(low8, pltpu.roll(p1, 64, 1), p2)
                    l8[a] = la if l8[a] is None else l8[a] + la
                    l8[b] = lb if l8[b] is None else l8[b] + lb
                    e1, e2b = tie(e1, p1), tie(e2b, p2)
                    P[a].append(jnp.concatenate(
                        [jnp.where(low64, e1, pltpu.roll(e2a, 64, 1)),
                         jnp.where(low64, 0.0, pltpu.roll(e2b, 64, 1))], axis=0).astype(bf16))
                    P[b].append(jnp.concatenate(
                        [jnp.where(low64, pltpu.roll(e1, 64, 1), e2a),
                         jnp.where(low64, 0.0, e2b)], axis=0).astype(bf16))
            for h in range(4):
                Linv[h] = 1.0 / jnp.sum(l8[h], axis=0, keepdims=True)
            return P, Linv

        def pv(PL, gi, s, t, lhs_m):
            g = gs[gi]
            P, Linv = PL
            acc = [None] * 4
            for j in range(t + 1):
                for h in range(4):
                    vth = _unpack(vt[s, pl.ds(g64[gi] + 16 * h, 16), j * 128:(j + 1) * 128])
                    o = jnp.dot(vth, P[h][j], preferred_element_type=f32)
                    acc[h] = o if acc[h] is None else acc[h] + o
            if lhs_m is not None:
                pqt = _unpack(tile(pq, g, s, t))
                nd = lax.dot_general(lhs_m, pqt, _NT, preferred_element_type=f32)
            outs = []
            for h in range(4):
                o = acc[h] * (gt[pl.ds(H + g * 4 + h, 1), :] * Linv[h])
                if lhs_m is not None:
                    den = nd[128 + h:129 + h, :] + 1e-6
                    o = o + nd[32 * h:32 * h + 32, :] * (gt[pl.ds(g * 4 + h, 1), :] / den)
                outs.append(o)
            ot = jnp.concatenate(outs, axis=0).astype(bf16)
            o_s[g, (s * L + t * 128) // 2:(s * L + (t + 1) * 128) // 2, :] = (
                pltpu.bitcast(ot.T, i32))
            zero = zero_s[0]
            return o_s[g, pl.ds(pl.multiple_of((s * L + t * 128) // 2 + zero, 8), 8), :] & zero

        def mem_update(gi, s, R):
            g = gs[gi]
            vtg = _unpack(vt[s, pl.ds(g64[gi], 64), :])
            pks = _unpack(pk[g, s * L // 2:(s + 1) * L // 2, :])
            upd = jnp.dot(vtg, pks, preferred_element_type=f32)
            return upd if R is None else R + upd

        def mem_lhs(gi, s, R):
            g = gs[gi]
            mt = jnp.where(blockdiag, R, 0.0)
            z = zs[0, g]
            for s2 in range(1, s):
                z = z + zs[s2, g]
            z = jnp.sum(z, axis=0, keepdims=True)
            zr = jnp.where(zmask, z, 0.0)
            return jnp.concatenate([mt, zr], axis=0).astype(bf16)

        order = [int(c) for c in str(TORD).zfill(4)]
        steps = [(gi, s, t) for gi in range(ng) for s in range(NSEG) for t in order]
        n = len(steps)
        Sc, PL = {}, {}
        R = None
        lhs = {}
        links = {}
        for i in range(n + LAG):
            if i < n:
                Sc[i] = qk(*steps[i], i % 2 == 1,
                           links.get(i - LAG - ODELAY) if ODELAY else None)
                gi, s, t = steps[i]
                if t == order[0] and s == 0:
                    R = None
                    lhs[gi, 0] = None
                if t == order[-1] and s < NSEG - 1:
                    R = mem_update(gi, s, R)
                    lhs[gi, s + 1] = mem_lhs(gi, s + 1, R)
                PL[i] = sm(Sc.pop(i), t)
            if 0 <= i - LAG < n:
                gi, s, t = steps[i - LAG]
                links[i - LAG] = pv(PL.pop(i - LAG), gi, s, t, lhs[gi, s])

    CP, RP = D // ONP, OB // ONP

    def o_lhs(r0):
        return jnp.concatenate([_unpack(o_s[g, _half(r0, OB), :]) for g in range(G)], axis=1)

    def o_epilogue(refs, r0, out, last):
        xa_, x1_, y_, xo_ = refs
        res = xa_[r0:r0 + RP, :] if last else xo_[r0:r0 + RP, :].astype(f32)
        x1 = _r(res + _r(out))
        x1_[r0:r0 + RP, :] = x1.astype(bf16)
        y = _layernorm(x1)
        y_[r0:r0 + RP, :] = y.astype(bf16)
        if last:
            xo_[r0:r0 + RP, :] = (x1 + y).astype(bf16)
        else:
            xa_[r0:r0 + RP, :] = _r(x1 + y)
        wr = wr_ref[...].astype(f32).reshape(1, D)
        return _r(jnp.sum(y * wr, axis=1, keepdims=True))

    def o_refs(r0, n):
        return [xa.at[pl.ds(r0, n)], x1_s.at[pl.ds(r0, n)], y_s.at[pl.ds(r0, n)],
                xio.at[pl.ds(r0, n)]]

    def o_step(refs, k, blk, src, dst, last):
        if dst is not None:
            ob = o_lhs((blk + 1) * OB)
        rcols = []
        for p in range(ONP):
            if dst is not None:
                dst[:, p * CP:(p + 1) * CP] = jnp.dot(
                    ob, _unpack(wo[:, p * CP:(p + 1) * CP]), preferred_element_type=f32)
            rcols.append(o_epilogue(refs, k * OB + p * RP, src[p * RP:(p + 1) * RP, :], last))
        rb = jnp.broadcast_to(jnp.concatenate(rcols, axis=0), (OB, 128))
        lane_ob = lax.broadcasted_iota(i32, (OB, 128), 1)
        row_ob = lax.broadcasted_iota(i32, (OB, 128), 0)
        r_s[pl.ds(blk, 1), :] = jnp.max(jnp.where(row_ob == lane_ob, rb, -jnp.inf),
                                        axis=0, keepdims=True)

    def o_phase(last):
        nb = S // OB
        oc[0] = jnp.dot(o_lhs(0), _unpack(wo[...]), preferred_element_type=f32)
        nloop = (nb - 2) // OSTEP
        assert OSTEP % ONB == 0

        def out_rows(r0, n):
            return pltpu.make_async_copy(xio.at[pl.ds(r0, n)], out_hbm.at[0, pl.ds(r0, n)],
                                         sems.at[2])

        def body(i, carry):
            if last:
                @pl.when(i > 0)
                def _():
                    out_rows(pl.multiple_of((i - 1) * OSTEP * OB, OSTEP * OB),
                             OSTEP * OB).start()

            refs = o_refs(pl.multiple_of(i * OSTEP * OB, OSTEP * OB), OSTEP * OB)
            for k in range(OSTEP):
                o_step(refs, k, i * OSTEP + k, oc.at[k % ONB], oc.at[(k + 1) % ONB], last)
            return carry

        lax.fori_loop(0, nloop, body, 0)
        b0 = nloop * OSTEP
        if last:
            out_rows((b0 - OSTEP) * OB, OSTEP * OB).start()
        refs = o_refs(b0 * OB, (nb - b0) * OB)
        for k in range(nb - b0):
            o_step(refs, k, b0 + k, oc.at[k % ONB],
                   oc.at[(k + 1) % ONB] if b0 + k + 1 < nb else None, last)
        if last:
            out_rows(b0 * OB, (nb - b0) * OB).start()

    out_cp = pltpu.make_async_copy(xio, out_hbm.at[0], sems.at[2])

    def moe_phase(last):
        r_all = r_s[...]
        ridx = (lax.broadcasted_iota(i32, r_all.shape, 0) * OB
                + lax.broadcasted_iota(i32, r_all.shape, 1)).astype(f32)

        def red(fn, x):
            return fn(fn(x, axis=0, keepdims=True), axis=1, keepdims=True)

        m1 = red(jnp.max, r_all)
        i1f = red(jnp.min, jnp.where(r_all == m1, ridx, 1e9))
        r2 = jnp.where(ridx == i1f, -jnp.inf, r_all)
        m2 = red(jnp.max, r2)
        i2f = red(jnp.min, jnp.where((r2 == m2) & (ridx != i1f), ridx, 1e9))
        idx = [jnp.clip(v[0, 0].astype(i32), 0, S - 1) for v in (i1f, i2f)]
        base = [pl.multiple_of((ix >> 4) << 4, 16) for ix in idx]
        off = [ix & 15 for ix in idx]
        row16 = lax.broadcasted_iota(i32, (16, D), 0)

        def gather(ref):
            res = None
            for kk in range(2):
                blk = ref[pl.ds(base[kk], 16), :].astype(f32)
                one = jnp.sum(jnp.where(row16 == off[kk], blk, 0.0), axis=0, keepdims=True)
                part = jnp.where(row16 == kk, one, 0.0)
                res = part if res is None else res + part
            return res

        ysel = gather(y_s)
        x1sel = gather(x1_s)
        xsel32 = _pack(ysel)
        yf = None
        after = None
        nch = F // FCH
        rp = L // NLN
        for ci, c0 in enumerate(range(0, F, FCH)):
            if not last and ci % LNE == 0 and ci // LNE < NLN:
                ln_rows(ci // LNE * rp, rp, None, after)
                xsel = _unpack(pin(xsel32, xn))
            else:
                xsel = _unpack(xsel32)
            gte = _r(jnp.dot(xsel, wg[:, c0:c0 + FCH], preferred_element_type=f32))
            after = pltpu.bitcast(gte[0:8, 0:128], i32) & zero_s[0]
            up = _r(jnp.dot(xsel, wu[:, c0:c0 + FCH], preferred_element_type=f32))
            act = _r(gte * jax.nn.sigmoid(gte))
            hcol = (act * up).astype(bf16)
            part = jnp.dot(hcol, wd[c0:c0 + FCH, :], preferred_element_type=f32)
            yf = part if yf is None else yf + part
        rsel = _r(jax.nn.sigmoid(jnp.where(row16 == 0, m1, m2)))
        upd = _r(_r(yf) * rsel)
        x2 = _r(x1sel + _r(ysel + upd))
        rows2 = [jnp.sum(jnp.where(row16 == kk, x2, 0.0), axis=0, keepdims=True)
                 for kk in range(2)]
        if not last:
            xn2 = _layernorm(x2)
            for kk in range(2):
                xa[pl.ds(idx[kk], 1), :] = rows2[kk]
                one = jnp.sum(jnp.where(row16 == kk, xn2, 0.0), axis=0, keepdims=True)
                blk = _unpack(xn[_half(base[kk], 16), :]).astype(f32)
                xn[_half(base[kk], 16), :] = _pack(jnp.where(row16 == off[kk], one, blk))
        else:
            out_cp.wait()
            for kk in range(2):
                blk = xio[pl.ds(base[kk], 16), :].astype(f32)
                xio[pl.ds(base[kk], 16), :] = jnp.where(
                    row16 == off[kk], rows2[kk], blk).astype(bf16)
            cp0 = pltpu.make_async_copy(xio.at[pl.ds(base[0], 16), :],
                                        out_hbm.at[0, pl.ds(base[0], 16), :], sems.at[0])
            cp1 = pltpu.make_async_copy(xio.at[pl.ds(base[1], 16), :],
                                        out_hbm.at[0, pl.ds(base[1], 16), :], sems.at[1])
            cp0.start()

            @pl.when(base[0] != base[1])
            def _():
                cp1.start()
                cp1.wait()

            cp0.wait()

    if _ONLY:
        for c in x0_cp + x_cp[1:] + wv_cp + w_cp:
            c.wait()
        dict(O0=lambda: o_phase(False), O1=lambda: o_phase(True),
             B0=lambda: moe_phase(False),
             A=lambda: lax.fori_loop(0, G // AG, lambda i, c: (attn_groups(i * AG, AG, False), c)[1], 0))[_ONLY]()
        out_cp.start()
        out_cp.wait()
        return

    for li in range(2):
        last = li == 1
        if li == 0:
            qmax, kmax = lax.fori_loop(1, NSEG, lambda s, c: proj_block(s, c, 0), proj_first())
        else:
            z8 = jnp.zeros((8, 128), f32)
            qmax, kmax = lax.fori_loop(0, NSEG, lambda s, c: proj_block(s, c, 1), (z8, z8))
        bound = DH * jnp.max(qmax) * jnp.max(kmax)
        safe = bound <= SAFE_BOUND

        @pl.when(safe)
        def _():
            lax.fori_loop(0, G // AG, lambda i, c: (attn_groups(i * AG, AG, False), c)[1], 0)

        @pl.when(jnp.logical_not(safe))
        def _():
            lax.fori_loop(0, G, lambda g, c: (attn_groups(g, 1, True), c)[1], 0)

        o_phase(last)
        if li == 0:
            for c in w_cp[3:]:
                c.wait()
        moe_phase(last)


@jax.jit
def pallas_interleave_layers__memory_aug_infini_attn__moe_arch_mod__prompt_kernel(
    A_x: jax.Array,
    A_wq: jax.Array,
    A_wk: jax.Array,
    A_wv: jax.Array,
    A_wo: jax.Array,
    A_beta: jax.Array,
    B_x: jax.Array,
    B_w_r: jax.Array,
    B_w_gate: jax.Array,
    B_w_up: jax.Array,
    B_w_down: jax.Array,
):
    del B_x
    any_spec = pl.BlockSpec(memory_space=pl.ANY)
    vm = pltpu.VMEM
    return pl.pallas_call(
        _kernel,
        out_shape=jax.ShapeDtypeStruct((1, S, D), bf16),
        in_specs=[pl.BlockSpec(memory_space=pltpu.SMEM),
                  pl.BlockSpec(memory_space=vm), pl.BlockSpec(memory_space=vm)] + [any_spec] * 8,
        out_specs=any_spec,
        scratch_shapes=[
            vm((S, D), bf16),
            vm((4, D, D), bf16),
            vm((S, D), f32),
            vm((S // 2, D), i32),
            vm((D // 2, D), i32),
            vm((G, S // 2, 128), i32), vm((G, S // 2, 128), i32),
            vm((G, S // 2, 128), i32), vm((G, S // 2, 128), i32),
            vm((NSEG, D // 2, L), i32),
            vm((G, S // 2, 128), i32),
            vm((S, D), bf16), vm((S, D), bf16),
            vm((NSEG, G, 8, 128), f32),
            vm((2 * H, 128), f32),
            vm((S // OB, 128), f32),
            vm((ONB, OB, D), f32),
            vm((D, F), bf16), vm((D, F), bf16), vm((F, D), bf16),
            pltpu.SemaphoreType.DMA((16,)),
        ],
        compiler_params=pltpu.CompilerParams(vmem_limit_bytes=120 * 1024 * 1024, flags=_FLAGS),
    )(np.zeros((1,), np.int32), A_beta, B_w_r, A_x, A_wq, A_wk, A_wv, A_wo, B_w_gate, B_w_up, B_w_down)
```

```python
import math

import jax
import jax.numpy as jnp
import numpy as np
from jax import lax
import jax.experimental.pallas as pl
import jax.experimental.pallas.tpu as pltpu

S = 2048
D = 1024
H = 32
DH = D // H
NSEG = 4
L = S // NSEG
G = 8
F = 3584
OB = 32
OSTEP = 30
ONP = 2
NLN = 4
LNE = 1
ODELAY = 0
DTIE = 0
MEMPOS = 0
ROT = 2
TORD = 1302
ONB = 5
AG = 2
LAG = 4
FCH = 896

bf16 = jnp.bfloat16
f32 = jnp.float32
i32 = jnp.int32

QSCALE = (DH ** -0.5) * math.log2(math.e)
SAFE_BOUND = 24.0
NEG = -1e30
EPS_BF16 = 1.0013580322265625e-05

_NT = (((1,), (1,)), ((), ()))
_ONLY = None
_FLAGS = None


def _r(x):
    return x.astype(bf16).astype(f32)


def _pack(x):
    return pltpu.bitcast(x.astype(bf16), i32)


def _unpack(w):
    return pltpu.bitcast(w, bf16)


def _layernorm(xf):
    mean = jnp.sum(xf, axis=1, keepdims=True) * (1.0 / D)
    c = xf - mean
    var = jnp.sum(c * c, axis=1, keepdims=True) * (1.0 / D)
    d = _r(xf - _r(mean))
    s = _r(jnp.sqrt(_r(_r(var) + EPS_BF16)))
    return _r(d * (1.0 / s))


def _phi(t):
    return jnp.where(t > 0, t + 1.0, jnp.exp(t))


def _head_lanes(qi, h):
    lane = lax.broadcasted_iota(i32, qi.shape, 1)
    return _unpack(jnp.where((lane >> 5) == h, qi, 0))


def _fold8(x):
    return x.reshape(x.shape[0] // 8, 8, x.shape[1])


def _half(i, n):
    return pl.ds(i // 2 if isinstance(i, int) else pl.multiple_of(i // 2, n // 2), n // 2)


def _kernel(zero_s, beta_ref, wr_ref,
            x_hbm, wq_hbm, wk_hbm, wv_hbm, wo_hbm, wg_hbm, wu_hbm, wd_hbm,
            out_hbm,
            xio, wst, xa, xn, wo, qs, pq, ks, pk, vt, o_s, y_s, x1_s,
            zs, gt, r_s, oc, wg, wu, wd, sems):
    nx = NSEG
    XP = L // 4
    QD = D // 4

    def cp(src, dst, i):
        return pltpu.make_async_copy(src, dst, sems.at[i])

    def wcols(lo, n):
        return wv_hbm.at[:, pl.ds(lo, n)], wst.at[0, :, pl.ds(lo, n)]

    x0_cp = [cp(x_hbm.at[0, pl.ds(i * XP, XP), :], xio.at[pl.ds(i * XP, XP), :], i)
             for i in range(4)]
    x_cp = [None] + [cp(x_hbm.at[0, pl.ds(i * L, L), :], xio.at[pl.ds(i * L, L), :], 3 + i)
                     for i in range(1, nx)]
    wv_cp = [cp(*wcols(0, QD), 7), cp(*wcols(QD, QD), 8), cp(*wcols(2 * QD, 2 * QD), 9)]
    w_cp = [cp(src, dst, 10 + i) for i, (src, dst) in
            enumerate([(wq_hbm, wst.at[1]), (wk_hbm, wst.at[2]), (wo_hbm, wst.at[3]),
                       (wg_hbm, wg), (wu_hbm, wu), (wd_hbm, wd)])]
    for c in x0_cp + wv_cp + w_cp[:2] + x_cp[1:2] + w_cp[2:3] + x_cp[2:] + w_cp[3:]:
        c.start()

    b = jnp.broadcast_to(beta_ref[...].astype(f32).reshape(1, H), (H, H))
    rr = lax.broadcasted_iota(i32, (H, H), 0)
    cc = lax.broadcasted_iota(i32, (H, H), 1)
    bcol = jnp.sum(jnp.where(rr == cc, b, 0.0), axis=1, keepdims=True)
    gsig = _r(jax.nn.sigmoid(jnp.broadcast_to(bcol, (H, 128))))
    gt[0:H, :] = gsig
    gt[H:2 * H, :] = 1.0 - gsig

    lane = lax.broadcasted_iota(i32, (128, 128), 1)
    row = lax.broadcasted_iota(i32, (128, 128), 0)

    def ln_rows(r0, n, src=None, after=None):
        src = xa if src is None else src
        xf = src[pl.ds(r0, n), :].astype(f32)
        if after is not None:
            z = pltpu.bitcast(jnp.concatenate([after] * (n // 8), axis=0), f32)
            xf = jnp.concatenate([xf[:, 0:128] + z, xf[:, 128:]], axis=1)
        xn[_half(r0, n), :] = _pack(_layernorm(xf))

    def ln_block(r0, src=None):
        ln_rows(r0, L, src)

    def pin(w32, ref):
        zero = zero_s[0]
        lk = ref[pl.ds(pl.multiple_of(zero, 8), 8), 0:128] & zero
        head = jnp.concatenate([w32[0:8, 0:128] | lk, w32[0:8, 128:]], axis=1)
        return head if w32.shape[0] == 8 else jnp.concatenate([head, w32[8:]], axis=0)

    CB = 256

    def next_block(s):
        return pl.multiple_of(jnp.minimum(s + 1, NSEG - 1) * L, L)

    def v_cols(s, xb, lo, hi):
        for c0 in range(lo, hi, CB):
            v = jnp.dot(xb, wst[0, :, c0:c0 + CB], preferred_element_type=f32)
            vt[s, c0 // 2:(c0 + CB) // 2, :] = pltpu.bitcast(v.astype(bf16).T, i32)

    def q_cols(s, r0, xb, c0, qmax):
        q = jnp.dot(xb, wst[1, :, c0:c0 + CB], preferred_element_type=f32)
        for j in range(CB // 128):
            g = c0 // 128 + j
            qg = q[:, j * 128:(j + 1) * 128]
            qsc = qg * QSCALE
            qs[g, _half(r0, L), :] = _pack(qsc)
            pq[g, _half(r0, L), :] = _pack(_phi(qg))
            qmax = jnp.maximum(qmax, jnp.max(_fold8(jnp.abs(qsc)), axis=0))
        return qmax

    def k_cols(s, r0, xb, c0, kmax):
        k = jnp.dot(xb, wst[2, :, c0:c0 + CB], preferred_element_type=f32)
        for j in range(CB // 128):
            g = c0 // 128 + j
            kg = k[:, j * 128:(j + 1) * 128]
            ks[g, _half(r0, L), :] = _pack(kg)
            pkg = _phi(kg)
            pk[g, _half(r0, L), :] = _pack(pkg)
            zs[s, g] = jnp.sum(_fold8(pkg), axis=0)
            kmax = jnp.maximum(kmax, jnp.max(_fold8(jnp.abs(kg)), axis=0))
        return kmax

    def proj_first():
        for i in range(4):
            x0_cp[i].wait()
            ln_rows(i * XP, XP, xio)
        for c, lo, hi in zip(wv_cp, (0, QD, 2 * QD), (QD, 2 * QD, D)):
            c.wait()
            v_cols(0, _unpack(xn[0:L // 2, :]), lo, hi)
        w_cp[0].wait()
        qmax = kmax = jnp.zeros((8, 128), f32)
        xb = _unpack(xn[0:L // 2, :])
        for c0 in range(0, D, CB):
            qmax = q_cols(0, 0, xb, c0, qmax)
        w_cp[1].wait()
        x_cp[1].wait()
        xb = _unpack(xn[0:L // 2, :])
        for c0 in range(0, D, CB):
            kmax = k_cols(0, 0, xb, c0, kmax)
        ln_block(L, xio)
        w_cp[2].wait()
        return qmax, kmax

    def proj_block(s, carry, li):
        qmax, kmax = carry
        if li == 0:
            for i in range(2, nx):
                @pl.when(s == i - 1)
                def _():
                    x_cp[i].wait()
        r0 = pl.multiple_of(s * L, L)
        xb = _unpack(xn[_half(r0, L), :])
        v_cols(s, xb, 0, D)
        for c0 in range(0, D, CB):
            qmax = q_cols(s, r0, xb, c0, qmax)
            kmax = k_cols(s, r0, xb, c0, kmax)
        ln_block(next_block(s), xio if li == 0 else xa)
        if li == 0:
            w0 = pl.multiple_of((s - 1) * 168, 8)
            wo[pl.ds(w0, 176), :] = _pack(wst[3, pl.ds(pl.multiple_of(2 * w0, 16), 352), :])
        return qmax, kmax

    def attn_groups(g0, ng, use_max):
        causal = row <= lane
        gs = [g0 + i for i in range(ng)]
        g64 = [pl.multiple_of(g * 64, 64) for g in gs]
        blockdiag = (row >> 5) == (lane >> 5)
        lane16 = lax.broadcasted_iota(i32, (16, 128), 1)
        row16 = lax.broadcasted_iota(i32, (16, 128), 0)
        zmask = (lane16 >> 5) == row16

        def tile(ref, g, s, t):
            return ref[g, (s * L + t * 128) // 2:(s * L + (t + 1) * 128) // 2, :]

        split_diag = not use_max
        causal32 = (lax.broadcasted_iota(i32, (32, 128), 0)
                    <= (lax.broadcasted_iota(i32, (32, 128), 1) & 31))

        def block_transpose(src):
            rows = next(x for x in src if x is not None).shape[0]
            ln = lax.broadcasted_iota(i32, (rows, 128), 1)

            def pick(lo_mask, a, b):
                if a is None and b is None:
                    return None
                return jnp.where(lo_mask, 0.0 if a is None else a, 0.0 if b is None else b)

            def rot(x, n):
                return None if x is None else pltpu.roll(x, n, 1)

            x = [None] * 4
            for i in range(2):
                a, c = src[i], src[i + 2]
                x[i] = pick(ln < 64, a, rot(c, 64))
                x[i + 2] = pick(ln < 64, rot(a, 64), c)
            y = [None] * 4
            for i in (0, 2):
                a, c = x[i], x[i + 1]
                y[i] = pick((ln & 32) == 0, a, rot(c, 32))
                y[i + 1] = pick((ln & 32) == 0, rot(a, 96), c)
            return [jnp.zeros((rows, 128), f32) if v is None else v for v in y]

        def qk(gi, s, t, step, link=None):
            g = gs[gi]
            qt = tile(qs, g, s, t)
            if link is not None:
                qt = jnp.concatenate([qt[0:8] | link, qt[8:]], axis=0)
            qlane = lax.broadcasted_iota(i32, qt.shape, 1)
            qi = [jnp.where((qlane >> 5) == h, qt, 0) for h in range(4)]
            qm = [_unpack(x) for x in qi]
            Sc = [[None] * (t + 1) for _ in range(4)]
            for j in range(t if split_diag else t + 1):
                kk = _unpack(tile(ks, g, s, j))
                for h in range(4):
                    Sc[h][j] = lax.dot_general(kk, qm[h], _NT, preferred_element_type=f32)
            if not split_diag:
                return Sc, None
            kd = tile(ks, g, s, t)
            T = [None] * 4
            for u in [((3 - n if ROT & 1 else n) + (step if ROT & 2 else -step if ROT & 4 else 0)) % 4
                      for n in range(4)]:
                w = _unpack(jnp.concatenate([x[16 * u:16 * u + 16] for x in qi], axis=0))
                T[u] = lax.dot_general(_unpack(kd[0:16 * (u + 1)]), w, _NT,
                                       preferred_element_type=f32)
            return Sc, T

        def tie(x, part):
            n = x.shape[0] - 8
            return jnp.concatenate([x[:n], x[n:] + part * 0.0], axis=0)

        def sm(ScD, t):
            Sc, T = ScD
            P = [None] * 4
            Linv = [None] * 4
            l8 = [None] * 4
            for h in range(4):
                sc = list(Sc[h])
                if not split_diag:
                    sc[t] = jnp.where(causal, sc[t], NEG)
                else:
                    sc = sc[:t]
                if use_max:
                    m = sc[0]
                    for j in range(1, t + 1):
                        m = jnp.maximum(m, sc[j])
                    m = jnp.max(m, axis=0, keepdims=True)
                    p = [jnp.exp2(x - m) for x in sc]
                else:
                    p = [jnp.exp2(x) for x in sc]
                P[h] = []
                for x in p:
                    part = jnp.sum(_fold8(x), axis=0)
                    l8[h] = part if l8[h] is None else l8[h] + part
                    P[h].append(tie(x, part).astype(bf16))
            if split_diag:
                E, ps = [], []
                for u in range(4):
                    e = jnp.exp2(jnp.where(causal32, T[u][32 * u:], NEG))
                    if u:
                        e = jnp.concatenate([jnp.exp2(T[u][:32 * u]), e], axis=0)
                    part = jnp.sum(_fold8(e), axis=0)
                    ps.append(part)
                    E.append(tie(e, part) if DTIE else e)
                lh = block_transpose(ps)
                rows = [block_transpose([E[u][32 * r:32 * r + 32] if u >= r else None
                                         for u in range(4)]) for r in range(4)]
                for h in range(4):
                    l8[h] = lh[h] if l8[h] is None else l8[h] + lh[h]
                    P[h].append(jnp.concatenate([rows[r][h] for r in range(4)],
                                                axis=0).astype(bf16))
            for h in range(4):
                Linv[h] = 1.0 / jnp.sum(l8[h], axis=0, keepdims=True)
            return P, Linv

        def pv(PL, gi, s, t, lhs_m):
            g = gs[gi]
            P, Linv = PL
            acc = [None] * 4
            for j in range(t + 1):
                for h in range(4):
                    vth = _unpack(vt[s, pl.ds(g64[gi] + 16 * h, 16), j * 128:(j + 1) * 128])
                    o = jnp.dot(vth, P[h][j], preferred_element_type=f32)
                    acc[h] = o if acc[h] is None else acc[h] + o
            if lhs_m is not None:
                pqt = _unpack(tile(pq, g, s, t))
                nd = lax.dot_general(lhs_m, pqt, _NT, preferred_element_type=f32)
            outs = []
            for h in range(4):
                o = acc[h] * (gt[pl.ds(H + g * 4 + h, 1), :] * Linv[h])
                if lhs_m is not None:
                    den = nd[128 + h:129 + h, :] + 1e-6
                    o = o + nd[32 * h:32 * h + 32, :] * (gt[pl.ds(g * 4 + h, 1), :] / den)
                outs.append(o)
            ot = jnp.concatenate(outs, axis=0).astype(bf16)
            o_s[g, (s * L + t * 128) // 2:(s * L + (t + 1) * 128) // 2, :] = (
                pltpu.bitcast(ot.T, i32))
            zero = zero_s[0]
            return o_s[g, pl.ds(pl.multiple_of((s * L + t * 128) // 2 + zero, 8), 8), :] & zero

        def mem_update(gi, s, R):
            g = gs[gi]
            vtg = _unpack(vt[s, pl.ds(g64[gi], 64), :])
            pks = _unpack(pk[g, s * L // 2:(s + 1) * L // 2, :])
            upd = jnp.dot(vtg, pks, preferred_element_type=f32)
            return upd if R is None else R + upd

        def mem_lhs(gi, s, R):
            g = gs[gi]
            mt = jnp.where(blockdiag, R, 0.0)
            z = zs[0, g]
            for s2 in range(1, s):
                z = z + zs[s2, g]
            z = jnp.sum(z, axis=0, keepdims=True)
            zr = jnp.where(zmask, z, 0.0)
            return jnp.concatenate([mt, zr], axis=0).astype(bf16)

        order = [int(c) for c in str(TORD).zfill(4)]
        steps = [(gi, s, t) for gi in range(ng) for s in range(NSEG) for t in order]
        n = len(steps)
        Sc, PL = {}, {}
        R = None
        lhs = {}
        links = {}
        for i in range(n + LAG):
            if i < n:
                Sc[i] = qk(*steps[i], i,
                           links.get(i - LAG - ODELAY) if ODELAY else None)
                gi, s, t = steps[i]
                if t == order[0] and s == 0:
                    R = None
                    lhs[gi, 0] = None
                if t == order[MEMPOS] and s < NSEG - 1:
                    R = mem_update(gi, s, R)
                    lhs[gi, s + 1] = mem_lhs(gi, s + 1, R)
                PL[i] = sm(Sc.pop(i), t)
            if 0 <= i - LAG < n:
                gi, s, t = steps[i - LAG]
                links[i - LAG] = pv(PL.pop(i - LAG), gi, s, t, lhs[gi, s])

    CP, RP = D // ONP, OB // ONP

    def o_lhs(r0):
        return jnp.concatenate([_unpack(o_s[g, _half(r0, OB), :]) for g in range(G)], axis=1)

    def o_epilogue(refs, r0, out, last):
        xa_, x1_, y_, xo_ = refs
        res = xa_[r0:r0 + RP, :] if last else xo_[r0:r0 + RP, :].astype(f32)
        x1 = _r(res + _r(out))
        x1_[r0:r0 + RP, :] = x1.astype(bf16)
        y = _layernorm(x1)
        y_[r0:r0 + RP, :] = y.astype(bf16)
        if last:
            xo_[r0:r0 + RP, :] = (x1 + y).astype(bf16)
        else:
            xa_[r0:r0 + RP, :] = _r(x1 + y)
        wr = wr_ref[...].astype(f32).reshape(1, D)
        return _r(jnp.sum(y * wr, axis=1, keepdims=True))

    def o_refs(r0, n):
        return [xa.at[pl.ds(r0, n)], x1_s.at[pl.ds(r0, n)], y_s.at[pl.ds(r0, n)],
                xio.at[pl.ds(r0, n)]]

    def o_step(refs, k, blk, src, dst, last):
        if dst is not None:
            ob = o_lhs((blk + 1) * OB)
        rcols = []
        for p in range(ONP):
            if dst is not None:
                dst[:, p * CP:(p + 1) * CP] = jnp.dot(
                    ob, _unpack(wo[:, p * CP:(p + 1) * CP]), preferred_element_type=f32)
            rcols.append(o_epilogue(refs, k * OB + p * RP, src[p * RP:(p + 1) * RP, :], last))
        rb = jnp.broadcast_to(jnp.concatenate(rcols, axis=0), (OB, 128))
        lane_ob = lax.broadcasted_iota(i32, (OB, 128), 1)
        row_ob = lax.broadcasted_iota(i32, (OB, 128), 0)
        r_s[pl.ds(blk, 1), :] = jnp.max(jnp.where(row_ob == lane_ob, rb, -jnp.inf),
                                        axis=0, keepdims=True)

    def o_phase(last):
        nb = S // OB
        oc[0] = jnp.dot(o_lhs(0), _unpack(wo[...]), preferred_element_type=f32)
        nloop = (nb - 2) // OSTEP
        assert OSTEP % ONB == 0

        def out_rows(r0, n):
            return pltpu.make_async_copy(xio.at[pl.ds(r0, n)], out_hbm.at[0, pl.ds(r0, n)],
                                         sems.at[2])

        def body(i, carry):
            if last:
                @pl.when(i > 0)
                def _():
                    out_rows(pl.multiple_of((i - 1) * OSTEP * OB, OSTEP * OB),
                             OSTEP * OB).start()

            refs = o_refs(pl.multiple_of(i * OSTEP * OB, OSTEP * OB), OSTEP * OB)
            for k in range(OSTEP):
                o_step(refs, k, i * OSTEP + k, oc.at[k % ONB], oc.at[(k + 1) % ONB], last)
            return carry

        lax.fori_loop(0, nloop, body, 0)
        b0 = nloop * OSTEP
        if last:
            out_rows((b0 - OSTEP) * OB, OSTEP * OB).start()
        refs = o_refs(b0 * OB, (nb - b0) * OB)
        for k in range(nb - b0):
            o_step(refs, k, b0 + k, oc.at[k % ONB],
                   oc.at[(k + 1) % ONB] if b0 + k + 1 < nb else None, last)
        if last:
            out_rows(b0 * OB, (nb - b0) * OB).start()

    out_cp = pltpu.make_async_copy(xio, out_hbm.at[0], sems.at[2])

    def moe_phase(last):
        r_all = r_s[...]
        ridx = (lax.broadcasted_iota(i32, r_all.shape, 0) * OB
                + lax.broadcasted_iota(i32, r_all.shape, 1)).astype(f32)

        def red(fn, x):
            return fn(fn(x, axis=0, keepdims=True), axis=1, keepdims=True)

        m1 = red(jnp.max, r_all)
        i1f = red(jnp.min, jnp.where(r_all == m1, ridx, 1e9))
        r2 = jnp.where(ridx == i1f, -jnp.inf, r_all)
        m2 = red(jnp.max, r2)
        i2f = red(jnp.min, jnp.where((r2 == m2) & (ridx != i1f), ridx, 1e9))
        idx = [jnp.clip(v[0, 0].astype(i32), 0, S - 1) for v in (i1f, i2f)]
        base = [pl.multiple_of((ix >> 4) << 4, 16) for ix in idx]
        off = [ix & 15 for ix in idx]
        row16 = lax.broadcasted_iota(i32, (16, D), 0)

        def gather(ref):
            res = None
            for kk in range(2):
                blk = ref[pl.ds(base[kk], 16), :].astype(f32)
                one = jnp.sum(jnp.where(row16 == off[kk], blk, 0.0), axis=0, keepdims=True)
                part = jnp.where(row16 == kk, one, 0.0)
                res = part if res is None else res + part
            return res

        ysel = gather(y_s)
        x1sel = gather(x1_s)
        xsel32 = _pack(ysel)
        yf = None
        after = None
        nch = F // FCH
        rp = L // NLN
        for ci, c0 in enumerate(range(0, F, FCH)):
            if not last and ci % LNE == 0 and ci // LNE < NLN:
                ln_rows(ci // LNE * rp, rp, None, after)
                xsel = _unpack(pin(xsel32, xn))
            else:
                xsel = _unpack(xsel32)
            gte = _r(jnp.dot(xsel, wg[:, c0:c0 + FCH], preferred_element_type=f32))
            after = pltpu.bitcast(gte[0:8, 0:128], i32) & zero_s[0]
            up = _r(jnp.dot(xsel, wu[:, c0:c0 + FCH], preferred_element_type=f32))
            act = _r(gte * jax.nn.sigmoid(gte))
            hcol = (act * up).astype(bf16)
            part = jnp.dot(hcol, wd[c0:c0 + FCH, :], preferred_element_type=f32)
            yf = part if yf is None else yf + part
        rsel = _r(jax.nn.sigmoid(jnp.where(row16 == 0, m1, m2)))
        upd = _r(_r(yf) * rsel)
        x2 = _r(x1sel + _r(ysel + upd))
        rows2 = [jnp.sum(jnp.where(row16 == kk, x2, 0.0), axis=0, keepdims=True)
                 for kk in range(2)]
        if not last:
            xn2 = _layernorm(x2)
            for kk in range(2):
                xa[pl.ds(idx[kk], 1), :] = rows2[kk]
                one = jnp.sum(jnp.where(row16 == kk, xn2, 0.0), axis=0, keepdims=True)
                blk = _unpack(xn[_half(base[kk], 16), :]).astype(f32)
                xn[_half(base[kk], 16), :] = _pack(jnp.where(row16 == off[kk], one, blk))
        else:
            out_cp.wait()
            for kk in range(2):
                blk = xio[pl.ds(base[kk], 16), :].astype(f32)
                xio[pl.ds(base[kk], 16), :] = jnp.where(
                    row16 == off[kk], rows2[kk], blk).astype(bf16)
            cp0 = pltpu.make_async_copy(xio.at[pl.ds(base[0], 16), :],
                                        out_hbm.at[0, pl.ds(base[0], 16), :], sems.at[0])
            cp1 = pltpu.make_async_copy(xio.at[pl.ds(base[1], 16), :],
                                        out_hbm.at[0, pl.ds(base[1], 16), :], sems.at[1])
            cp0.start()

            @pl.when(base[0] != base[1])
            def _():
                cp1.start()
                cp1.wait()

            cp0.wait()

    if _ONLY:
        for c in x0_cp + x_cp[1:] + wv_cp + w_cp:
            c.wait()
        dict(O0=lambda: o_phase(False), O1=lambda: o_phase(True),
             B0=lambda: moe_phase(False),
             A=lambda: lax.fori_loop(0, G // AG, lambda i, c: (attn_groups(i * AG, AG, False), c)[1], 0))[_ONLY]()
        out_cp.start()
        out_cp.wait()
        return

    for li in range(2):
        last = li == 1
        if li == 0:
            qmax, kmax = lax.fori_loop(1, NSEG, lambda s, c: proj_block(s, c, 0), proj_first())
        else:
            z8 = jnp.zeros((8, 128), f32)
            qmax, kmax = lax.fori_loop(0, NSEG, lambda s, c: proj_block(s, c, 1), (z8, z8))
        bound = DH * jnp.max(qmax) * jnp.max(kmax)
        safe = bound <= SAFE_BOUND

        @pl.when(safe)
        def _():
            lax.fori_loop(0, G // AG, lambda i, c: (attn_groups(i * AG, AG, False), c)[1], 0)

        @pl.when(jnp.logical_not(safe))
        def _():
            lax.fori_loop(0, G, lambda g, c: (attn_groups(g, 1, True), c)[1], 0)

        o_phase(last)
        if li == 0:
            for c in w_cp[3:]:
                c.wait()
        moe_phase(last)


@jax.jit
def pallas_interleave_layers__memory_aug_infini_attn__moe_arch_mod__prompt_kernel(
    A_x: jax.Array,
    A_wq: jax.Array,
    A_wk: jax.Array,
    A_wv: jax.Array,
    A_wo: jax.Array,
    A_beta: jax.Array,
    B_x: jax.Array,
    B_w_r: jax.Array,
    B_w_gate: jax.Array,
    B_w_up: jax.Array,
    B_w_down: jax.Array,
):
    del B_x
    any_spec = pl.BlockSpec(memory_space=pl.ANY)
    vm = pltpu.VMEM
    return pl.pallas_call(
        _kernel,
        out_shape=jax.ShapeDtypeStruct((1, S, D), bf16),
        in_specs=[pl.BlockSpec(memory_space=pltpu.SMEM),
                  pl.BlockSpec(memory_space=vm), pl.BlockSpec(memory_space=vm)] + [any_spec] * 8,
        out_specs=any_spec,
        scratch_shapes=[
            vm((S, D), bf16),
            vm((4, D, D), bf16),
            vm((S, D), f32),
            vm((S // 2, D), i32),
            vm((D // 2, D), i32),
            vm((G, S // 2, 128), i32), vm((G, S // 2, 128), i32),
            vm((G, S // 2, 128), i32), vm((G, S // 2, 128), i32),
            vm((NSEG, D // 2, L), i32),
            vm((G, S // 2, 128), i32),
            vm((S, D), bf16), vm((S, D), bf16),
            vm((NSEG, G, 8, 128), f32),
            vm((2 * H, 128), f32),
            vm((S // OB, 128), f32),
            vm((ONB, OB, D), f32),
            vm((D, F), bf16), vm((D, F), bf16), vm((F, D), bf16),
            pltpu.SemaphoreType.DMA((16,)),
        ],
        compiler_params=pltpu.CompilerParams(vmem_limit_bytes=120 * 1024 * 1024, flags=_FLAGS),
    )(np.zeros((1,), np.int32), A_beta, B_w_r, A_x, A_wq, A_wk, A_wv, A_wo, B_w_gate, B_w_up, B_w_down)
```

```python
import math

import jax
import jax.numpy as jnp
import numpy as np
from jax import lax
import jax.experimental.pallas as pl
import jax.experimental.pallas.tpu as pltpu

S = 2048
D = 1024
H = 32
DH = D // H
NSEG = 4
L = S // NSEG
G = 8
F = 3584
OB = 32
OSTEP = 30
ONP = 2
NLN = 4
LNE = 1
MEMPOS = 2
TORD = 1302
ONB = 5
AG = 2
LAG = 3
FCH = 896

bf16 = jnp.bfloat16
f32 = jnp.float32
i32 = jnp.int32

QSCALE = (DH ** -0.5) * math.log2(math.e)
SAFE_BOUND = 24.0
NEG = -1e30
EPS_BF16 = 1.0013580322265625e-05

_NT = (((1,), (1,)), ((), ()))
_ONLY = None
_FLAGS = None


def _r(x):
    return x.astype(bf16).astype(f32)


def _pack(x):
    return pltpu.bitcast(x.astype(bf16), i32)


def _unpack(w):
    return pltpu.bitcast(w, bf16)


def _layernorm(xf):
    mean = jnp.sum(xf, axis=1, keepdims=True) * (1.0 / D)
    c = xf - mean
    var = jnp.sum(c * c, axis=1, keepdims=True) * (1.0 / D)
    d = _r(xf - _r(mean))
    s = _r(jnp.sqrt(_r(_r(var) + EPS_BF16)))
    return _r(d * (1.0 / s))


def _phi(t):
    return jnp.where(t > 0, t + 1.0, jnp.exp(t))


def _head_lanes(qi, h):
    lane = lax.broadcasted_iota(i32, qi.shape, 1)
    return _unpack(jnp.where((lane >> 5) == h, qi, 0))


def _fold8(x):
    return x.reshape(x.shape[0] // 8, 8, x.shape[1])


def _half(i, n):
    return pl.ds(i // 2 if isinstance(i, int) else pl.multiple_of(i // 2, n // 2), n // 2)


def _kernel(zero_s, beta_ref, wr_ref,
            x_hbm, wq_hbm, wk_hbm, wv_hbm, wo_hbm, wg_hbm, wu_hbm, wd_hbm,
            out_hbm,
            xio, wst, xa, xn, wo, qs, pq, ks, pk, vt, o_s, y_s, x1_s,
            zs, gt, r_s, oc, wg, wu, wd, sems):
    nx = NSEG
    XP = L // 4
    QD = D // 4

    def cp(src, dst, i):
        return pltpu.make_async_copy(src, dst, sems.at[i])

    def wcols(lo, n):
        return wv_hbm.at[:, pl.ds(lo, n)], wst.at[0, :, pl.ds(lo, n)]

    x0_cp = [cp(x_hbm.at[0, pl.ds(i * XP, XP), :], xio.at[pl.ds(i * XP, XP), :], i)
             for i in range(4)]
    x_cp = [None] + [cp(x_hbm.at[0, pl.ds(i * L, L), :], xio.at[pl.ds(i * L, L), :], 3 + i)
                     for i in range(1, nx)]
    wv_cp = [cp(*wcols(0, QD), 7), cp(*wcols(QD, QD), 8), cp(*wcols(2 * QD, 2 * QD), 9)]
    w_cp = [cp(src, dst, 10 + i) for i, (src, dst) in
            enumerate([(wq_hbm, wst.at[1]), (wk_hbm, wst.at[2]), (wo_hbm, wst.at[3]),
                       (wg_hbm, wg), (wu_hbm, wu), (wd_hbm, wd)])]
    for c in x0_cp + wv_cp + w_cp[:2] + x_cp[1:2] + w_cp[2:3] + x_cp[2:] + w_cp[3:]:
        c.start()

    b = jnp.broadcast_to(beta_ref[...].astype(f32).reshape(1, H), (H, H))
    rr = lax.broadcasted_iota(i32, (H, H), 0)
    cc = lax.broadcasted_iota(i32, (H, H), 1)
    bcol = jnp.sum(jnp.where(rr == cc, b, 0.0), axis=1, keepdims=True)
    gsig = _r(jax.nn.sigmoid(jnp.broadcast_to(bcol, (H, 128))))
    gt[0:H, :] = gsig
    gt[H:2 * H, :] = 1.0 - gsig

    lane = lax.broadcasted_iota(i32, (128, 128), 1)
    row = lax.broadcasted_iota(i32, (128, 128), 0)

    def ln_rows(r0, n, src=None, after=None):
        src = xa if src is None else src
        xf = src[pl.ds(r0, n), :].astype(f32)
        if after is not None:
            z = pltpu.bitcast(jnp.concatenate([after] * (n // 8), axis=0), f32)
            xf = jnp.concatenate([xf[:, 0:128] + z, xf[:, 128:]], axis=1)
        xn[_half(r0, n), :] = _pack(_layernorm(xf))

    def ln_block(r0, src=None):
        ln_rows(r0, L, src)

    def pin(w32, ref):
        zero = zero_s[0]
        lk = ref[pl.ds(pl.multiple_of(zero, 8), 8), 0:128] & zero
        head = jnp.concatenate([w32[0:8, 0:128] | lk, w32[0:8, 128:]], axis=1)
        return head if w32.shape[0] == 8 else jnp.concatenate([head, w32[8:]], axis=0)

    CB = 256

    def next_block(s):
        return pl.multiple_of(jnp.minimum(s + 1, NSEG - 1) * L, L)

    def v_cols(s, xb, lo, hi):
        for c0 in range(lo, hi, CB):
            v = jnp.dot(xb, wst[0, :, c0:c0 + CB], preferred_element_type=f32)
            vt[s, c0 // 2:(c0 + CB) // 2, :] = pltpu.bitcast(v.astype(bf16).T, i32)

    def q_cols(s, r0, xb, c0, qmax):
        q = jnp.dot(xb, wst[1, :, c0:c0 + CB], preferred_element_type=f32)
        for j in range(CB // 128):
            g = c0 // 128 + j
            qg = q[:, j * 128:(j + 1) * 128]
            qsc = qg * QSCALE
            qs[g, _half(r0, L), :] = _pack(qsc)
            pq[g, _half(r0, L), :] = _pack(_phi(qg))
            qmax = jnp.maximum(qmax, jnp.max(_fold8(jnp.abs(qsc)), axis=0))
        return qmax

    def k_cols(s, r0, xb, c0, kmax):
        k = jnp.dot(xb, wst[2, :, c0:c0 + CB], preferred_element_type=f32)
        for j in range(CB // 128):
            g = c0 // 128 + j
            kg = k[:, j * 128:(j + 1) * 128]
            ks[g, _half(r0, L), :] = _pack(kg)
            pkg = _phi(kg)
            pk[g, _half(r0, L), :] = _pack(pkg)
            zs[s, g] = jnp.sum(_fold8(pkg), axis=0)
            kmax = jnp.maximum(kmax, jnp.max(_fold8(jnp.abs(kg)), axis=0))
        return kmax

    def proj_first():
        for i in range(4):
            x0_cp[i].wait()
            ln_rows(i * XP, XP, xio)
        for c, lo, hi in zip(wv_cp, (0, QD, 2 * QD), (QD, 2 * QD, D)):
            c.wait()
            v_cols(0, _unpack(xn[0:L // 2, :]), lo, hi)
        w_cp[0].wait()
        qmax = kmax = jnp.zeros((8, 128), f32)
        xb = _unpack(xn[0:L // 2, :])
        for c0 in range(0, D, CB):
            qmax = q_cols(0, 0, xb, c0, qmax)
        w_cp[1].wait()
        x_cp[1].wait()
        xb = _unpack(xn[0:L // 2, :])
        for c0 in range(0, D, CB):
            kmax = k_cols(0, 0, xb, c0, kmax)
        ln_block(L, xio)
        w_cp[2].wait()
        return qmax, kmax

    def proj_block(s, carry, li):
        qmax, kmax = carry
        if li == 0:
            for i in range(2, nx):
                @pl.when(s == i - 1)
                def _():
                    x_cp[i].wait()
        r0 = pl.multiple_of(s * L, L)
        xb = _unpack(xn[_half(r0, L), :])
        v_cols(s, xb, 0, D)
        for c0 in range(0, D, CB):
            qmax = q_cols(s, r0, xb, c0, qmax)
            kmax = k_cols(s, r0, xb, c0, kmax)
        ln_block(next_block(s), xio if li == 0 else xa)
        if li == 0:
            w0 = pl.multiple_of((s - 1) * 168, 8)
            wo[pl.ds(w0, 176), :] = _pack(wst[3, pl.ds(pl.multiple_of(2 * w0, 16), 352), :])
        return qmax, kmax

    def attn_groups(g0, ng, use_max):
        causal = row <= lane
        gs = [g0 + i for i in range(ng)]
        g64 = [pl.multiple_of(g * 64, 64) for g in gs]
        blockdiag = (row >> 5) == (lane >> 5)
        lane16 = lax.broadcasted_iota(i32, (16, 128), 1)
        row16 = lax.broadcasted_iota(i32, (16, 128), 0)
        zmask = (lane16 >> 5) == row16

        def tile(ref, g, s, t):
            return ref[g, (s * L + t * 128) // 2:(s * L + (t + 1) * 128) // 2, :]

        split_diag = not use_max
        causal32 = (lax.broadcasted_iota(i32, (32, 128), 0)
                    <= (lax.broadcasted_iota(i32, (32, 128), 1) & 31))

        def block_transpose(src):
            rows = next(x for x in src if x is not None).shape[0]
            ln = lax.broadcasted_iota(i32, (rows, 128), 1)

            def pick(lo_mask, a, b):
                if a is None and b is None:
                    return None
                return jnp.where(lo_mask, 0.0 if a is None else a, 0.0 if b is None else b)

            def rot(x, n):
                return None if x is None else pltpu.roll(x, n, 1)

            x = [None] * 4
            for i in range(2):
                a, c = src[i], src[i + 2]
                x[i] = pick(ln < 64, a, rot(c, 64))
                x[i + 2] = pick(ln < 64, rot(a, 64), c)
            y = [None] * 4
            for i in (0, 2):
                a, c = x[i], x[i + 1]
                y[i] = pick((ln & 32) == 0, a, rot(c, 32))
                y[i + 1] = pick((ln & 32) == 0, rot(a, 96), c)
            return [jnp.zeros((rows, 128), f32) if v is None else v for v in y]

        def qk(gi, s, t, step):
            g = gs[gi]
            qt = tile(qs, g, s, t)
            qlane = lax.broadcasted_iota(i32, qt.shape, 1)
            qi = [jnp.where((qlane >> 5) == h, qt, 0) for h in range(4)]
            qm = [_unpack(x) for x in qi]
            Sc = [[None] * (t + 1) for _ in range(4)]
            for j in range(t if split_diag else t + 1):
                kk = _unpack(tile(ks, g, s, j))
                for h in range(4):
                    Sc[h][j] = lax.dot_general(kk, qm[h], _NT, preferred_element_type=f32)
            if not split_diag:
                return Sc, None
            kd = tile(ks, g, s, t)
            T = [None] * 4
            for u in range(4):
                w = _unpack(jnp.concatenate([x[16 * u:16 * u + 16] for x in qi], axis=0))
                T[u] = lax.dot_general(_unpack(kd[0:16 * (u + 1)]), w, _NT,
                                       preferred_element_type=f32)
            return Sc, T

        def tie(x, part):
            n = x.shape[0] - 8
            return jnp.concatenate([x[:n], x[n:] + part * 0.0], axis=0)

        def sm(ScD, t):
            Sc, T = ScD
            P = [None] * 4
            Linv = [None] * 4
            l8 = [None] * 4
            for h in range(4):
                sc = list(Sc[h])
                if not split_diag:
                    sc[t] = jnp.where(causal, sc[t], NEG)
                else:
                    sc = sc[:t]
                if use_max:
                    m = sc[0]
                    for j in range(1, t + 1):
                        m = jnp.maximum(m, sc[j])
                    m = jnp.max(m, axis=0, keepdims=True)
                    p = [jnp.exp2(x - m) for x in sc]
                else:
                    p = [jnp.exp2(x) for x in sc]
                P[h] = []
                for x in p:
                    part = jnp.sum(_fold8(x), axis=0)
                    l8[h] = part if l8[h] is None else l8[h] + part
                    P[h].append(tie(x, part).astype(bf16))
            if split_diag:
                E, ps = [], []
                for u in range(4):
                    e = jnp.exp2(jnp.where(causal32, T[u][32 * u:], NEG))
                    if u:
                        e = jnp.concatenate([jnp.exp2(T[u][:32 * u]), e], axis=0)
                    part = jnp.sum(_fold8(e), axis=0)
                    ps.append(part)
                    E.append(e)
                lh = block_transpose(ps)
                rows = [block_transpose([E[u][32 * r:32 * r + 32] if u >= r else None
                                         for u in range(4)]) for r in range(4)]
                for h in range(4):
                    l8[h] = lh[h] if l8[h] is None else l8[h] + lh[h]
                    P[h].append(jnp.concatenate([rows[r][h] for r in range(4)],
                                                axis=0).astype(bf16))
            for h in range(4):
                Linv[h] = 1.0 / jnp.sum(l8[h], axis=0, keepdims=True)
            return P, Linv

        def pv(PL, gi, s, t, lhs_m):
            g = gs[gi]
            P, Linv = PL
            acc = [None] * 4

            def mem_read():
                pqt = _unpack(tile(pq, g, s, t))
                return lax.dot_general(lhs_m, pqt, _NT, preferred_element_type=f32)

            if lhs_m is not None:
                nd = mem_read()
            for j in range(t + 1):
                for h in range(4):
                    vth = _unpack(vt[s, pl.ds(g64[gi] + 16 * h, 16), j * 128:(j + 1) * 128])
                    o = jnp.dot(vth, P[h][j], preferred_element_type=f32)
                    acc[h] = o if acc[h] is None else acc[h] + o
            outs = []
            for h in range(4):
                o = acc[h] * (gt[pl.ds(H + g * 4 + h, 1), :] * Linv[h])
                if lhs_m is not None:
                    den = nd[128 + h:129 + h, :] + 1e-6
                    o = o + nd[32 * h:32 * h + 32, :] * (gt[pl.ds(g * 4 + h, 1), :] / den)
                outs.append(o)
            ot = jnp.concatenate(outs, axis=0).astype(bf16)
            o_s[g, (s * L + t * 128) // 2:(s * L + (t + 1) * 128) // 2, :] = (
                pltpu.bitcast(ot.T, i32))

        def mem_update(gi, s, R):
            g = gs[gi]
            vtg = _unpack(vt[s, pl.ds(g64[gi], 64), :])
            pks = _unpack(pk[g, s * L // 2:(s + 1) * L // 2, :])
            upd = jnp.dot(vtg, pks, preferred_element_type=f32)
            return upd if R is None else R + upd

        def mem_lhs(gi, s, R):
            g = gs[gi]
            mt = jnp.where(blockdiag, R, 0.0)
            z = zs[0, g]
            for s2 in range(1, s):
                z = z + zs[s2, g]
            z = jnp.sum(z, axis=0, keepdims=True)
            zr = jnp.where(zmask, z, 0.0)
            return jnp.concatenate([mt, zr], axis=0).astype(bf16)

        order = [int(c) for c in str(TORD).zfill(4)]
        steps = [(gi, s, t) for gi in range(ng) for s in range(NSEG) for t in order]
        n = len(steps)
        Sc, PL = {}, {}
        R = None
        lhs = {}
        for i in range(n + LAG):
            if i < n:
                Sc[i] = qk(*steps[i], i)
                gi, s, t = steps[i]
                if t == order[0] and s == 0:
                    R = None
                    lhs[gi, 0] = None
                if t == order[MEMPOS] and s < NSEG - 1:
                    R = mem_update(gi, s, R)
                    lhs[gi, s + 1] = mem_lhs(gi, s + 1, R)
                PL[i] = sm(Sc.pop(i), t)
            if 0 <= i - LAG < n:
                gi, s, t = steps[i - LAG]
                pv(PL.pop(i - LAG), gi, s, t, lhs[gi, s])

    CP, RP = D // ONP, OB // ONP

    def o_lhs(r0):
        return jnp.concatenate([_unpack(o_s[g, _half(r0, OB), :]) for g in range(G)], axis=1)

    def o_epilogue(refs, r0, out, last):
        xa_, x1_, y_, xo_ = refs
        res = xa_[r0:r0 + RP, :] if last else xo_[r0:r0 + RP, :].astype(f32)
        x1 = _r(res + _r(out))
        x1_[r0:r0 + RP, :] = x1.astype(bf16)
        y = _layernorm(x1)
        y_[r0:r0 + RP, :] = y.astype(bf16)
        if last:
            xo_[r0:r0 + RP, :] = (x1 + y).astype(bf16)
        else:
            xa_[r0:r0 + RP, :] = _r(x1 + y)
        wr = wr_ref[...].astype(f32).reshape(1, D)
        return _r(jnp.sum(y * wr, axis=1, keepdims=True))

    def o_refs(r0, n):
        return [xa.at[pl.ds(r0, n)], x1_s.at[pl.ds(r0, n)], y_s.at[pl.ds(r0, n)],
                xio.at[pl.ds(r0, n)]]

    def o_step(refs, k, blk, src, dst, last):
        if dst is not None:
            ob = o_lhs((blk + 1) * OB)
        rcols = []
        for p in range(ONP):
            if dst is not None:
                dst[:, p * CP:(p + 1) * CP] = jnp.dot(
                    ob, _unpack(wo[:, p * CP:(p + 1) * CP]), preferred_element_type=f32)
            rcols.append(o_epilogue(refs, k * OB + p * RP, src[p * RP:(p + 1) * RP, :], last))
        rb = jnp.broadcast_to(jnp.concatenate(rcols, axis=0), (OB, 128))
        lane_ob = lax.broadcasted_iota(i32, (OB, 128), 1)
        row_ob = lax.broadcasted_iota(i32, (OB, 128), 0)
        r_s[pl.ds(blk, 1), :] = jnp.max(jnp.where(row_ob == lane_ob, rb, -jnp.inf),
                                        axis=0, keepdims=True)

    def o_phase(last):
        nb = S // OB
        oc[0] = jnp.dot(o_lhs(0), _unpack(wo[...]), preferred_element_type=f32)
        nloop = (nb - 2) // OSTEP
        assert OSTEP % ONB == 0

        def out_rows(r0, n):
            return pltpu.make_async_copy(xio.at[pl.ds(r0, n)], out_hbm.at[0, pl.ds(r0, n)],
                                         sems.at[2])

        def body(i, carry):
            if last:
                @pl.when(i > 0)
                def _():
                    out_rows(pl.multiple_of((i - 1) * OSTEP * OB, OSTEP * OB),
                             OSTEP * OB).start()

            refs = o_refs(pl.multiple_of(i * OSTEP * OB, OSTEP * OB), OSTEP * OB)
            for k in range(OSTEP):
                o_step(refs, k, i * OSTEP + k, oc.at[k % ONB], oc.at[(k + 1) % ONB], last)
            return carry

        lax.fori_loop(0, nloop, body, 0)
        b0 = nloop * OSTEP
        if last:
            out_rows((b0 - OSTEP) * OB, OSTEP * OB).start()
        refs = o_refs(b0 * OB, (nb - b0) * OB)
        for k in range(nb - b0):
            o_step(refs, k, b0 + k, oc.at[k % ONB],
                   oc.at[(k + 1) % ONB] if b0 + k + 1 < nb else None, last)
        if last:
            out_rows(b0 * OB, (nb - b0) * OB).start()

    out_cp = pltpu.make_async_copy(xio, out_hbm.at[0], sems.at[2])

    def moe_phase(last):
        r_all = r_s[...]
        ridx = (lax.broadcasted_iota(i32, r_all.shape, 0) * OB
                + lax.broadcasted_iota(i32, r_all.shape, 1)).astype(f32)

        def red(fn, x):
            return fn(fn(x, axis=0, keepdims=True), axis=1, keepdims=True)

        m1 = red(jnp.max, r_all)
        i1f = red(jnp.min, jnp.where(r_all == m1, ridx, 1e9))
        r2 = jnp.where(ridx == i1f, -jnp.inf, r_all)
        m2 = red(jnp.max, r2)
        i2f = red(jnp.min, jnp.where((r2 == m2) & (ridx != i1f), ridx, 1e9))
        idx = [jnp.clip(v[0, 0].astype(i32), 0, S - 1) for v in (i1f, i2f)]
        base = [pl.multiple_of((ix >> 4) << 4, 16) for ix in idx]
        off = [ix & 15 for ix in idx]
        row16 = lax.broadcasted_iota(i32, (16, D), 0)

        def gather(ref):
            res = None
            for kk in range(2):
                blk = ref[pl.ds(base[kk], 16), :].astype(f32)
                one = jnp.sum(jnp.where(row16 == off[kk], blk, 0.0), axis=0, keepdims=True)
                part = jnp.where(row16 == kk, one, 0.0)
                res = part if res is None else res + part
            return res

        ysel = gather(y_s)
        x1sel = gather(x1_s)
        xsel32 = _pack(ysel)
        yf = None
        after = None
        nch = F // FCH
        rp = L // NLN
        for ci, c0 in enumerate(range(0, F, FCH)):
            if not last and ci % LNE == 0 and ci // LNE < NLN:
                ln_rows(ci // LNE * rp, rp, None, after)
                xsel = _unpack(pin(xsel32, xn))
            else:
                xsel = _unpack(xsel32)
            gte = _r(jnp.dot(xsel, wg[:, c0:c0 + FCH], preferred_element_type=f32))
            after = pltpu.bitcast(gte[0:8, 0:128], i32) & zero_s[0]
            up = _r(jnp.dot(xsel, wu[:, c0:c0 + FCH], preferred_element_type=f32))
            act = _r(gte * jax.nn.sigmoid(gte))
            hcol = (act * up).astype(bf16)
            part = jnp.dot(hcol, wd[c0:c0 + FCH, :], preferred_element_type=f32)
            yf = part if yf is None else yf + part
        rsel = _r(jax.nn.sigmoid(jnp.where(row16 == 0, m1, m2)))
        upd = _r(_r(yf) * rsel)
        x2 = _r(x1sel + _r(ysel + upd))
        rows2 = [jnp.sum(jnp.where(row16 == kk, x2, 0.0), axis=0, keepdims=True)
                 for kk in range(2)]
        if not last:
            xn2 = _layernorm(x2)
            for kk in range(2):
                xa[pl.ds(idx[kk], 1), :] = rows2[kk]
                one = jnp.sum(jnp.where(row16 == kk, xn2, 0.0), axis=0, keepdims=True)
                blk = _unpack(xn[_half(base[kk], 16), :]).astype(f32)
                xn[_half(base[kk], 16), :] = _pack(jnp.where(row16 == off[kk], one, blk))
        else:
            out_cp.wait()
            for kk in range(2):
                blk = xio[pl.ds(base[kk], 16), :].astype(f32)
                xio[pl.ds(base[kk], 16), :] = jnp.where(
                    row16 == off[kk], rows2[kk], blk).astype(bf16)
            cp0 = pltpu.make_async_copy(xio.at[pl.ds(base[0], 16), :],
                                        out_hbm.at[0, pl.ds(base[0], 16), :], sems.at[0])
            cp1 = pltpu.make_async_copy(xio.at[pl.ds(base[1], 16), :],
                                        out_hbm.at[0, pl.ds(base[1], 16), :], sems.at[1])
            cp0.start()

            @pl.when(base[0] != base[1])
            def _():
                cp1.start()
                cp1.wait()

            cp0.wait()

    if _ONLY:
        for c in x0_cp + x_cp[1:] + wv_cp + w_cp:
            c.wait()
        dict(O0=lambda: o_phase(False), O1=lambda: o_phase(True),
             B0=lambda: moe_phase(False),
             A=lambda: lax.fori_loop(0, G // AG, lambda i, c: (attn_groups(i * AG, AG, False), c)[1], 0))[_ONLY]()
        out_cp.start()
        out_cp.wait()
        return

    for li in range(2):
        last = li == 1
        if li == 0:
            qmax, kmax = lax.fori_loop(1, NSEG, lambda s, c: proj_block(s, c, 0), proj_first())
        else:
            z8 = jnp.zeros((8, 128), f32)
            qmax, kmax = lax.fori_loop(0, NSEG, lambda s, c: proj_block(s, c, 1), (z8, z8))
        bound = DH * jnp.max(qmax) * jnp.max(kmax)
        safe = bound <= SAFE_BOUND

        @pl.when(safe)
        def _():
            lax.fori_loop(0, G // AG, lambda i, c: (attn_groups(i * AG, AG, False), c)[1], 0)

        @pl.when(jnp.logical_not(safe))
        def _():
            lax.fori_loop(0, G, lambda g, c: (attn_groups(g, 1, True), c)[1], 0)

        o_phase(last)
        if li == 0:
            for c in w_cp[3:]:
                c.wait()
        moe_phase(last)


@jax.jit
def pallas_interleave_layers__memory_aug_infini_attn__moe_arch_mod__prompt_kernel(
    A_x: jax.Array,
    A_wq: jax.Array,
    A_wk: jax.Array,
    A_wv: jax.Array,
    A_wo: jax.Array,
    A_beta: jax.Array,
    B_x: jax.Array,
    B_w_r: jax.Array,
    B_w_gate: jax.Array,
    B_w_up: jax.Array,
    B_w_down: jax.Array,
):
    del B_x
    any_spec = pl.BlockSpec(memory_space=pl.ANY)
    vm = pltpu.VMEM
    return pl.pallas_call(
        _kernel,
        out_shape=jax.ShapeDtypeStruct((1, S, D), bf16),
        in_specs=[pl.BlockSpec(memory_space=pltpu.SMEM),
                  pl.BlockSpec(memory_space=vm), pl.BlockSpec(memory_space=vm)] + [any_spec] * 8,
        out_specs=any_spec,
        scratch_shapes=[
            vm((S, D), bf16),
            vm((4, D, D), bf16),
            vm((S, D), f32),
            vm((S // 2, D), i32),
            vm((D // 2, D), i32),
            vm((G, S // 2, 128), i32), vm((G, S // 2, 128), i32),
            vm((G, S // 2, 128), i32), vm((G, S // 2, 128), i32),
            vm((NSEG, D // 2, L), i32),
            vm((G, S // 2, 128), i32),
            vm((S, D), bf16), vm((S, D), bf16),
            vm((NSEG, G, 8, 128), f32),
            vm((2 * H, 128), f32),
            vm((S // OB, 128), f32),
            vm((ONB, OB, D), f32),
            vm((D, F), bf16), vm((D, F), bf16), vm((F, D), bf16),
            pltpu.SemaphoreType.DMA((16,)),
        ],
        compiler_params=pltpu.CompilerParams(vmem_limit_bytes=120 * 1024 * 1024, flags=_FLAGS),
    )(np.zeros((1,), np.int32), A_beta, B_w_r, A_x, A_wq, A_wk, A_wv, A_wo, B_w_gate, B_w_up, B_w_down)
```

```python
import math

import jax
import jax.numpy as jnp
import numpy as np
from jax import lax
import jax.experimental.pallas as pl
import jax.experimental.pallas.tpu as pltpu

S = 2048
D = 1024
H = 32
DH = D // H
NSEG = 4
L = S // NSEG
G = 8
F = 3584
OB = 32
OSTEP = 30
ONP = 2
MEMPOS = 2
TORD = 1302
ONB = 5
AG = 2
LAG = 3
FCH = 896

bf16 = jnp.bfloat16
f32 = jnp.float32
i32 = jnp.int32

QSCALE = (DH ** -0.5) * math.log2(math.e)
SAFE_BOUND = 24.0
NEG = -1e30
EPS_BF16 = 1.0013580322265625e-05

_NT = (((1,), (1,)), ((), ()))


def _r(x):
    return x.astype(bf16).astype(f32)


def _pack(x):
    return pltpu.bitcast(x.astype(bf16), i32)


def _unpack(w):
    return pltpu.bitcast(w, bf16)


def _layernorm(xf):
    mean = jnp.sum(xf, axis=1, keepdims=True) * (1.0 / D)
    c = xf - mean
    var = jnp.sum(c * c, axis=1, keepdims=True) * (1.0 / D)
    d = _r(xf - _r(mean))
    s = _r(jnp.sqrt(_r(_r(var) + EPS_BF16)))
    return _r(d * (1.0 / s))


def _phi(t):
    return jnp.where(t > 0, t + 1.0, jnp.exp(t))


def _fold8(x):
    return x.reshape(x.shape[0] // 8, 8, x.shape[1])


def _half(i, n):
    return pl.ds(i // 2 if isinstance(i, int) else pl.multiple_of(i // 2, n // 2), n // 2)


def _kernel(zero_s, beta_ref, wr_ref,
            x_hbm, wq_hbm, wk_hbm, wv_hbm, wo_hbm, wg_hbm, wu_hbm, wd_hbm,
            out_hbm,
            xio, wst, xa, xn, wo, qs, pq, ks, pk, vt, o_s, y_s, x1_s,
            zs, gt, r_s, oc, wg, wu, wd, sems):
    nx = NSEG
    XP = L // 4
    QD = D // 4

    def cp(src, dst, i):
        return pltpu.make_async_copy(src, dst, sems.at[i])

    def wcols(lo, n):
        return wv_hbm.at[:, pl.ds(lo, n)], wst.at[0, :, pl.ds(lo, n)]

    x0_cp = [cp(x_hbm.at[0, pl.ds(i * XP, XP), :], xio.at[pl.ds(i * XP, XP), :], i)
             for i in range(4)]
    x_cp = [None] + [cp(x_hbm.at[0, pl.ds(i * L, L), :], xio.at[pl.ds(i * L, L), :], 3 + i)
                     for i in range(1, nx)]
    wv_cp = [cp(*wcols(0, QD), 7), cp(*wcols(QD, QD), 8), cp(*wcols(2 * QD, 2 * QD), 9)]
    w_cp = [cp(src, dst, 10 + i) for i, (src, dst) in
            enumerate([(wq_hbm, wst.at[1]), (wk_hbm, wst.at[2]), (wo_hbm, wst.at[3]),
                       (wg_hbm, wg), (wu_hbm, wu), (wd_hbm, wd)])]
    for c in x0_cp + wv_cp + w_cp[:2] + x_cp[1:2] + w_cp[2:3] + x_cp[2:] + w_cp[3:]:
        c.start()

    b = jnp.broadcast_to(beta_ref[...].astype(f32).reshape(1, H), (H, H))
    rr = lax.broadcasted_iota(i32, (H, H), 0)
    cc = lax.broadcasted_iota(i32, (H, H), 1)
    bcol = jnp.sum(jnp.where(rr == cc, b, 0.0), axis=1, keepdims=True)
    gsig = _r(jax.nn.sigmoid(jnp.broadcast_to(bcol, (H, 128))))
    gt[0:H, :] = gsig
    gt[H:2 * H, :] = 1.0 - gsig

    lane = lax.broadcasted_iota(i32, (128, 128), 1)
    row = lax.broadcasted_iota(i32, (128, 128), 0)

    def ln_rows(r0, n, src=None, after=None):
        src = xa if src is None else src
        xf = src[pl.ds(r0, n), :].astype(f32)
        if after is not None:
            z = pltpu.bitcast(jnp.concatenate([after] * (n // 8), axis=0), f32)
            xf = jnp.concatenate([xf[:, 0:128] + z, xf[:, 128:]], axis=1)
        xn[_half(r0, n), :] = _pack(_layernorm(xf))

    def ln_block(r0, src=None):
        ln_rows(r0, L, src)

    def pin(w32, ref):
        zero = zero_s[0]
        lk = ref[pl.ds(pl.multiple_of(zero, 8), 8), 0:128] & zero
        head = jnp.concatenate([w32[0:8, 0:128] | lk, w32[0:8, 128:]], axis=1)
        return head if w32.shape[0] == 8 else jnp.concatenate([head, w32[8:]], axis=0)

    CB = 256

    def next_block(s):
        return pl.multiple_of(jnp.minimum(s + 1, NSEG - 1) * L, L)

    def v_cols(s, xb, lo, hi):
        for c0 in range(lo, hi, CB):
            v = jnp.dot(xb, wst[0, :, c0:c0 + CB], preferred_element_type=f32)
            vt[s, c0 // 2:(c0 + CB) // 2, :] = pltpu.bitcast(v.astype(bf16).T, i32)

    def q_cols(s, r0, xb, c0, qmax):
        q = jnp.dot(xb, wst[1, :, c0:c0 + CB], preferred_element_type=f32)
        for j in range(CB // 128):
            g = c0 // 128 + j
            qg = q[:, j * 128:(j + 1) * 128]
            qsc = qg * QSCALE
            qs[g, _half(r0, L), :] = _pack(qsc)
            pq[g, _half(r0, L), :] = _pack(_phi(qg))
            qmax = jnp.maximum(qmax, jnp.max(_fold8(jnp.abs(qsc)), axis=0))
        return qmax

    def k_cols(s, r0, xb, c0, kmax):
        k = jnp.dot(xb, wst[2, :, c0:c0 + CB], preferred_element_type=f32)
        for j in range(CB // 128):
            g = c0 // 128 + j
            kg = k[:, j * 128:(j + 1) * 128]
            ks[g, _half(r0, L), :] = _pack(kg)
            pkg = _phi(kg)
            pk[g, _half(r0, L), :] = _pack(pkg)
            zs[s, g] = jnp.sum(_fold8(pkg), axis=0)
            kmax = jnp.maximum(kmax, jnp.max(_fold8(jnp.abs(kg)), axis=0))
        return kmax

    def proj_first():
        for i in range(4):
            x0_cp[i].wait()
            ln_rows(i * XP, XP, xio)
        for c, lo, hi in zip(wv_cp, (0, QD, 2 * QD), (QD, 2 * QD, D)):
            c.wait()
            v_cols(0, _unpack(xn[0:L // 2, :]), lo, hi)
        w_cp[0].wait()
        qmax = kmax = jnp.zeros((8, 128), f32)
        xb = _unpack(xn[0:L // 2, :])
        for c0 in range(0, D, CB):
            qmax = q_cols(0, 0, xb, c0, qmax)
        w_cp[1].wait()
        x_cp[1].wait()
        xb = _unpack(xn[0:L // 2, :])
        for c0 in range(0, D, CB):
            kmax = k_cols(0, 0, xb, c0, kmax)
        ln_block(L, xio)
        w_cp[2].wait()
        return qmax, kmax

    def proj_block(s, carry, li):
        qmax, kmax = carry
        if li == 0:
            for i in range(2, nx):
                @pl.when(s == i - 1)
                def _():
                    x_cp[i].wait()
        r0 = pl.multiple_of(s * L, L)
        xb = _unpack(xn[_half(r0, L), :])
        v_cols(s, xb, 0, D)
        for c0 in range(0, D, CB):
            qmax = q_cols(s, r0, xb, c0, qmax)
            kmax = k_cols(s, r0, xb, c0, kmax)
        ln_block(next_block(s), xio if li == 0 else xa)
        if li == 0:
            w0 = pl.multiple_of((s - 1) * 168, 8)
            wo[pl.ds(w0, 176), :] = _pack(wst[3, pl.ds(pl.multiple_of(2 * w0, 16), 352), :])
        return qmax, kmax

    def attn_groups(g0, ng, use_max):
        causal = row <= lane
        gs = [g0 + i for i in range(ng)]
        g64 = [pl.multiple_of(g * 64, 64) for g in gs]
        blockdiag = (row >> 5) == (lane >> 5)
        lane16 = lax.broadcasted_iota(i32, (16, 128), 1)
        row16 = lax.broadcasted_iota(i32, (16, 128), 0)
        zmask = (lane16 >> 5) == row16

        def tile(ref, g, s, t):
            return ref[g, (s * L + t * 128) // 2:(s * L + (t + 1) * 128) // 2, :]

        split_diag = not use_max
        causal32 = (lax.broadcasted_iota(i32, (32, 128), 0)
                    <= (lax.broadcasted_iota(i32, (32, 128), 1) & 31))

        def block_transpose(src):
            rows = next(x for x in src if x is not None).shape[0]
            ln = lax.broadcasted_iota(i32, (rows, 128), 1)

            def pick(lo_mask, a, b):
                if a is None and b is None:
                    return None
                return jnp.where(lo_mask, 0.0 if a is None else a, 0.0 if b is None else b)

            def rot(x, n):
                return None if x is None else pltpu.roll(x, n, 1)

            x = [None] * 4
            for i in range(2):
                a, c = src[i], src[i + 2]
                x[i] = pick(ln < 64, a, rot(c, 64))
                x[i + 2] = pick(ln < 64, rot(a, 64), c)
            y = [None] * 4
            for i in (0, 2):
                a, c = x[i], x[i + 1]
                y[i] = pick((ln & 32) == 0, a, rot(c, 32))
                y[i + 1] = pick((ln & 32) == 0, rot(a, 96), c)
            return [jnp.zeros((rows, 128), f32) if v is None else v for v in y]

        def qk(gi, s, t):
            g = gs[gi]
            qt = tile(qs, g, s, t)
            qlane = lax.broadcasted_iota(i32, qt.shape, 1)
            qi = [jnp.where((qlane >> 5) == h, qt, 0) for h in range(4)]
            qm = [_unpack(x) for x in qi]
            Sc = [[None] * (t + 1) for _ in range(4)]
            for j in range(t if split_diag else t + 1):
                kk = _unpack(tile(ks, g, s, j))
                for h in range(4):
                    Sc[h][j] = lax.dot_general(kk, qm[h], _NT, preferred_element_type=f32)
            if not split_diag:
                return Sc, None
            kd = tile(ks, g, s, t)
            T = [None] * 4
            for u in range(4):
                w = _unpack(jnp.concatenate([x[16 * u:16 * u + 16] for x in qi], axis=0))
                T[u] = lax.dot_general(_unpack(kd[0:16 * (u + 1)]), w, _NT,
                                       preferred_element_type=f32)
            return Sc, T

        def tie(x, part):
            n = x.shape[0] - 8
            return jnp.concatenate([x[:n], x[n:] + part * 0.0], axis=0)

        def sm(ScD, t):
            Sc, T = ScD
            P = [None] * 4
            Linv = [None] * 4
            l8 = [None] * 4
            for h in range(4):
                sc = list(Sc[h])
                if not split_diag:
                    sc[t] = jnp.where(causal, sc[t], NEG)
                else:
                    sc = sc[:t]
                if use_max:
                    m = sc[0]
                    for j in range(1, t + 1):
                        m = jnp.maximum(m, sc[j])
                    m = jnp.max(m, axis=0, keepdims=True)
                    p = [jnp.exp2(x - m) for x in sc]
                else:
                    p = [jnp.exp2(x) for x in sc]
                P[h] = []
                for x in p:
                    part = jnp.sum(_fold8(x), axis=0)
                    l8[h] = part if l8[h] is None else l8[h] + part
                    P[h].append(tie(x, part).astype(bf16))
            if split_diag:
                E, ps = [], []
                for u in range(4):
                    e = jnp.exp2(jnp.where(causal32, T[u][32 * u:], NEG))
                    if u:
                        e = jnp.concatenate([jnp.exp2(T[u][:32 * u]), e], axis=0)
                    part = jnp.sum(_fold8(e), axis=0)
                    ps.append(part)
                    E.append(e)
                lh = block_transpose(ps)
                rows = [block_transpose([E[u][32 * r:32 * r + 32] if u >= r else None
                                         for u in range(4)]) for r in range(4)]
                for h in range(4):
                    l8[h] = lh[h] if l8[h] is None else l8[h] + lh[h]
                    P[h].append(jnp.concatenate([rows[r][h] for r in range(4)],
                                                axis=0).astype(bf16))
            for h in range(4):
                Linv[h] = 1.0 / jnp.sum(l8[h], axis=0, keepdims=True)
            return P, Linv

        def pv(PL, gi, s, t, lhs_m):
            g = gs[gi]
            P, Linv = PL
            acc = [None] * 4

            def mem_read():
                pqt = _unpack(tile(pq, g, s, t))
                return lax.dot_general(lhs_m, pqt, _NT, preferred_element_type=f32)

            if lhs_m is not None:
                nd = mem_read()
            for j in range(t + 1):
                for h in range(4):
                    vth = _unpack(vt[s, pl.ds(g64[gi] + 16 * h, 16), j * 128:(j + 1) * 128])
                    o = jnp.dot(vth, P[h][j], preferred_element_type=f32)
                    acc[h] = o if acc[h] is None else acc[h] + o
            outs = []
            for h in range(4):
                o = acc[h] * (gt[pl.ds(H + g * 4 + h, 1), :] * Linv[h])
                if lhs_m is not None:
                    den = nd[128 + h:129 + h, :] + 1e-6
                    o = o + nd[32 * h:32 * h + 32, :] * (gt[pl.ds(g * 4 + h, 1), :] / den)
                outs.append(o)
            ot = jnp.concatenate(outs, axis=0).astype(bf16)
            o_s[g, (s * L + t * 128) // 2:(s * L + (t + 1) * 128) // 2, :] = (
                pltpu.bitcast(ot.T, i32))

        def mem_update(gi, s, R):
            g = gs[gi]
            vtg = _unpack(vt[s, pl.ds(g64[gi], 64), :])
            pks = _unpack(pk[g, s * L // 2:(s + 1) * L // 2, :])
            upd = jnp.dot(vtg, pks, preferred_element_type=f32)
            return upd if R is None else R + upd

        def mem_lhs(gi, s, R):
            g = gs[gi]
            mt = jnp.where(blockdiag, R, 0.0)
            z = zs[0, g]
            for s2 in range(1, s):
                z = z + zs[s2, g]
            z = jnp.sum(z, axis=0, keepdims=True)
            zr = jnp.where(zmask, z, 0.0)
            return jnp.concatenate([mt, zr], axis=0).astype(bf16)

        order = [int(c) for c in str(TORD).zfill(4)]
        steps = [(gi, s, t) for gi in range(ng) for s in range(NSEG) for t in order]
        n = len(steps)
        Sc, PL = {}, {}
        R = None
        lhs = {}
        for i in range(n + LAG):
            if i < n:
                Sc[i] = qk(*steps[i])
                gi, s, t = steps[i]
                if t == order[0] and s == 0:
                    R = None
                    lhs[gi, 0] = None
                if t == order[MEMPOS] and s < NSEG - 1:
                    R = mem_update(gi, s, R)
                    lhs[gi, s + 1] = mem_lhs(gi, s + 1, R)
                PL[i] = sm(Sc.pop(i), t)
            if 0 <= i - LAG < n:
                gi, s, t = steps[i - LAG]
                pv(PL.pop(i - LAG), gi, s, t, lhs[gi, s])

    CP, RP = D // ONP, OB // ONP

    def o_lhs(r0):
        return jnp.concatenate([_unpack(o_s[g, _half(r0, OB), :]) for g in range(G)], axis=1)

    def o_epilogue(refs, r0, out, last):
        xa_, x1_, y_, xo_ = refs
        res = xa_[r0:r0 + RP, :] if last else xo_[r0:r0 + RP, :].astype(f32)
        x1 = _r(res + _r(out))
        x1_[r0:r0 + RP, :] = x1.astype(bf16)
        y = _layernorm(x1)
        y_[r0:r0 + RP, :] = y.astype(bf16)
        if last:
            xo_[r0:r0 + RP, :] = (x1 + y).astype(bf16)
        else:
            xa_[r0:r0 + RP, :] = _r(x1 + y)
        wr = wr_ref[...].astype(f32).reshape(1, D)
        return _r(jnp.sum(y * wr, axis=1, keepdims=True))

    def o_refs(r0, n):
        return [xa.at[pl.ds(r0, n)], x1_s.at[pl.ds(r0, n)], y_s.at[pl.ds(r0, n)],
                xio.at[pl.ds(r0, n)]]

    def o_step(refs, k, blk, src, dst, last):
        if dst is not None:
            ob = o_lhs((blk + 1) * OB)
        rcols = []
        for p in range(ONP):
            if dst is not None:
                dst[:, p * CP:(p + 1) * CP] = jnp.dot(
                    ob, _unpack(wo[:, p * CP:(p + 1) * CP]), preferred_element_type=f32)
            rcols.append(o_epilogue(refs, k * OB + p * RP, src[p * RP:(p + 1) * RP, :], last))
        rb = jnp.broadcast_to(jnp.concatenate(rcols, axis=0), (OB, 128))
        lane_ob = lax.broadcasted_iota(i32, (OB, 128), 1)
        row_ob = lax.broadcasted_iota(i32, (OB, 128), 0)
        r_s[pl.ds(blk, 1), :] = jnp.max(jnp.where(row_ob == lane_ob, rb, -jnp.inf),
                                        axis=0, keepdims=True)

    def o_phase(last):
        nb = S // OB
        oc[0] = jnp.dot(o_lhs(0), _unpack(wo[...]), preferred_element_type=f32)
        nloop = (nb - 2) // OSTEP
        assert OSTEP % ONB == 0

        def out_rows(r0, n):
            return pltpu.make_async_copy(xio.at[pl.ds(r0, n)], out_hbm.at[0, pl.ds(r0, n)],
                                         sems.at[2])

        def body(i, carry):
            if last:
                @pl.when(i > 0)
                def _():
                    out_rows(pl.multiple_of((i - 1) * OSTEP * OB, OSTEP * OB),
                             OSTEP * OB).start()

            refs = o_refs(pl.multiple_of(i * OSTEP * OB, OSTEP * OB), OSTEP * OB)
            for k in range(OSTEP):
                o_step(refs, k, i * OSTEP + k, oc.at[k % ONB], oc.at[(k + 1) % ONB], last)
            return carry

        lax.fori_loop(0, nloop, body, 0)
        b0 = nloop * OSTEP
        if last:
            out_rows((b0 - OSTEP) * OB, OSTEP * OB).start()
        refs = o_refs(b0 * OB, (nb - b0) * OB)
        for k in range(nb - b0):
            o_step(refs, k, b0 + k, oc.at[k % ONB],
                   oc.at[(k + 1) % ONB] if b0 + k + 1 < nb else None, last)
        if last:
            out_rows(b0 * OB, (nb - b0) * OB).start()

    out_cp = pltpu.make_async_copy(xio, out_hbm.at[0], sems.at[2])

    def moe_phase(last):
        r_all = r_s[...]
        ridx = (lax.broadcasted_iota(i32, r_all.shape, 0) * OB
                + lax.broadcasted_iota(i32, r_all.shape, 1)).astype(f32)

        def red(fn, x):
            return fn(fn(x, axis=0, keepdims=True), axis=1, keepdims=True)

        m1 = red(jnp.max, r_all)
        i1f = red(jnp.min, jnp.where(r_all == m1, ridx, 1e9))
        r2 = jnp.where(ridx == i1f, -jnp.inf, r_all)
        m2 = red(jnp.max, r2)
        i2f = red(jnp.min, jnp.where((r2 == m2) & (ridx != i1f), ridx, 1e9))
        idx = [jnp.clip(v[0, 0].astype(i32), 0, S - 1) for v in (i1f, i2f)]
        base = [pl.multiple_of((ix >> 4) << 4, 16) for ix in idx]
        off = [ix & 15 for ix in idx]
        row16 = lax.broadcasted_iota(i32, (16, D), 0)

        def gather(ref):
            res = None
            for kk in range(2):
                blk = ref[pl.ds(base[kk], 16), :].astype(f32)
                one = jnp.sum(jnp.where(row16 == off[kk], blk, 0.0), axis=0, keepdims=True)
                part = jnp.where(row16 == kk, one, 0.0)
                res = part if res is None else res + part
            return res

        ysel = gather(y_s)
        x1sel = gather(x1_s)
        xsel32 = _pack(ysel)
        yf = None
        after = None
        rp = L // (F // FCH)
        for ci, c0 in enumerate(range(0, F, FCH)):
            if not last:
                ln_rows(ci * rp, rp, None, after)
                xsel = _unpack(pin(xsel32, xn))
            else:
                xsel = _unpack(xsel32)
            gte = _r(jnp.dot(xsel, wg[:, c0:c0 + FCH], preferred_element_type=f32))
            after = pltpu.bitcast(gte[0:8, 0:128], i32) & zero_s[0]
            up = _r(jnp.dot(xsel, wu[:, c0:c0 + FCH], preferred_element_type=f32))
            act = _r(gte * jax.nn.sigmoid(gte))
            hcol = (act * up).astype(bf16)
            part = jnp.dot(hcol, wd[c0:c0 + FCH, :], preferred_element_type=f32)
            yf = part if yf is None else yf + part
        rsel = _r(jax.nn.sigmoid(jnp.where(row16 == 0, m1, m2)))
        upd = _r(_r(yf) * rsel)
        x2 = _r(x1sel + _r(ysel + upd))
        rows2 = [jnp.sum(jnp.where(row16 == kk, x2, 0.0), axis=0, keepdims=True)
                 for kk in range(2)]
        if not last:
            xn2 = _layernorm(x2)
            for kk in range(2):
                xa[pl.ds(idx[kk], 1), :] = rows2[kk]
                one = jnp.sum(jnp.where(row16 == kk, xn2, 0.0), axis=0, keepdims=True)
                blk = _unpack(xn[_half(base[kk], 16), :]).astype(f32)
                xn[_half(base[kk], 16), :] = _pack(jnp.where(row16 == off[kk], one, blk))
        else:
            out_cp.wait()
            for kk in range(2):
                blk = xio[pl.ds(base[kk], 16), :].astype(f32)
                xio[pl.ds(base[kk], 16), :] = jnp.where(
                    row16 == off[kk], rows2[kk], blk).astype(bf16)
            cp0 = pltpu.make_async_copy(xio.at[pl.ds(base[0], 16), :],
                                        out_hbm.at[0, pl.ds(base[0], 16), :], sems.at[0])
            cp1 = pltpu.make_async_copy(xio.at[pl.ds(base[1], 16), :],
                                        out_hbm.at[0, pl.ds(base[1], 16), :], sems.at[1])
            cp0.start()

            @pl.when(base[0] != base[1])
            def _():
                cp1.start()
                cp1.wait()

            cp0.wait()

    for li in range(2):
        last = li == 1
        if li == 0:
            qmax, kmax = lax.fori_loop(1, NSEG, lambda s, c: proj_block(s, c, 0), proj_first())
        else:
            z8 = jnp.zeros((8, 128), f32)
            qmax, kmax = lax.fori_loop(0, NSEG, lambda s, c: proj_block(s, c, 1), (z8, z8))
        bound = DH * jnp.max(qmax) * jnp.max(kmax)
        safe = bound <= SAFE_BOUND

        @pl.when(safe)
        def _():
            lax.fori_loop(0, G // AG, lambda i, c: (attn_groups(i * AG, AG, False), c)[1], 0)

        @pl.when(jnp.logical_not(safe))
        def _():
            lax.fori_loop(0, G, lambda g, c: (attn_groups(g, 1, True), c)[1], 0)

        o_phase(last)
        if li == 0:
            for c in w_cp[3:]:
                c.wait()
        moe_phase(last)


@jax.jit
def pallas_interleave_layers__memory_aug_infini_attn__moe_arch_mod__prompt_kernel(
    A_x: jax.Array,
    A_wq: jax.Array,
    A_wk: jax.Array,
    A_wv: jax.Array,
    A_wo: jax.Array,
    A_beta: jax.Array,
    B_x: jax.Array,
    B_w_r: jax.Array,
    B_w_gate: jax.Array,
    B_w_up: jax.Array,
    B_w_down: jax.Array,
):
    del B_x
    any_spec = pl.BlockSpec(memory_space=pl.ANY)
    vm = pltpu.VMEM
    return pl.pallas_call(
        _kernel,
        out_shape=jax.ShapeDtypeStruct((1, S, D), bf16),
        in_specs=[pl.BlockSpec(memory_space=pltpu.SMEM),
                  pl.BlockSpec(memory_space=vm), pl.BlockSpec(memory_space=vm)] + [any_spec] * 8,
        out_specs=any_spec,
        scratch_shapes=[
            vm((S, D), bf16),
            vm((4, D, D), bf16),
            vm((S, D), f32),
            vm((S // 2, D), i32),
            vm((D // 2, D), i32),
            vm((G, S // 2, 128), i32), vm((G, S // 2, 128), i32),
            vm((G, S // 2, 128), i32), vm((G, S // 2, 128), i32),
            vm((NSEG, D // 2, L), i32),
            vm((G, S // 2, 128), i32),
            vm((S, D), bf16), vm((S, D), bf16),
            vm((NSEG, G, 8, 128), f32),
            vm((2 * H, 128), f32),
            vm((S // OB, 128), f32),
            vm((ONB, OB, D), f32),
            vm((D, F), bf16), vm((D, F), bf16), vm((F, D), bf16),
            pltpu.SemaphoreType.DMA((16,)),
        ],
        compiler_params=pltpu.CompilerParams(vmem_limit_bytes=120 * 1024 * 1024),
    )(np.zeros((1,), np.int32), A_beta, B_w_r, A_x, A_wq, A_wk, A_wv, A_wo, B_w_gate, B_w_up, B_w_down)
```

```python
import math

import jax
import jax.numpy as jnp
import numpy as np
from jax import lax
import jax.experimental.pallas as pl
import jax.experimental.pallas.tpu as pltpu

S = 2048
D = 1024
H = 32
DH = D // H
NSEG = 4
L = S // NSEG
G = 8
F = 3584
OB = 32
OSTEP = 30
ONP = 2
MEMPOS = 2
TORD = 1302
ONB = 5
AG = 2
LAG = 3
FCH = 896

bf16 = jnp.bfloat16
f32 = jnp.float32
i32 = jnp.int32

QSCALE = (DH ** -0.5) * math.log2(math.e)
SAFE_BOUND = 24.0
NEG = -1e30
EPS_BF16 = 1.0013580322265625e-05

_NT = (((1,), (1,)), ((), ()))


def _r(x):
    return x.astype(bf16).astype(f32)


def _pack(x):
    return pltpu.bitcast(x.astype(bf16), i32)


def _unpack(w):
    return pltpu.bitcast(w, bf16)


def _layernorm(xf):
    mean = jnp.sum(xf, axis=1, keepdims=True) * (1.0 / D)
    c = xf - mean
    var = jnp.sum(c * c, axis=1, keepdims=True) * (1.0 / D)
    d = _r(xf - _r(mean))
    s = _r(jnp.sqrt(_r(_r(var) + EPS_BF16)))
    return _r(d * (1.0 / s))


def _phi(t):
    return jnp.where(t > 0, t + 1.0, jnp.exp(t))


def _fold8(x):
    return x.reshape(x.shape[0] // 8, 8, x.shape[1])


def _half(i, n):
    return pl.ds(i // 2 if isinstance(i, int) else pl.multiple_of(i // 2, n // 2), n // 2)


def _kernel(zero_s, beta_ref, wr_ref,
            x_hbm, wq_hbm, wk_hbm, wv_hbm, wo_hbm, wg_hbm, wu_hbm, wd_hbm,
            out_hbm,
            xio, wst, xa, xn, vn, wo, qs, pq, ks, pk, vt, o_s, y_s, x1_s,
            zs, gt, r_s, oc, wg, wu, wd, sems):
    nx = NSEG
    XP = L // 4
    QD = D // 4

    def cp(src, dst, i):
        return pltpu.make_async_copy(src, dst, sems.at[i])

    def wcols(lo, n):
        return wv_hbm.at[:, pl.ds(lo, n)], wst.at[0, :, pl.ds(lo, n)]

    x0_cp = [cp(x_hbm.at[0, pl.ds(i * XP, XP), :], xio.at[pl.ds(i * XP, XP), :], i)
             for i in range(4)]
    x_cp = [None] + [cp(x_hbm.at[0, pl.ds(i * L, L), :], xio.at[pl.ds(i * L, L), :], 3 + i)
                     for i in range(1, nx)]
    wv_cp = [cp(*wcols(0, QD), 7), cp(*wcols(QD, QD), 8), cp(*wcols(2 * QD, 2 * QD), 9)]
    w_cp = [cp(src, dst, 10 + i) for i, (src, dst) in
            enumerate([(wq_hbm, wst.at[1]), (wk_hbm, wst.at[2]), (wo_hbm, wst.at[3]),
                       (wg_hbm, wg), (wu_hbm, wu), (wd_hbm, wd)])]
    for c in x0_cp + wv_cp + w_cp[:2] + x_cp[1:2] + w_cp[2:3] + x_cp[2:] + w_cp[3:]:
        c.start()

    b = jnp.broadcast_to(beta_ref[...].astype(f32).reshape(1, H), (H, H))
    rr = lax.broadcasted_iota(i32, (H, H), 0)
    cc = lax.broadcasted_iota(i32, (H, H), 1)
    bcol = jnp.sum(jnp.where(rr == cc, b, 0.0), axis=1, keepdims=True)
    gsig = _r(jax.nn.sigmoid(jnp.broadcast_to(bcol, (H, 128))))
    gt[0:H, :] = gsig
    gt[H:2 * H, :] = 1.0 - gsig

    lane = lax.broadcasted_iota(i32, (128, 128), 1)
    row = lax.broadcasted_iota(i32, (128, 128), 0)

    def ln_rows(r0, n, src=None, after=None):
        src = xa if src is None else src
        xf = src[pl.ds(r0, n), :].astype(f32)
        if after is not None:
            z = pltpu.bitcast(jnp.concatenate([after] * (n // 8), axis=0), f32)
            xf = jnp.concatenate([xf[:, 0:128] + z, xf[:, 128:]], axis=1)
        xn[_half(r0, n), :] = _pack(_layernorm(xf))

    def ln_block(r0, src=None):
        ln_rows(r0, L, src)

    def pin(w32, ref):
        zero = zero_s[0]
        lk = ref[pl.ds(pl.multiple_of(zero, 8), 8), 0:128] & zero
        head = jnp.concatenate([w32[0:8, 0:128] | lk, w32[0:8, 128:]], axis=1)
        return head if w32.shape[0] == 8 else jnp.concatenate([head, w32[8:]], axis=0)

    CB = 256

    def next_block(s):
        return pl.multiple_of(jnp.minimum(s + 1, NSEG - 1) * L, L)

    def v_cols(s, xb, lo, hi):
        for c0 in range(lo, hi, CB):
            v = jnp.dot(xb, wst[0, :, c0:c0 + CB], preferred_element_type=f32)
            vt[s, c0 // 2:(c0 + CB) // 2, :] = pltpu.bitcast(v.astype(bf16).T, i32)

    def q_cols(s, r0, xb, c0, qmax):
        q = jnp.dot(xb, wst[1, :, c0:c0 + CB], preferred_element_type=f32)
        for j in range(CB // 128):
            g = c0 // 128 + j
            qg = q[:, j * 128:(j + 1) * 128]
            qsc = qg * QSCALE
            qs[g, _half(r0, L), :] = _pack(qsc)
            pq[g, _half(r0, L), :] = _pack(_phi(qg))
            qmax = jnp.maximum(qmax, jnp.max(_fold8(jnp.abs(qsc)), axis=0))
        return qmax

    def k_cols(s, r0, xb, c0, kmax):
        k = jnp.dot(xb, wst[2, :, c0:c0 + CB], preferred_element_type=f32)
        for j in range(CB // 128):
            g = c0 // 128 + j
            kg = k[:, j * 128:(j + 1) * 128]
            ks[g, _half(r0, L), :] = _pack(kg)
            pkg = _phi(kg)
            pk[g, _half(r0, L), :] = _pack(pkg)
            zs[s, g] = jnp.sum(_fold8(pkg), axis=0)
            kmax = jnp.maximum(kmax, jnp.max(_fold8(jnp.abs(kg)), axis=0))
        return kmax

    def proj_first():
        for i in range(4):
            x0_cp[i].wait()
            ln_rows(i * XP, XP, xio)
        for c, lo, hi in zip(wv_cp, (0, QD, 2 * QD), (QD, 2 * QD, D)):
            c.wait()
            vn[:, lo:hi] = jnp.dot(_unpack(xn[0:L // 2, :]), wst[0, :, lo:hi],
                                   preferred_element_type=f32).astype(bf16)
        w_cp[0].wait()
        qmax = kmax = jnp.zeros((8, 128), f32)
        xb = _unpack(xn[0:L // 2, :])
        vt[0] = pltpu.bitcast(vn[...].T, i32)
        for c0 in range(0, D, CB):
            qmax = q_cols(0, 0, xb, c0, qmax)
        w_cp[1].wait()
        x_cp[1].wait()
        xb = _unpack(xn[0:L // 2, :])
        for c0 in range(0, D, CB):
            kmax = k_cols(0, 0, xb, c0, kmax)
        ln_block(L, xio)
        w_cp[2].wait()
        return qmax, kmax

    def proj_block(s, carry, li):
        qmax, kmax = carry
        if li == 0:
            for i in range(2, nx):
                @pl.when(s == i - 1)
                def _():
                    x_cp[i].wait()
        r0 = pl.multiple_of(s * L, L)
        xb = _unpack(xn[_half(r0, L), :])
        v_cols(s, xb, 0, D)
        for c0 in range(0, D, CB):
            qmax = q_cols(s, r0, xb, c0, qmax)
            kmax = k_cols(s, r0, xb, c0, kmax)
        ln_block(next_block(s), xio if li == 0 else xa)
        if li == 0:
            w0 = pl.multiple_of((s - 1) * 168, 8)
            wo[pl.ds(w0, 176), :] = _pack(wst[3, pl.ds(pl.multiple_of(2 * w0, 16), 352), :])
        return qmax, kmax

    def attn_groups(g0, ng, use_max):
        causal = row <= lane
        gs = [g0 + i for i in range(ng)]
        g64 = [pl.multiple_of(g * 64, 64) for g in gs]
        blockdiag = (row >> 5) == (lane >> 5)
        lane16 = lax.broadcasted_iota(i32, (16, 128), 1)
        row16 = lax.broadcasted_iota(i32, (16, 128), 0)
        zmask = (lane16 >> 5) == row16

        def tile(ref, g, s, t):
            return ref[g, (s * L + t * 128) // 2:(s * L + (t + 1) * 128) // 2, :]

        split_diag = not use_max
        causal32 = (lax.broadcasted_iota(i32, (32, 128), 0)
                    <= (lax.broadcasted_iota(i32, (32, 128), 1) & 31))

        def block_transpose(src):
            rows = next(x for x in src if x is not None).shape[0]
            ln = lax.broadcasted_iota(i32, (rows, 128), 1)

            def pick(lo_mask, a, b):
                if a is None and b is None:
                    return None
                return jnp.where(lo_mask, 0.0 if a is None else a, 0.0 if b is None else b)

            def rot(x, n):
                return None if x is None else pltpu.roll(x, n, 1)

            x = [None] * 4
            for i in range(2):
                a, c = src[i], src[i + 2]
                x[i] = pick(ln < 64, a, rot(c, 64))
                x[i + 2] = pick(ln < 64, rot(a, 64), c)
            y = [None] * 4
            for i in (0, 2):
                a, c = x[i], x[i + 1]
                y[i] = pick((ln & 32) == 0, a, rot(c, 32))
                y[i + 1] = pick((ln & 32) == 0, rot(a, 96), c)
            return [jnp.zeros((rows, 128), f32) if v is None else v for v in y]

        def qk(gi, s, t):
            g = gs[gi]
            qt = tile(qs, g, s, t)
            qlane = lax.broadcasted_iota(i32, qt.shape, 1)
            qi = [jnp.where((qlane >> 5) == h, qt, 0) for h in range(4)]
            qm = [_unpack(x) for x in qi]
            Sc = [[None] * (t + 1) for _ in range(4)]
            for j in range(t if split_diag else t + 1):
                kk = _unpack(tile(ks, g, s, j))
                for h in range(4):
                    Sc[h][j] = lax.dot_general(kk, qm[h], _NT, preferred_element_type=f32)
            if not split_diag:
                return Sc, None
            kd = tile(ks, g, s, t)
            T = [None] * 4
            for u in range(4):
                w = _unpack(jnp.concatenate([x[16 * u:16 * u + 16] for x in qi], axis=0))
                T[u] = lax.dot_general(_unpack(kd[0:16 * (u + 1)]), w, _NT,
                                       preferred_element_type=f32)
            return Sc, T

        def tie(x, part):
            n = x.shape[0] - 8
            return jnp.concatenate([x[:n], x[n:] + part * 0.0], axis=0)

        def sm(ScD, t):
            Sc, T = ScD
            P = [None] * 4
            Linv = [None] * 4
            l8 = [None] * 4
            for h in range(4):
                sc = list(Sc[h])
                if not split_diag:
                    sc[t] = jnp.where(causal, sc[t], NEG)
                else:
                    sc = sc[:t]
                if use_max:
                    m = sc[0]
                    for j in range(1, t + 1):
                        m = jnp.maximum(m, sc[j])
                    m = jnp.max(m, axis=0, keepdims=True)
                    p = [jnp.exp2(x - m) for x in sc]
                else:
                    p = [jnp.exp2(x) for x in sc]
                P[h] = []
                for x in p:
                    part = jnp.sum(_fold8(x), axis=0)
                    l8[h] = part if l8[h] is None else l8[h] + part
                    P[h].append(tie(x, part).astype(bf16))
            if split_diag:
                E, ps = [], []
                for u in range(4):
                    e = jnp.exp2(jnp.where(causal32, T[u][32 * u:], NEG))
                    if u:
                        e = jnp.concatenate([jnp.exp2(T[u][:32 * u]), e], axis=0)
                    part = jnp.sum(_fold8(e), axis=0)
                    ps.append(part)
                    E.append(e)
                lh = block_transpose(ps)
                rows = [block_transpose([E[u][32 * r:32 * r + 32] if u >= r else None
                                         for u in range(4)]) for r in range(4)]
                for h in range(4):
                    l8[h] = lh[h] if l8[h] is None else l8[h] + lh[h]
                    P[h].append(jnp.concatenate([rows[r][h] for r in range(4)],
                                                axis=0).astype(bf16))
            for h in range(4):
                Linv[h] = 1.0 / jnp.sum(l8[h], axis=0, keepdims=True)
            return P, Linv

        def pv(PL, gi, s, t, lhs_m):
            g = gs[gi]
            P, Linv = PL
            acc = [None] * 4

            def mem_read():
                pqt = _unpack(tile(pq, g, s, t))
                return lax.dot_general(lhs_m, pqt, _NT, preferred_element_type=f32)

            if lhs_m is not None:
                nd = mem_read()
            for j in range(t + 1):
                for h in range(4):
                    vth = _unpack(vt[s, pl.ds(g64[gi] + 16 * h, 16), j * 128:(j + 1) * 128])
                    o = jnp.dot(vth, P[h][j], preferred_element_type=f32)
                    acc[h] = o if acc[h] is None else acc[h] + o
            outs = []
            for h in range(4):
                o = acc[h] * (gt[pl.ds(H + g * 4 + h, 1), :] * Linv[h])
                if lhs_m is not None:
                    den = nd[128 + h:129 + h, :] + 1e-6
                    o = o + nd[32 * h:32 * h + 32, :] * (gt[pl.ds(g * 4 + h, 1), :] / den)
                outs.append(o)
            ot = jnp.concatenate(outs, axis=0).astype(bf16)
            o_s[g, (s * L + t * 128) // 2:(s * L + (t + 1) * 128) // 2, :] = (
                pltpu.bitcast(ot.T, i32))

        def mem_update(gi, s, R):
            g = gs[gi]
            vtg = _unpack(vt[s, pl.ds(g64[gi], 64), :])
            pks = _unpack(pk[g, s * L // 2:(s + 1) * L // 2, :])
            upd = jnp.dot(vtg, pks, preferred_element_type=f32)
            return upd if R is None else R + upd

        def mem_lhs(gi, s, R):
            g = gs[gi]
            mt = jnp.where(blockdiag, R, 0.0)
            z = zs[0, g]
            for s2 in range(1, s):
                z = z + zs[s2, g]
            z = jnp.sum(z, axis=0, keepdims=True)
            zr = jnp.where(zmask, z, 0.0)
            return jnp.concatenate([mt, zr], axis=0).astype(bf16)

        order = [int(c) for c in str(TORD).zfill(4)]
        steps = [(gi, s, t) for gi in range(ng) for s in range(NSEG) for t in order]
        n = len(steps)
        Sc, PL = {}, {}
        R = None
        lhs = {}
        for i in range(n + LAG):
            if i < n:
                Sc[i] = qk(*steps[i])
                gi, s, t = steps[i]
                if t == order[0] and s == 0:
                    R = None
                    lhs[gi, 0] = None
                if t == order[MEMPOS] and s < NSEG - 1:
                    R = mem_update(gi, s, R)
                    lhs[gi, s + 1] = mem_lhs(gi, s + 1, R)
                PL[i] = sm(Sc.pop(i), t)
            if 0 <= i - LAG < n:
                gi, s, t = steps[i - LAG]
                pv(PL.pop(i - LAG), gi, s, t, lhs[gi, s])

    CP, RP = D // ONP, OB // ONP

    def o_lhs(r0):
        return jnp.concatenate([_unpack(o_s[g, _half(r0, OB), :]) for g in range(G)], axis=1)

    def o_epilogue(refs, r0, out, last):
        xa_, x1_, y_, xo_ = refs
        res = xa_[r0:r0 + RP, :] if last else xo_[r0:r0 + RP, :].astype(f32)
        x1 = _r(res + _r(out))
        x1_[r0:r0 + RP, :] = x1.astype(bf16)
        y = _layernorm(x1)
        y_[r0:r0 + RP, :] = y.astype(bf16)
        if last:
            xo_[r0:r0 + RP, :] = (x1 + y).astype(bf16)
        else:
            xa_[r0:r0 + RP, :] = _r(x1 + y)
        wr = wr_ref[...].astype(f32).reshape(1, D)
        return _r(jnp.sum(y * wr, axis=1, keepdims=True))

    def o_refs(r0, n):
        return [xa.at[pl.ds(r0, n)], x1_s.at[pl.ds(r0, n)], y_s.at[pl.ds(r0, n)],
                xio.at[pl.ds(r0, n)]]

    def o_step(refs, k, blk, src, dst, last):
        if dst is not None:
            ob = o_lhs((blk + 1) * OB)
        rcols = []
        for p in range(ONP):
            if dst is not None:
                dst[:, p * CP:(p + 1) * CP] = jnp.dot(
                    ob, _unpack(wo[:, p * CP:(p + 1) * CP]), preferred_element_type=f32)
            rcols.append(o_epilogue(refs, k * OB + p * RP, src[p * RP:(p + 1) * RP, :], last))
        rb = jnp.broadcast_to(jnp.concatenate(rcols, axis=0), (OB, 128))
        lane_ob = lax.broadcasted_iota(i32, (OB, 128), 1)
        row_ob = lax.broadcasted_iota(i32, (OB, 128), 0)
        r_s[pl.ds(blk, 1), :] = jnp.max(jnp.where(row_ob == lane_ob, rb, -jnp.inf),
                                        axis=0, keepdims=True)

    def o_phase(last):
        nb = S // OB
        oc[0] = jnp.dot(o_lhs(0), _unpack(wo[...]), preferred_element_type=f32)
        nloop = (nb - 2) // OSTEP
        assert OSTEP % ONB == 0

        def out_rows(r0, n):
            return pltpu.make_async_copy(xio.at[pl.ds(r0, n)], out_hbm.at[0, pl.ds(r0, n)],
                                         sems.at[2])

        def body(i, carry):
            if last:
                @pl.when(i > 0)
                def _():
                    out_rows(pl.multiple_of((i - 1) * OSTEP * OB, OSTEP * OB),
                             OSTEP * OB).start()

            refs = o_refs(pl.multiple_of(i * OSTEP * OB, OSTEP * OB), OSTEP * OB)
            for k in range(OSTEP):
                o_step(refs, k, i * OSTEP + k, oc.at[k % ONB], oc.at[(k + 1) % ONB], last)
            return carry

        lax.fori_loop(0, nloop, body, 0)
        b0 = nloop * OSTEP
        if last:
            out_rows((b0 - OSTEP) * OB, OSTEP * OB).start()
        refs = o_refs(b0 * OB, (nb - b0) * OB)
        for k in range(nb - b0):
            o_step(refs, k, b0 + k, oc.at[k % ONB],
                   oc.at[(k + 1) % ONB] if b0 + k + 1 < nb else None, last)
        if last:
            out_rows(b0 * OB, (nb - b0) * OB).start()

    out_cp = pltpu.make_async_copy(xio, out_hbm.at[0], sems.at[2])

    def moe_phase(last):
        r_all = r_s[...]
        ridx = (lax.broadcasted_iota(i32, r_all.shape, 0) * OB
                + lax.broadcasted_iota(i32, r_all.shape, 1)).astype(f32)

        def red(fn, x):
            return fn(fn(x, axis=0, keepdims=True), axis=1, keepdims=True)

        m1 = red(jnp.max, r_all)
        i1f = red(jnp.min, jnp.where(r_all == m1, ridx, 1e9))
        r2 = jnp.where(ridx == i1f, -jnp.inf, r_all)
        m2 = red(jnp.max, r2)
        i2f = red(jnp.min, jnp.where((r2 == m2) & (ridx != i1f), ridx, 1e9))
        idx = [jnp.clip(v[0, 0].astype(i32), 0, S - 1) for v in (i1f, i2f)]
        base = [pl.multiple_of((ix >> 4) << 4, 16) for ix in idx]
        off = [ix & 15 for ix in idx]
        row16 = lax.broadcasted_iota(i32, (16, D), 0)

        def gather(ref):
            res = None
            for kk in range(2):
                blk = ref[pl.ds(base[kk], 16), :].astype(f32)
                one = jnp.sum(jnp.where(row16 == off[kk], blk, 0.0), axis=0, keepdims=True)
                part = jnp.where(row16 == kk, one, 0.0)
                res = part if res is None else res + part
            return res

        ysel = gather(y_s)
        x1sel = gather(x1_s)
        xsel32 = _pack(ysel)
        yf = None
        after = None
        rp = L // (F // FCH)
        for ci, c0 in enumerate(range(0, F, FCH)):
            if not last:
                ln_rows(ci * rp, rp, None, after)
                xsel = _unpack(pin(xsel32, xn))
            else:
                xsel = _unpack(xsel32)
            gte = _r(jnp.dot(xsel, wg[:, c0:c0 + FCH], preferred_element_type=f32))
            after = pltpu.bitcast(gte[0:8, 0:128], i32) & zero_s[0]
            up = _r(jnp.dot(xsel, wu[:, c0:c0 + FCH], preferred_element_type=f32))
            act = _r(gte * jax.nn.sigmoid(gte))
            hcol = (act * up).astype(bf16)
            part = jnp.dot(hcol, wd[c0:c0 + FCH, :], preferred_element_type=f32)
            yf = part if yf is None else yf + part
        rsel = _r(jax.nn.sigmoid(jnp.where(row16 == 0, m1, m2)))
        upd = _r(_r(yf) * rsel)
        x2 = _r(x1sel + _r(ysel + upd))
        rows2 = [jnp.sum(jnp.where(row16 == kk, x2, 0.0), axis=0, keepdims=True)
                 for kk in range(2)]
        if not last:
            xn2 = _layernorm(x2)
            for kk in range(2):
                xa[pl.ds(idx[kk], 1), :] = rows2[kk]
                one = jnp.sum(jnp.where(row16 == kk, xn2, 0.0), axis=0, keepdims=True)
                blk = _unpack(xn[_half(base[kk], 16), :]).astype(f32)
                xn[_half(base[kk], 16), :] = _pack(jnp.where(row16 == off[kk], one, blk))
        else:
            out_cp.wait()
            for kk in range(2):
                blk = xio[pl.ds(base[kk], 16), :].astype(f32)
                xio[pl.ds(base[kk], 16), :] = jnp.where(
                    row16 == off[kk], rows2[kk], blk).astype(bf16)
            cp0 = pltpu.make_async_copy(xio.at[pl.ds(base[0], 16), :],
                                        out_hbm.at[0, pl.ds(base[0], 16), :], sems.at[0])
            cp1 = pltpu.make_async_copy(xio.at[pl.ds(base[1], 16), :],
                                        out_hbm.at[0, pl.ds(base[1], 16), :], sems.at[1])
            cp0.start()

            @pl.when(base[0] != base[1])
            def _():
                cp1.start()
                cp1.wait()

            cp0.wait()

    for li in range(2):
        last = li == 1
        if li == 0:
            qmax, kmax = lax.fori_loop(1, NSEG, lambda s, c: proj_block(s, c, 0), proj_first())
        else:
            z8 = jnp.zeros((8, 128), f32)
            qmax, kmax = lax.fori_loop(0, NSEG, lambda s, c: proj_block(s, c, 1), (z8, z8))
        bound = DH * jnp.max(qmax) * jnp.max(kmax)
        safe = bound <= SAFE_BOUND

        @pl.when(safe)
        def _():
            lax.fori_loop(0, G // AG, lambda i, c: (attn_groups(i * AG, AG, False), c)[1], 0)

        @pl.when(jnp.logical_not(safe))
        def _():
            lax.fori_loop(0, G, lambda g, c: (attn_groups(g, 1, True), c)[1], 0)

        o_phase(last)
        if li == 0:
            for c in w_cp[3:]:
                c.wait()
        moe_phase(last)


@jax.jit
def pallas_interleave_layers__memory_aug_infini_attn__moe_arch_mod__prompt_kernel(
    A_x: jax.Array,
    A_wq: jax.Array,
    A_wk: jax.Array,
    A_wv: jax.Array,
    A_wo: jax.Array,
    A_beta: jax.Array,
    B_x: jax.Array,
    B_w_r: jax.Array,
    B_w_gate: jax.Array,
    B_w_up: jax.Array,
    B_w_down: jax.Array,
):
    del B_x
    any_spec = pl.BlockSpec(memory_space=pl.ANY)
    vm = pltpu.VMEM
    return pl.pallas_call(
        _kernel,
        out_shape=jax.ShapeDtypeStruct((1, S, D), bf16),
        in_specs=[pl.BlockSpec(memory_space=pltpu.SMEM),
                  pl.BlockSpec(memory_space=vm), pl.BlockSpec(memory_space=vm)] + [any_spec] * 8,
        out_specs=any_spec,
        scratch_shapes=[
            vm((S, D), bf16),
            vm((4, D, D), bf16),
            vm((S, D), f32),
            vm((S // 2, D), i32),
            vm((L, D), bf16),
            vm((D // 2, D), i32),
            vm((G, S // 2, 128), i32), vm((G, S // 2, 128), i32),
            vm((G, S // 2, 128), i32), vm((G, S // 2, 128), i32),
            vm((NSEG, D // 2, L), i32),
            vm((G, S // 2, 128), i32),
            vm((S, D), bf16), vm((S, D), bf16),
            vm((NSEG, G, 8, 128), f32),
            vm((2 * H, 128), f32),
            vm((S // OB, 128), f32),
            vm((ONB, OB, D), f32),
            vm((D, F), bf16), vm((D, F), bf16), vm((F, D), bf16),
            pltpu.SemaphoreType.DMA((16,)),
        ],
        compiler_params=pltpu.CompilerParams(vmem_limit_bytes=120 * 1024 * 1024),
    )(np.zeros((1,), np.int32), A_beta, B_w_r, A_x, A_wq, A_wk, A_wv, A_wo, B_w_gate, B_w_up, B_w_down)
```
